```python
import jax
import jax.numpy as jnp

def _softmax(x, axis=-1):
    return jax.nn.softmax(x, axis=axis)
def _gelu(x):
    return jax.nn.gelu(x, approximate=True)
def _silu(x):
    return jax.nn.silu(x)
def _sigmoid(x):
    return jax.nn.sigmoid(x)
def _layernorm(x, axis=-1, eps=1e-5):
    m = jnp.mean(x, axis=axis, keepdims=True)
    v = jnp.var(x, axis=axis, keepdims=True)
    return (x - m) / jnp.sqrt(v + eps)
def _scatter_add(tgt, idx, src, axis=0):
    return tgt.at[idx].add(src)
def _segment_sum(src, seg, n):
    return jax.ops.segment_sum(src, seg, n)
class _Rng:
    def __init__(self, key):
        self._k = key
    def _next(self):
        self._k, sub = jax.random.split(self._k)
        return sub
    def normal(self, shape):
        return jax.random.normal(self._next(), shape, dtype=jnp.bfloat16)
    def randint(self, lo, hi, shape):
        return jax.random.randint(self._next(), shape, lo, hi, dtype=jnp.int32)
    def uniform(self, shape, lo=0.0, hi=1.0):
        return jax.random.uniform(self._next(), shape, jnp.bfloat16, lo, hi)
    def permutation(self, n):
        return jax.random.permutation(self._next(), n)


kernel_name = 'concat_heads__sliding_block_cached__compressed_kv_cla__decode'

def setup_inputs():
    _rng = _Rng(jax.random.key(int.from_bytes(__import__("os").urandom(4), "little")))
    _w = (lambda a: (lambda t: t.astype(jnp.bfloat16) if jnp.issubdtype(t.dtype, jnp.floating) else t)(jnp.asarray(a)))
    def _A_setup():
        B, Sq, D = 4, 1, 512
        Hq, Hkv, Sk, Dh = 32, 32, 4096, 128
        assert Hq % Hkv == 0, (Hq, Hkv)
        return {
            "x": _w((lambda *s: _rng.normal(s) * 0.05)(B, Sq, D)),
            "k_cache": _w((lambda *s: _rng.normal(s) * 0.05)(B, Hkv, Sk, Dh)),
            "v_cache": _w((lambda *s: _rng.normal(s) * 0.05)(B, Hkv, Sk, Dh)),
            "wq": _w((lambda *s: _rng.normal(s) * 0.05)(D, Hq * Dh) * (D ** -0.5)),
            "wo": _w((lambda *s: _rng.normal(s) * 0.05)(Hq * Dh, D) * ((Hq * Dh) ** -0.5)),
        }
    _A_in = _A_setup()

    def _B_setup():
        B, H, Sq, Sk, D, M = 4, 32, 1, 4096, 128, 512
        Dc = 4 * D
        return {
            "x": _w((lambda *s: _rng.normal(s) * 0.05)(B, Sq, M)),
            "c_kv": _w((lambda *s: _rng.normal(s) * 0.05)(B, Sk, Dc)),
            "w_q": _w((lambda *s: _rng.normal(s) * 0.05)(M, H, D) * (M ** -0.5)),
            "w_uk": _w((lambda *s: _rng.normal(s) * 0.05)(Dc, H, D) * (Dc ** -0.5)),
            "w_uv": _w((lambda *s: _rng.normal(s) * 0.05)(Dc, H, D) * (Dc ** -0.5)),
            "w_o": _w((lambda *s: _rng.normal(s) * 0.05)(H, D, M) * ((H * D) ** -0.5)),
        }
    _B_in = _B_setup()

    return {
        "A_x": _A_in["x"],
        "A_k_cache": _A_in["k_cache"],
        "A_v_cache": _A_in["v_cache"],
        "A_wq": _A_in["wq"],
        "A_wo": _A_in["wo"],
        "B_x": _B_in["x"],
        "B_c_kv": _B_in["c_kv"],
        "B_w_q": _B_in["w_q"],
        "B_w_uk": _B_in["w_uk"],
        "B_w_uv": _B_in["w_uv"],
        "B_w_o": _B_in["w_o"],
    }

def reference(A_x, A_k_cache, A_v_cache, A_wq, A_wo, B_x, B_c_kv, B_w_q, B_w_uk, B_w_uv, B_w_o):
    def _A_ref(x, k_cache, v_cache, wq, wo):
        B, Sq, D = x.shape
        Hq, Dh = 32, 128
        Hkv, Sk = k_cache.shape[1], k_cache.shape[2]
        W = min(4096, max(256, Sk // 4))
        rep = Hq // Hkv
        q = (lambda x, *d: x.transpose(*d))((x @ wq).reshape(B, Sq, Hq, Dh), 0, 2, 1, 3)
        k = jnp.repeat(k_cache[:, :, Sk - W:, :], rep, axis=1)
        v = jnp.repeat(v_cache[:, :, Sk - W:, :], rep, axis=1)
        scores = jnp.einsum("bhqd,bhkd->bhqk", q, k) * (Dh ** -0.5)
        p = _softmax(scores, axis=-1)
        o = jnp.einsum("bhqk,bhkd->bhqd", p, v)
        return (lambda x, *d: x.transpose(*d))(o, 0, 2, 1, 3).reshape(B, Sq, Hq * Dh) @ wo

    def _B_ref(x, c_kv, w_q, w_uk, w_uv, w_o):
        B, Sq, M = x.shape[0], x.shape[1], x.shape[2]
        Sk = c_kv.shape[1]
        H, D = w_q.shape[1], w_q.shape[2]
        q = jnp.einsum("bqm,mhd->bhqd", x, w_q)
        k = jnp.einsum("bkc,chd->bhkd", c_kv, w_uk)
        v = jnp.einsum("bkc,chd->bhkd", c_kv, w_uv)
        scores = jnp.einsum("bhqd,bhkd->bhqk", q, k) * (D ** -0.5)
        off = Sk - Sq
        qi = jnp.arange(Sq)[:, None]
        kj = jnp.arange(Sk)[None, :]
        cmask = kj <= (qi + off)
        scores = jnp.where(cmask[None, None], scores, -1e9)
        p = _softmax(scores, axis=-1)
        ctx = jnp.einsum("bhqk,bhkd->bhqd", p, v)
        return jnp.einsum("bhqd,hdm->bqm", ctx, w_o)

    a = _A_ref(A_x, A_k_cache, A_v_cache, A_wq, A_wo)
    b = _B_ref(B_x, B_c_kv, B_w_q, B_w_uk, B_w_uv, B_w_o)
    return jnp.concatenate([a, b], axis=-1)
```

```python
import functools

import jax
import jax.numpy as jnp
from jax import lax
import jax.experimental.pallas as pl
import jax.experimental.pallas.tpu as pltpu

BF = jnp.bfloat16
F32 = jnp.float32
NT = (((1,), (1,)), ((), ()))

NB = 4
NH = 32
DH = 128
DM = 512
SK = 4096
WIN = 1024
NSLOT = 8
CCH = 1024


def _dot(a, b):
    return jnp.dot(a, b, preferred_element_type=F32)


def _dot_nt(a, b):
    return lax.dot_general(a, b, NT, preferred_element_type=F32)


def _deinterleave(src_ref, dst_ref):
    s32 = src_ref.bitcast(jnp.uint32)
    lo_mask = jnp.uint32(0x0000FFFF)
    hi_mask = jnp.uint32(0xFFFF0000)

    def body(i, c):
        rows = pl.ds(pl.multiple_of(i * 16, 16), 16)
        for j in range(NH // 2):
            a = s32[i, pl.ds(j, 8, stride=32), :]
            b = s32[i, pl.ds(16 + j, 8, stride=32), :]
            dst_ref[2 * j, rows, :] = pltpu.bitcast((a & lo_mask) | (b << 16), BF)
            dst_ref[2 * j + 1, rows, :] = pltpu.bitcast((a >> 16) | (b & hi_mask), BF)
        return c
    lax.fori_loop(0, DM // 16, body, 0)


def _kernel(xa_hbm, k_hbm, v_hbm, wq_hbm, wo_hbm, xb_hbm, c_hbm, bwq_hbm, bwuk_hbm, bwuv_hbm, bwo_hbm,
            out_ref,
            xa_v, xb_v, wq_v, wo_v, bwq_v, bwuk_v, bwuv_v, bwo_v, c_v, k_v, v_v,
            qa_s, qlat_s, clat_s, w1_s, w2_s,
            wsem, csem, ksem, vsem):
    scale = DH ** -0.5
    ncc = SK // CCH

    def wcopy(i):
        src, dst = [(xa_hbm, xa_v), (xb_hbm, xb_v), (wq_hbm, wq_v), (bwq_hbm, bwq_v), (bwuk_hbm, bwuk_v),
                    (bwuv_hbm, bwuv_v), (bwo_hbm, bwo_v), (wo_hbm, wo_v)][i]
        return pltpu.make_async_copy(src, dst, wsem.at[i])

    def ccopy(b, r):
        return pltpu.make_async_copy(c_hbm.at[b, pl.ds(r * CCH, CCH), :],
                                     c_v.at[b, pl.ds(r * CCH, CCH), :], csem.at[b * ncc + r])

    def kcopy(h, b, slot):
        return pltpu.make_async_copy(k_hbm.at[b, h, pl.ds(SK - WIN, WIN), :], k_v.at[slot, b],
                                     ksem.at[slot * NB + b])

    def vcopy(h, b, slot):
        return pltpu.make_async_copy(v_hbm.at[b, h, pl.ds(SK - WIN, WIN), :], v_v.at[slot, b],
                                     vsem.at[slot * NB + b])

    for i in (0, 1, 3, 4):
        wcopy(i).start()
    for b in range(NB):
        for r in range(ncc):
            ccopy(b, r).start()
    for i in (5, 6, 2, 7):
        wcopy(i).start()
    for s in range(NSLOT):
        for b in range(NB):
            kcopy(s, b, s).start()
        for b in range(NB):
            vcopy(s, b, s).start()

    row8 = lax.broadcasted_iota(jnp.int32, (8, 1), 0)

    def pad8(x4):
        return jnp.concatenate([x4.astype(F32), jnp.zeros((4, x4.shape[1]), F32)], axis=0).astype(BF)

    wcopy(0).wait()
    wcopy(1).wait()
    wcopy(3).wait()
    wcopy(4).wait()
    xb = pad8(xb_v[...])
    _deinterleave(bwq_v, w1_s)
    _deinterleave(bwuk_v, w2_s)

    def qlat_body(h, c):
        q = _dot(xb, w1_s[h]).astype(BF)
        ql = _dot_nt(q, w2_s[h]) * scale
        for cb in range(DM // 128):
            qlat_s[cb, pl.ds(pl.multiple_of(h * 8, 8), 8), :] = ql[:, cb * 128:(cb + 1) * 128]
        return c
    lax.fori_loop(0, NH, qlat_body, 0, unroll=2)

    clat_s[...] = jnp.zeros(clat_s.shape, F32)
    for b in range(NB):
        ql = jnp.concatenate([qlat_s[cb, pl.ds(b, NH, stride=8), :] for cb in range(DM // 128)],
                             axis=1).astype(BF)
        ss = []
        for r in range(ncc):
            ccopy(b, r).wait()
            ss.append(_dot_nt(ql, c_v[b, pl.ds(r * CCH, CCH), :]))
        s = jnp.concatenate(ss, axis=1)
        m = jnp.max(s, axis=1, keepdims=True)
        p = jnp.exp(s - m)
        l = jnp.sum(p, axis=1, keepdims=True)
        cl = _dot(p.astype(BF), c_v[b]) / l
        for cb in range(DM // 128):
            clat_s[cb, pl.ds(b, NH, stride=8), :] = cl[:, cb * 128:(cb + 1) * 128]

    wcopy(5).wait()
    wcopy(6).wait()
    _deinterleave(bwuv_v, w1_s)

    def outb_body(h, acc):
        cl = jnp.concatenate([clat_s[cb, pl.ds(pl.multiple_of(h * 8, 8), 8), :] for cb in range(DM // 128)],
                             axis=1).astype(BF)
        ctx = _dot(cl, w1_s[h]).astype(BF)
        return acc + _dot(ctx, bwo_v[pl.ds(pl.multiple_of(h * DH, DH), DH), :])
    out_b = lax.fori_loop(0, NH, outb_body, jnp.zeros((8, DM), F32), unroll=2)
    out_ref[:, DM:] = out_b[:NB].astype(BF)

    wcopy(2).wait()
    xa = pad8(xa_v[...])
    qa = _dot(xa, wq_v[...]) * scale
    for h in range(NH):
        qa_s[h] = qa[:, h * DH:(h + 1) * DH]
    wcopy(7).wait()

    def a_body(h, acc):
        slot = h % NSLOT
        q = qa_s[h].astype(BF)
        s = jnp.zeros((8, WIN), F32)
        for b in range(NB):
            kcopy(h, b, slot).wait()
            sb = _dot_nt(q, k_v[slot, b])
            s = jnp.where(row8 == b, sb, s)
        m = jnp.max(s, axis=1, keepdims=True)
        p = jnp.exp(s - m)
        l = jnp.sum(p, axis=1, keepdims=True)
        pb = p.astype(BF)
        o = jnp.zeros((8, DH), F32)
        for b in range(NB):
            vcopy(h, b, slot).wait()
            ob = _dot(pb, v_v[slot, b])
            o = jnp.where(row8 == b, ob, o)
        o = (o / l).astype(BF)

        @pl.when(h + NSLOT < NH)
        def _():
            for b in range(NB):
                kcopy(h + NSLOT, b, slot).start()
            for b in range(NB):
                vcopy(h + NSLOT, b, slot).start()
        return acc + _dot(o, wo_v[pl.ds(pl.multiple_of(h * DH, DH), DH), :])
    out_a = lax.fori_loop(0, NH, a_body, jnp.zeros((8, DM), F32))
    out_ref[:, :DM] = out_a[:NB].astype(BF)


@jax.jit
def pallas_concat_heads__sliding_block_cached__compressed_kv_cla__decode_kernel(
    A_x: jax.Array,
    A_k_cache: jax.Array,
    A_v_cache: jax.Array,
    A_wq: jax.Array,
    A_wo: jax.Array,
    B_x: jax.Array,
    B_c_kv: jax.Array,
    B_w_q: jax.Array,
    B_w_uk: jax.Array,
    B_w_uv: jax.Array,
    B_w_o: jax.Array,
):
    ncc = SK // CCH
    out = pl.pallas_call(
        _kernel,
        out_shape=jax.ShapeDtypeStruct((NB, 2 * DM), BF),
        in_specs=[pl.BlockSpec(memory_space=pl.ANY)] * 11,
        out_specs=pl.BlockSpec(memory_space=pltpu.VMEM),
        scratch_shapes=[
            pltpu.VMEM((NB, DM), BF), pltpu.VMEM((NB, DM), BF),
            pltpu.VMEM((DM, NH * DH), BF), pltpu.VMEM((NH * DH, DM), BF),
            pltpu.VMEM((32, 512, DH), BF), pltpu.VMEM((32, 512, DH), BF), pltpu.VMEM((32, 512, DH), BF),
            pltpu.VMEM((NH * DH, DM), BF),
            pltpu.VMEM((NB, SK, DM), BF),
            pltpu.VMEM((NSLOT, NB, WIN, DH), BF), pltpu.VMEM((NSLOT, NB, WIN, DH), BF),
            pltpu.VMEM((NH, 8, DH), F32),
            pltpu.VMEM((DM // 128, NH * 8, 128), F32),
            pltpu.VMEM((DM // 128, NH * 8, 128), F32),
            pltpu.VMEM((NH, DM, DH), BF), pltpu.VMEM((NH, DM, DH), BF),
            pltpu.SemaphoreType.DMA((8,)),
            pltpu.SemaphoreType.DMA((NB * ncc,)),
            pltpu.SemaphoreType.DMA((NSLOT * NB,)),
            pltpu.SemaphoreType.DMA((NSLOT * NB,)),
        ],
        compiler_params=pltpu.CompilerParams(vmem_limit_bytes=100 * 1024 * 1024),
    )(
        A_x.reshape(NB, DM), A_k_cache, A_v_cache, A_wq, A_wo,
        B_x.reshape(NB, DM), B_c_kv,
        B_w_q.reshape(32, 512, DH), B_w_uk.reshape(32, 512, DH), B_w_uv.reshape(32, 512, DH),
        B_w_o.reshape(NH * DH, DM),
    )
    return out.reshape(NB, 1, 2 * DM)
```

```python
import functools

import jax
import jax.numpy as jnp
from jax import lax
import jax.experimental.pallas as pl
import jax.experimental.pallas.tpu as pltpu

BF = jnp.bfloat16
F32 = jnp.float32
NT = (((1,), (1,)), ((), ()))

NB = 4
NH = 32
DH = 128
DM = 512
SK = 4096
WIN = 1024
NSLOT = 8
CCH = 1024


def _dot(a, b):
    return jnp.dot(a, b, preferred_element_type=F32)


def _dot_nt(a, b):
    return lax.dot_general(a, b, NT, preferred_element_type=F32)


def _deinterleave(src_ref, dst_ref):
    s32 = src_ref.bitcast(jnp.uint32)
    lo_mask = jnp.uint32(0x0000FFFF)
    hi_mask = jnp.uint32(0xFFFF0000)

    def body(i, c):
        rows = pl.ds(pl.multiple_of(i * 16, 16), 16)
        for j in range(NH // 2):
            a = s32[i, pl.ds(j, 8, stride=32), :]
            b = s32[i, pl.ds(16 + j, 8, stride=32), :]
            dst_ref[2 * j, rows, :] = pltpu.bitcast((a & lo_mask) | (b << 16), BF)
            dst_ref[2 * j + 1, rows, :] = pltpu.bitcast((a >> 16) | (b & hi_mask), BF)
        return c
    lax.fori_loop(0, DM // 16, body, 0)


def _kernel(xa_hbm, k_hbm, v_hbm, wq_hbm, wo_hbm, xb_hbm, c_hbm, bwq_hbm, bwuk_hbm, bwuv_hbm, bwo_hbm,
            out_ref,
            xa_v, xb_v, wq_v, wo_v, bwq_v, bwuk_v, bwuv_v, bwo_v, c_v, k_v, v_v,
            qa_s, qlat_s, clat_s, w1_s, w2_s,
            sem):
    scale = DH ** -0.5
    ncc = SK // CCH

    def wcopy(i):
        src, dst = [(xa_hbm, xa_v), (xb_hbm, xb_v), (wq_hbm, wq_v), (bwq_hbm, bwq_v), (bwuk_hbm, bwuk_v),
                    (bwuv_hbm, bwuv_v), (bwo_hbm, bwo_v), (wo_hbm, wo_v)][i]
        return pltpu.make_async_copy(src, dst, sem.at[i])

    def ccopy(b, r):
        return pltpu.make_async_copy(c_hbm.at[b, pl.ds(r * CCH, CCH), :],
                                     c_v.at[b, pl.ds(r * CCH, CCH), :], sem.at[8 + b * ncc + r])

    def kcopy(h, b, slot):
        return pltpu.make_async_copy(k_hbm.at[b, h, pl.ds(SK - WIN, WIN), :], k_v.at[slot, b],
                                     sem.at[8 + NB * ncc + slot * 2 * NB + b])

    def vcopy(h, b, slot):
        return pltpu.make_async_copy(v_hbm.at[b, h, pl.ds(SK - WIN, WIN), :], v_v.at[slot, b],
                                     sem.at[8 + NB * ncc + slot * 2 * NB + NB + b])

    for i in (0, 1, 3, 4):
        wcopy(i).start()
    for b in range(NB):
        for r in range(ncc):
            ccopy(b, r).start()
    for i in (5, 6, 2, 7):
        wcopy(i).start()
    for s in range(NSLOT):
        for b in range(NB):
            kcopy(s, b, s).start()
        for b in range(NB):
            vcopy(s, b, s).start()

    row8 = lax.broadcasted_iota(jnp.int32, (8, 1), 0)

    def pad8(x4):
        return jnp.concatenate([x4.astype(F32), jnp.zeros((4, x4.shape[1]), F32)], axis=0).astype(BF)

    wcopy(0).wait()
    wcopy(1).wait()
    wcopy(3).wait()
    wcopy(4).wait()
    xb = pad8(xb_v[...])
    _deinterleave(bwq_v, w1_s)
    _deinterleave(bwuk_v, w2_s)

    def qlat_body(h, c):
        q = _dot(xb, w1_s[h]).astype(BF)
        ql = _dot_nt(q, w2_s[h]) * scale
        for cb in range(DM // 128):
            qlat_s[cb, pl.ds(pl.multiple_of(h * 8, 8), 8), :] = ql[:, cb * 128:(cb + 1) * 128]
        return c
    lax.fori_loop(0, NH, qlat_body, 0, unroll=2)

    clat_s[...] = jnp.zeros(clat_s.shape, F32)
    for b in range(NB):
        ql = jnp.concatenate([qlat_s[cb, pl.ds(b, NH, stride=8), :] for cb in range(DM // 128)],
                             axis=1).astype(BF)
        ss = []
        for r in range(ncc):
            ccopy(b, r).wait()
            ss.append(_dot_nt(ql, c_v[b, pl.ds(r * CCH, CCH), :]))
        s = jnp.concatenate(ss, axis=1)
        m = jnp.max(s, axis=1, keepdims=True)
        p = jnp.exp(s - m)
        l = jnp.sum(p, axis=1, keepdims=True)
        cl = _dot(p.astype(BF), c_v[b]) / l
        for cb in range(DM // 128):
            clat_s[cb, pl.ds(b, NH, stride=8), :] = cl[:, cb * 128:(cb + 1) * 128]

    wcopy(5).wait()
    wcopy(6).wait()
    _deinterleave(bwuv_v, w1_s)

    def outb_body(h, acc):
        cl = jnp.concatenate([clat_s[cb, pl.ds(pl.multiple_of(h * 8, 8), 8), :] for cb in range(DM // 128)],
                             axis=1).astype(BF)
        ctx = _dot(cl, w1_s[h]).astype(BF)
        return acc + _dot(ctx, bwo_v[pl.ds(pl.multiple_of(h * DH, DH), DH), :])
    out_b = lax.fori_loop(0, NH, outb_body, jnp.zeros((8, DM), F32), unroll=2)
    out_ref[:, DM:] = out_b[:NB].astype(BF)

    wcopy(2).wait()
    xa = pad8(xa_v[...])
    qa = _dot(xa, wq_v[...]) * scale
    for h in range(NH):
        qa_s[h] = qa[:, h * DH:(h + 1) * DH]
    wcopy(7).wait()

    def a_body(h, acc):
        slot = h % NSLOT
        q = qa_s[h].astype(BF)
        s = jnp.zeros((8, WIN), F32)
        for b in range(NB):
            kcopy(h, b, slot).wait()
            sb = _dot_nt(q, k_v[slot, b])
            s = jnp.where(row8 == b, sb, s)
        m = jnp.max(s, axis=1, keepdims=True)
        p = jnp.exp(s - m)
        l = jnp.sum(p, axis=1, keepdims=True)
        pb = p.astype(BF)
        o = jnp.zeros((8, DH), F32)
        for b in range(NB):
            vcopy(h, b, slot).wait()
            ob = _dot(pb, v_v[slot, b])
            o = jnp.where(row8 == b, ob, o)
        o = (o / l).astype(BF)

        @pl.when(h + NSLOT < NH)
        def _():
            for b in range(NB):
                kcopy(h + NSLOT, b, slot).start()
            for b in range(NB):
                vcopy(h + NSLOT, b, slot).start()
        return acc + _dot(o, wo_v[pl.ds(pl.multiple_of(h * DH, DH), DH), :])
    out_a = lax.fori_loop(0, NH, a_body, jnp.zeros((8, DM), F32))
    out_ref[:, :DM] = out_a[:NB].astype(BF)


@jax.jit
def pallas_concat_heads__sliding_block_cached__compressed_kv_cla__decode_kernel(
    A_x: jax.Array,
    A_k_cache: jax.Array,
    A_v_cache: jax.Array,
    A_wq: jax.Array,
    A_wo: jax.Array,
    B_x: jax.Array,
    B_c_kv: jax.Array,
    B_w_q: jax.Array,
    B_w_uk: jax.Array,
    B_w_uv: jax.Array,
    B_w_o: jax.Array,
):
    ncc = SK // CCH
    out = pl.pallas_call(
        _kernel,
        out_shape=jax.ShapeDtypeStruct((NB, 2 * DM), BF),
        in_specs=[pl.BlockSpec(memory_space=pl.ANY)] * 11,
        out_specs=pl.BlockSpec(memory_space=pltpu.VMEM),
        scratch_shapes=[
            pltpu.VMEM((NB, DM), BF), pltpu.VMEM((NB, DM), BF),
            pltpu.VMEM((DM, NH * DH), BF), pltpu.VMEM((NH * DH, DM), BF),
            pltpu.VMEM((32, 512, DH), BF), pltpu.VMEM((32, 512, DH), BF), pltpu.VMEM((32, 512, DH), BF),
            pltpu.VMEM((NH * DH, DM), BF),
            pltpu.VMEM((NB, SK, DM), BF),
            pltpu.VMEM((NSLOT, NB, WIN, DH), BF), pltpu.VMEM((NSLOT, NB, WIN, DH), BF),
            pltpu.VMEM((NH, 8, DH), F32),
            pltpu.VMEM((DM // 128, NH * 8, 128), F32),
            pltpu.VMEM((DM // 128, NH * 8, 128), F32),
            pltpu.VMEM((NH, DM, DH), BF), pltpu.VMEM((NH, DM, DH), BF),
            pltpu.SemaphoreType.DMA((8 + NB * ncc + 2 * NSLOT * NB,)),
        ],
        compiler_params=pltpu.CompilerParams(vmem_limit_bytes=100 * 1024 * 1024,
                                             disable_bounds_checks=True,
                                             disable_semaphore_checks=True),
    )(
        A_x.reshape(NB, DM), A_k_cache, A_v_cache, A_wq, A_wo,
        B_x.reshape(NB, DM), B_c_kv,
        B_w_q.reshape(32, 512, DH), B_w_uk.reshape(32, 512, DH), B_w_uv.reshape(32, 512, DH),
        B_w_o.reshape(NH * DH, DM),
    )
    return out.reshape(NB, 1, 2 * DM)
```

```python
import jax
import jax.numpy as jnp
from jax import lax
import jax.experimental.pallas as pl
import jax.experimental.pallas.tpu as pltpu

BF = jnp.bfloat16
F32 = jnp.float32
NT = (((1,), (1,)), ((), ()))

NB = 4
NH = 32
DH = 128
DM = 512
SK = 4096
WIN = 1024
NSLOT = 4
NU = 32
F16 = 10


def _dot(a, b):
    return jnp.dot(a, b, preferred_element_type=F32)


def _dot_nt(a, b):
    return lax.dot_general(a, b, NT, preferred_element_type=F32)


def _kernel(xa_hbm, k_hbm, v_hbm, wq_hbm, wo_hbm, xb_hbm, c_hbm, bwq_hbm, bwuk_hbm, bwuv_hbm, bwo_hbm,
            out_ref,
            xa_v, xb_v, wq_v, wo_v, bwq_v, bwuk_v, bwuv_v, bwo_v, c_v, k_v, v_v,
            qa_s, qb_s, qlat_s, clat_s, s_s, w1_s, w2_s,
            sem):
    scale = DH ** -0.5

    def split_rows(src, dst, n, s):
        r = n * F16 // 16
        return ((src.at[pl.ds(0, r), :], dst.at[pl.ds(0, r), :], sem.at[s]),
                (src.at[pl.ds(r, n - r), :], dst.at[pl.ds(r, n - r), :], sem.at[s]),
                (src, dst, sem.at[s]))

    def unit3(src, dst, off=0):
        return lambda i: split_rows(src.at[off + i], dst.at[off + i], src.shape[1], i)

    def unit_wq(i):
        rows = pl.ds(pl.multiple_of(i * 16, 16), 16)
        n = NH * DH
        c = n * F16 // 16
        return ((wq_hbm.at[rows, pl.ds(0, c)], wq_v.at[rows, pl.ds(0, c)], sem.at[i]),
                (wq_hbm.at[rows, pl.ds(c, n - c)], wq_v.at[rows, pl.ds(c, n - c)], sem.at[i]),
                (wq_hbm.at[rows, :], wq_v.at[rows, :], sem.at[i]))

    def unit_kv(h, t, half):
        src, dst = ((k_hbm, k_v), (v_hbm, v_v))[t // NB]
        b = t % NB
        n = WIN // 2
        return split_rows(src.at[b, h, pl.ds(SK - WIN + half * n, n), :],
                          dst.at[h % NSLOT, b, pl.ds(half * n, n), :], n,
                          (h % 2) * 16 + t * 2 + half)

    def start(u):
        pltpu.make_async_copy(*u[0]).start(priority=1)
        pltpu.make_async_copy(*u[1]).start(priority=0)

    def wait(u):
        pltpu.make_async_copy(*u[2]).wait()

    def block(cur, nxt, body, init):
        def step(i, c):
            wait(cur(i))
            start(nxt(i))
            return body(i, c)
        return lax.fori_loop(0, NU, step, init)

    u_bwq, u_bwuk, u_bwuv = unit3(bwq_hbm, bwq_v), unit3(bwuk_hbm, bwuk_v), unit3(bwuv_hbm, bwuv_v)
    u_bwo, u_wo = unit3(bwo_hbm, bwo_v), unit3(wo_hbm, wo_v)
    u_c = [unit3(c_hbm, c_v, b * NU) for b in range(NB)]
    xa_cp = pltpu.make_async_copy(xa_hbm, xa_v, sem.at[NU])
    xb_cp = pltpu.make_async_copy(xb_hbm, xb_v, sem.at[NU + 1])

    for i in range(NU):
        pltpu.make_async_copy(*u_bwq(i)[2]).start(priority=1)
    xa_cp.start()
    xb_cp.start()

    row8 = lax.broadcasted_iota(jnp.int32, (8, 1), 0)

    def pad8(x4):
        return jnp.concatenate([x4.astype(F32), jnp.zeros((4, x4.shape[1]), F32)], axis=0).astype(BF)

    lo_mask = jnp.uint32(0x0000FFFF)
    hi_mask = jnp.uint32(0xFFFF0000)

    def deinterleave(src_ref, dst_ref, i):
        s32 = src_ref.bitcast(jnp.uint32)
        rows = pl.ds(pl.multiple_of(i * 16, 16), 16)
        for j in range(NH // 2):
            a = s32[i, pl.ds(j, 8, stride=32), :]
            b = s32[i, pl.ds(16 + j, 8, stride=32), :]
            dst_ref[2 * j, rows, :] = pltpu.bitcast((a & lo_mask) | (b << 16), BF)
            dst_ref[2 * j + 1, rows, :] = pltpu.bitcast((a >> 16) | (b & hi_mask), BF)

    def body(i, c):
        deinterleave(bwq_v, w1_s, i)
        return c
    block(u_bwq, u_bwuk, body, 0)

    xa_cp.wait()
    xb_cp.wait()
    xa = pad8(xa_v[...])
    xb = pad8(xb_v[...])

    def body(i, c):
        deinterleave(bwuk_v, w2_s, i)
        qb_s[i] = _dot(xb, w1_s[i])
        return c
    block(u_bwuk, unit_wq, body, 0)

    def body(h, c):
        ql = _dot_nt(qb_s[h].astype(BF), w2_s[h]) * scale
        for cb in range(DM // 128):
            qlat_s[cb, pl.ds(pl.multiple_of(h * 8, 8), 8), :] = ql[:, cb * 128:(cb + 1) * 128]
        return c
    block(unit_wq, u_c[0], body, 0)

    clat_s[...] = jnp.zeros(clat_s.shape, F32)
    m_prev = None
    for b in range(NB + 1):
        if b < NB:
            ql = jnp.concatenate([qlat_s[cb, pl.ds(b, NH, stride=8), :] for cb in range(DM // 128)],
                                 axis=1).astype(BF)

        def body(i, c, b=b, m_prev=m_prev, ql=ql):
            m_run, l_run, acc = c
            if b < NB:
                s = _dot_nt(ql, c_v[b * NU + i])
                s_s[b % 2, i] = s
                m_run = jnp.maximum(m_run, s)
            if b == 0:
                cols = pl.ds(pl.multiple_of(i * DH, DH), DH)
                qa_s[i] = _dot(xa, wq_v[:, cols]) * scale
            else:
                p = jnp.exp(s_s[(b - 1) % 2, i] - m_prev)
                l_run = l_run + p
                acc = acc + _dot(p.astype(BF), c_v[(b - 1) * NU + i])
            return m_run, l_run, acc
        init = (jnp.full((NH, 128), -jnp.inf, F32), jnp.zeros((NH, 128), F32), jnp.zeros((NH, DM), F32))
        cur = u_c[b] if b < NB else u_wo
        nxt = u_c[b + 1] if b + 1 < NB else (u_wo if b + 1 == NB else u_bwuv)
        m_run, l_run, acc = block(cur, nxt, body, init)
        if b > 0:
            cl = acc / jnp.sum(l_run, axis=1, keepdims=True)
            for cb in range(DM // 128):
                clat_s[cb, pl.ds(b - 1, NH, stride=8), :] = cl[:, cb * 128:(cb + 1) * 128]
        if b < NB:
            m_prev = jnp.broadcast_to(jnp.max(m_run, axis=1, keepdims=True), (NH, 128))

    def body(i, c):
        deinterleave(bwuv_v, w1_s, i)
        return c
    block(u_bwuv, u_bwo, body, 0)

    for i in range(NU):
        wait(u_bwo(i))
        start(unit_kv(i // 16, (i % 16) // 2, i % 2))

    def a_body(h, carry):
        acc_a, acc_b, o_prev = carry
        slot = h % NSLOT
        hn = jnp.minimum(h + 2, NH - 1)

        def tick(t, half):
            wait(unit_kv(h, t, half))

            @pl.when(h + 2 < NH)
            def _():
                start(unit_kv(hn, t, half))

        q = qa_s[h].astype(BF)
        s = jnp.zeros((8, WIN), F32)
        o = jnp.zeros((8, DH), F32)
        for t in range(2 * NB):
            tick(t, 0)
            if t == 0:
                acc_a = acc_a + _dot(o_prev, wo_v[jnp.maximum(h - 1, 0)])
            elif t == 1:
                cl = jnp.concatenate([clat_s[cb, pl.ds(pl.multiple_of(h * 8, 8), 8), :]
                                      for cb in range(DM // 128)], axis=1).astype(BF)
                ctx = _dot(cl, w1_s[h]).astype(BF)
            elif t == 2:
                acc_b = acc_b + _dot(ctx, bwo_v[h])
            elif t == NB:
                m = jnp.max(s, axis=1, keepdims=True)
                p = jnp.exp(s - m)
                l = jnp.sum(p, axis=1, keepdims=True)
                pb = p.astype(BF)
            tick(t, 1)
            if t < NB:
                s = jnp.where(row8 == t, _dot_nt(q, k_v[slot, t]), s)
            else:
                o = jnp.where(row8 == t - NB, _dot(pb, v_v[slot, t - NB]), o)
        return acc_a, acc_b, (o / l).astype(BF)

    zero = jnp.zeros((8, DM), F32)
    acc_a, acc_b, o_last = lax.fori_loop(0, NH, a_body, (zero, zero, jnp.zeros((8, DH), BF)))
    acc_a = acc_a + _dot(o_last, wo_v[NH - 1])
    out_ref[:, :DM] = acc_a[:NB].astype(BF)
    out_ref[:, DM:] = acc_b[:NB].astype(BF)


@jax.jit
def pallas_concat_heads__sliding_block_cached__compressed_kv_cla__decode_kernel(
    A_x: jax.Array,
    A_k_cache: jax.Array,
    A_v_cache: jax.Array,
    A_wq: jax.Array,
    A_wo: jax.Array,
    B_x: jax.Array,
    B_c_kv: jax.Array,
    B_w_q: jax.Array,
    B_w_uk: jax.Array,
    B_w_uv: jax.Array,
    B_w_o: jax.Array,
):
    out = pl.pallas_call(
        _kernel,
        out_shape=jax.ShapeDtypeStruct((NB, 2 * DM), BF),
        in_specs=[pl.BlockSpec(memory_space=pl.ANY)] * 11,
        out_specs=pl.BlockSpec(memory_space=pltpu.VMEM),
        scratch_shapes=[
            pltpu.VMEM((NB, DM), BF), pltpu.VMEM((NB, DM), BF),
            pltpu.VMEM((DM, NH * DH), BF), pltpu.VMEM((NH, DH, DM), BF),
            pltpu.VMEM((NU, 512, DH), BF), pltpu.VMEM((NU, 512, DH), BF), pltpu.VMEM((NU, 512, DH), BF),
            pltpu.VMEM((NH, DH, DM), BF),
            pltpu.VMEM((NB * NU, SK // NU, DM), BF),
            pltpu.VMEM((NSLOT, NB, WIN, DH), BF), pltpu.VMEM((NSLOT, NB, WIN, DH), BF),
            pltpu.VMEM((NH, 8, DH), F32), pltpu.VMEM((NH, 8, DH), F32),
            pltpu.VMEM((DM // 128, NH * 8, 128), F32),
            pltpu.VMEM((DM // 128, NH * 8, 128), F32),
            pltpu.VMEM((2, NU, NH, 128), F32),
            pltpu.VMEM((NH, DM, DH), BF), pltpu.VMEM((NH, DM, DH), BF),
            pltpu.SemaphoreType.DMA((NU + 2,)),
        ],
        compiler_params=pltpu.CompilerParams(vmem_limit_bytes=100 * 1024 * 1024,
                                             disable_bounds_checks=True,
                                             disable_semaphore_checks=True),
    )(
        A_x.reshape(NB, DM), A_k_cache, A_v_cache, A_wq, A_wo.reshape(NH, DH, DM),
        B_x.reshape(NB, DM), B_c_kv.reshape(NB * NU, SK // NU, DM),
        B_w_q.reshape(NU, 512, DH), B_w_uk.reshape(NU, 512, DH), B_w_uv.reshape(NU, 512, DH),
        B_w_o,
    )
    return out.reshape(NB, 1, 2 * DM)
```

```python
import jax
import jax.numpy as jnp
from jax import lax
import jax.experimental.pallas as pl
import jax.experimental.pallas.tpu as pltpu

BF = jnp.bfloat16
F32 = jnp.float32
NT = (((1,), (1,)), ((), ()))

NB = 4
NH = 32
DH = 128
DM = 512
SK = 4096
WIN = 1024
NSLOT = 4
NG = 8
PK2 = [52, 52, 52, 52, 48]
PK8 = [48, 56, 48, 56, 48]
NP = len(PK2)
assert sum(PK2) == 256 and sum(PK8) == 256 and len(PK8) == NP
NOCOMP = 0
PAIR = 1
QKJ = [0]
MJ = 2


def _dot(a, b):
    return jnp.dot(a, b, preferred_element_type=F32)


def _dot_nt(a, b):
    return lax.dot_general(a, b, NT, preferred_element_type=F32)


def _first_tick(pk, kib):
    return next(j for j in range(len(pk)) if sum(pk[:j + 1]) >= kib)


def _kernel(xa_hbm, k_hbm, v_hbm, wq_hbm, wo_hbm, xb_hbm, c_hbm, bwq_hbm, bwuk_hbm, bwuv_hbm, bwo_hbm,
            out_ref,
            xa_v, xb_v, wq_v, wo_v, bwq_v, bwuk_v, bwuv_v, bwo_v, c_v, k_v, v_v,
            qa_s, qb_s, qlat_s, clat_s, s_s, w1_s, w2_s,
            sem):
    scale = DH ** -0.5
    HI, XS = NG * NP, NG * NP + NG

    def piece(src, dst, base, seg, pk, j, s):
        a, n = sum(pk[:j]) * seg // sum(pk), pk[j] * seg // sum(pk)
        al = 8 if len(src.shape) == 2 else 1
        sl = pl.ds(base + a if isinstance(base, int) else pl.multiple_of(base + a, al), n)
        return pltpu.make_async_copy(src.at[sl], dst.at[sl], sem.at[s])

    class Stream:
        def __init__(self, src, dst, pk, nblk=1, blk=0):
            self.src, self.dst, self.pk = src, dst, pk
            self.seg = src.shape[0] // (nblk * 2 * NG)
            self.off = blk * 2 * NG * self.seg

        def lo(self, g, j):
            return piece(self.src, self.dst, self.off + g * self.seg, self.seg, self.pk, j, g * NP + j)

        def hi(self, g, j):
            return piece(self.src, self.dst, self.off + (NG + g) * self.seg, self.seg, self.pk, j, HI + g)

    class First(Stream):
        def lo(self, g, j):
            return piece(self.src, self.dst, g * 2 * self.seg, 2 * self.seg, self.pk, j, g * NP + j)

    def kv_piece(src, dst, h, b, j, s):
        return piece(src.at[b, h, pl.ds(SK - WIN, WIN), :], dst.at[h % NSLOT, b], 0, WIN, PK2, j, s)

    def v_lo(h, b, j):
        return kv_piece(v_hbm, v_v, h, b, j, ((h % 2) * NB + b) * NP + j)

    def k_hi(h, b, j):
        return kv_piece(k_hbm, k_v, h, b, j, HI + (h % 2) * NB + b)

    class KV01:
        lo = staticmethod(lambda g, j: v_lo(g // NB, g % NB, j))
        hi = staticmethod(lambda g, j: k_hi(g // NB, g % NB, j))

    def block(cur, nxt, body, init, pair=False):
        first = isinstance(cur, First)

        def group(g, c):
            if first:
                work = {_first_tick(cur.pk, 64 * (u + 1)): 4 * g + u for u in range(4)}
            elif pair:
                work = {0: 2 * NG + 2 * g, NP - 1: 2 * g}
            else:
                work = {0: 2 * NG + 2 * g, 1: 2 * NG + 2 * g + 1, _first_tick(cur.pk, 128): 2 * g, NP - 1: 2 * g + 1}
            for j in range(NP):
                cur.lo(g, j).wait()
                if j == 0 and not first:
                    for jj in range(NP):
                        cur.hi(g, jj).wait()
                nxt.lo(g, j).start(priority=1)
                nxt.hi(g, j).start(priority=0)
                if j in work and body is not None and not NOCOMP & 2:
                    c = body(work[j], c)
            return c
        return lax.fori_loop(0, NG, group, init)

    s_bwq = First(bwq_hbm, bwq_v, PK2)
    s_bwuk, s_bwuv = Stream(bwuk_hbm, bwuk_v, PK2), Stream(bwuv_hbm, bwuv_v, PK2)
    s_wq = Stream(wq_hbm, wq_v, PK2)
    s_wo, s_bwo = Stream(wo_hbm, wo_v, PK8), Stream(bwo_hbm, bwo_v, PK8)
    s_c = [Stream(c_hbm, c_v, PK8, NB, b) for b in range(NB)]
    xa_cp = pltpu.make_async_copy(xa_hbm, xa_v, sem.at[XS])
    xb_cp = pltpu.make_async_copy(xb_hbm, xb_v, sem.at[XS + 1])

    for g in range(NG):
        for j in range(NP):
            s_bwq.lo(g, j).start(priority=1)
    xa_cp.start()
    xb_cp.start()

    row8 = lax.broadcasted_iota(jnp.int32, (8, 1), 0)

    def pad8(x4):
        return jnp.concatenate([x4.astype(F32), jnp.zeros((4, x4.shape[1]), F32)], axis=0).astype(BF)

    def rows(u, n, k=1):
        return pl.ds(u * n if isinstance(u, int) else pl.multiple_of(u * n, n), n * k)

    def deinterleave(src_ref, dst_ref, u):
        dst_ref[:, rows(u, 16), :] = jnp.swapaxes(src_ref[rows(u, 16 * NH), :].reshape(16, NH, DH), 0, 1)

    def body(u, c):
        deinterleave(bwq_v, w1_s, u)
        return c
    block(s_bwq, s_bwuk, body, 0)

    xa_cp.wait()
    xb_cp.wait()
    xa = pad8(xa_v[...])
    xb = pad8(xb_v[...])

    def body(u, c):
        deinterleave(bwuk_v, w2_s, u)
        qb_s[u] = _dot(xb, w1_s[u])
        return c
    block(s_bwuk, s_wq, body, 0)

    def body(h, c):
        ql = _dot_nt(qb_s[h].astype(BF), w2_s[h]) * scale
        for cb in range(DM // 128):
            qlat_s[cb, rows(h, 8), :] = ql[:, cb * 128:(cb + 1) * 128]
        return c
    block(s_wq, s_c[0], body, 0)

    clat_s[...] = jnp.zeros(clat_s.shape, F32)
    m_prev = None
    nu = 2 if PAIR else 1
    for b in range(NB + 1):
        if b < NB:
            ql = jnp.concatenate([qlat_s[cb, pl.ds(b, NH, stride=8), :] for cb in range(DM // 128)],
                                 axis=1).astype(BF)

        def body(u, c, b=b, m_prev=m_prev, ql=ql):
            m_run, l_run, acc = c
            if b < NB:
                s = _dot_nt(ql, c_v[rows(b * 32 + u, 128, nu), :])
                for k in range(nu):
                    s_s[b % 2, u + k] = s[:, k * 128:(k + 1) * 128]
                    m_run = jnp.maximum(m_run, s[:, k * 128:(k + 1) * 128])
            if b == 0:
                for k in range(nu):
                    w = jnp.concatenate([wq_v[sl * NH + u + k] for sl in range(DM // 8)], axis=0)
                    qa_s[u + k] = _dot(xa, w) * scale
            else:
                ps = [jnp.exp(s_s[(b - 1) % 2, u + k] - m_prev) for k in range(nu)]
                for p in ps:
                    l_run = l_run + p
                p = jnp.concatenate(ps, axis=1).astype(BF)
                acc = acc + _dot(p, c_v[rows((b - 1) * 32 + u, 128, nu), :])
            return m_run, l_run, acc
        init = (jnp.full((NH, 128), -jnp.inf, F32), jnp.zeros((NH, 128), F32), jnp.zeros((NH, DM), F32))
        cur = s_c[b] if b < NB else s_wo
        nxt = s_c[b + 1] if b + 1 < NB else (s_wo if b + 1 == NB else s_bwuv)
        m_run, l_run, acc = block(cur, nxt, body, init, pair=bool(PAIR))
        if b > 0:
            cl = acc / jnp.sum(l_run, axis=1, keepdims=True)
            for cb in range(DM // 128):
                clat_s[cb, pl.ds(b - 1, NH, stride=8), :] = cl[:, cb * 128:(cb + 1) * 128]
        if b < NB:
            m_prev = jnp.broadcast_to(jnp.max(m_run, axis=1, keepdims=True), (NH, 128))

    def body(u, c):
        deinterleave(bwuv_v, w1_s, u)
        return c
    block(s_bwuv, s_bwo, body, 0)

    block(s_bwo, KV01, None, 0)

    def softmax(s):
        p = jnp.exp(s - jnp.max(s, axis=1, keepdims=True))
        return (p * (1.0 / jnp.sum(p, axis=1, keepdims=True))).astype(BF)

    def scores(h, b, s, part=0, nparts=1):
        n = WIN // nparts
        return jnp.where(row8 == b, _dot_nt(qa_s[h].astype(BF), k_v[h % NSLOT, b, pl.ds(part * n, n), :]), s)

    s = jnp.zeros((8, WIN), F32)
    for b in range(NB):
        for j in range(NP):
            k_hi(0, b, j).wait()
    for b in range(NB):
        s = scores(0, b, s)
    p0 = softmax(s)

    def misc(h, b, st):
        if b == 0:
            hp = max(h - 1, 0) if isinstance(h, int) else jnp.maximum(h - 1, 0)
            st["acc_a"] = st["acc_a"] + _dot(st["o_prev"], wo_v[rows(hp, DH), :])
        elif b == 1:
            cl = jnp.concatenate([clat_s[cb, rows(h, 8), :] for cb in range(DM // 128)],
                                 axis=1).astype(BF)
            st["ctx"] = _dot(cl, w1_s[h]).astype(BF)
        elif b == 2:
            st["acc_b"] = st["acc_b"] + _dot(st["ctx"], bwo_v[rows(h, DH), :])

    def a_body(h, carry):
        acc_a, acc_b, o_prev, p = carry
        st = dict(acc_a=acc_a, acc_b=acc_b, o_prev=o_prev)
        ss = [jnp.zeros((8, WIN // len(QKJ)), F32) for _ in QKJ]
        o = jnp.zeros((8, DH), F32)
        p_next = p
        for b in range(NB):
            for j in range(NP):
                v_lo(h, b, j).wait()
                if j == 0:
                    for jj in range(NP):
                        k_hi(h + 1, b, jj).wait()
                v_lo(h + 2, b, j).start(priority=1)
                k_hi(h + 2, b, j).start(priority=0)
                if NOCOMP & 1:
                    continue
                if j in QKJ:
                    ss[QKJ.index(j)] = scores(h + 1, b, ss[QKJ.index(j)], QKJ.index(j), len(QKJ))
                if j == MJ:
                    misc(h, b, st)
                    if b == NB - 1:
                        p_next = softmax(jnp.concatenate(ss, axis=1))
                if j == NP - 1:
                    o = jnp.where(row8 == b, _dot(p, v_v[h % NSLOT, b]), o)
        return st["acc_a"], st["acc_b"], o.astype(BF), p_next

    zero = jnp.zeros((8, DM), F32)
    acc_a, acc_b, o_prev, p = lax.fori_loop(0, NH - 2, a_body, (zero, zero, jnp.zeros((8, DH), BF), p0))

    st = dict(acc_a=acc_a, acc_b=acc_b, o_prev=o_prev)
    for h in (NH - 2, NH - 1):
        s = jnp.zeros((8, WIN), F32)
        o = jnp.zeros((8, DH), F32)
        for b in range(NB):
            if h + 1 < NH:
                for j in range(NP):
                    k_hi(h + 1, b, j).wait()
                s = scores(h + 1, b, s)
            misc(h, b, st)
            for j in range(NP):
                v_lo(h, b, j).wait()
            o = jnp.where(row8 == b, _dot(p, v_v[h % NSLOT, b]), o)
        st["o_prev"] = o.astype(BF)
        if h + 1 < NH:
            p = softmax(s)
    acc_a = st["acc_a"] + _dot(st["o_prev"], wo_v[pl.ds((NH - 1) * DH, DH), :])
    acc_b = st["acc_b"]
    out_ref[:, :DM] = acc_a[:NB].astype(BF)
    out_ref[:, DM:] = acc_b[:NB].astype(BF)


@jax.jit
def pallas_concat_heads__sliding_block_cached__compressed_kv_cla__decode_kernel(
    A_x: jax.Array,
    A_k_cache: jax.Array,
    A_v_cache: jax.Array,
    A_wq: jax.Array,
    A_wo: jax.Array,
    B_x: jax.Array,
    B_c_kv: jax.Array,
    B_w_q: jax.Array,
    B_w_uk: jax.Array,
    B_w_uv: jax.Array,
    B_w_o: jax.Array,
):
    wq_tiles = A_wq.reshape(DM // 8, 8, NH, DH).transpose(0, 2, 1, 3).reshape(DM // 8 * NH, 8, DH)
    out = pl.pallas_call(
        _kernel,
        out_shape=jax.ShapeDtypeStruct((NB, 2 * DM), BF),
        in_specs=[pl.BlockSpec(memory_space=pl.ANY)] * 11,
        out_specs=pl.BlockSpec(memory_space=pltpu.VMEM),
        scratch_shapes=[
            pltpu.VMEM((NB, DM), BF), pltpu.VMEM((NB, DM), BF),
            pltpu.VMEM((DM // 8 * NH, 8, DH), BF), pltpu.VMEM((NH * DH, DM), BF),
            pltpu.VMEM((DM * NH, DH), BF), pltpu.VMEM((DM * NH, DH), BF), pltpu.VMEM((DM * NH, DH), BF),
            pltpu.VMEM((NH * DH, DM), BF),
            pltpu.VMEM((NB * SK, DM), BF),
            pltpu.VMEM((NSLOT, NB, WIN, DH), BF), pltpu.VMEM((NSLOT, NB, WIN, DH), BF),
            pltpu.VMEM((NH, 8, DH), F32), pltpu.VMEM((NH, 8, DH), F32),
            pltpu.VMEM((DM // 128, NH * 8, 128), F32),
            pltpu.VMEM((DM // 128, NH * 8, 128), F32),
            pltpu.VMEM((2, SK // 128, NH, 128), F32),
            pltpu.VMEM((NH, DM, DH), BF), pltpu.VMEM((NH, DM, DH), BF),
            pltpu.SemaphoreType.DMA((NG * NP + NG + 2,)),
        ],
        compiler_params=pltpu.CompilerParams(vmem_limit_bytes=100 * 1024 * 1024,
                                             disable_bounds_checks=True,
                                             disable_semaphore_checks=True),
    )(
        A_x.reshape(NB, DM), A_k_cache, A_v_cache, wq_tiles, A_wo,
        B_x.reshape(NB, DM), B_c_kv.reshape(NB * SK, DM),
        B_w_q.reshape(DM * NH, DH), B_w_uk.reshape(DM * NH, DH), B_w_uv.reshape(DM * NH, DH),
        B_w_o.reshape(NH * DH, DM),
    )
    return out.reshape(NB, 1, 2 * DM)
```

```python
import jax
import jax.numpy as jnp
from jax import lax
import jax.experimental.pallas as pl
import jax.experimental.pallas.tpu as pltpu

BF = jnp.bfloat16
F32 = jnp.float32
NT = (((1,), (1,)), ((), ()))

NB = 4
NH = 32
DH = 128
DM = 512
SK = 4096
WIN = 1024
NSLOT = 4
NG = 8
PKV = ([22, 64, 64, 64, 42], [30, 64, 64, 64, 34])
PKA = ([30, 64, 64, 64, 34], [30, 64, 64, 64, 34])
PKB = ([32, 64, 64, 64, 32], [32, 64, 64, 64, 32])
PK8 = ([32, 64, 64, 64, 32], [32, 64, 64, 64, 32])
PK0 = [96, 128, 64, 128, 96]
NP = 5
assert all(sum(p) == 256 and len(p) == NP for pp in (PKV, PKA, PKB, PK8) for p in pp) and sum(PK0) == 512
NOCOMP = 0
PAIR = 1
QKJ = [0]
MJ = 2


def _dot(a, b):
    return jnp.dot(a, b, preferred_element_type=F32)


def _dot_nt(a, b):
    return lax.dot_general(a, b, NT, preferred_element_type=F32)


def _first_tick(pk, kib):
    return next(j for j in range(len(pk)) if sum(pk[:j + 1]) >= kib)


def _kernel(xa_hbm, k_hbm, v_hbm, wq_hbm, wo_hbm, xb_hbm, c_hbm, bwq_hbm, bwuk_hbm, bwuv_hbm, bwo_hbm,
            out_ref,
            xa_v, xb_v, wq_v, wo_v, bwq_v, bwuk_v, bwuv_v, bwo_v, c_v, k_v, v_v,
            qa_s, qb_s, qlat_s, clat_s, s_s, w1_s, w2_s,
            sem):
    scale = DH ** -0.5
    HI, XS = NG * NP, NG * NP + NG

    def piece(src, dst, base, seg, pk, j, s):
        a, n = sum(pk[:j]) * seg // sum(pk), pk[j] * seg // sum(pk)
        al = 8 if len(src.shape) == 2 else 1
        sl = pl.ds(base + a if isinstance(base, int) else pl.multiple_of(base + a, al), n)
        return pltpu.make_async_copy(src.at[sl], dst.at[sl], sem.at[s])

    class Stream:
        def __init__(self, src, dst, pk, nblk=1, blk=0):
            self.src, self.dst, self.pk = src, dst, pk
            self.seg = src.shape[0] // (nblk * 2 * NG)
            self.off = blk * 2 * NG * self.seg

        def lo(self, g, j):
            return piece(self.src, self.dst, self.off + g * self.seg, self.seg, self.pk[0], j, g * NP + j)

        def hi(self, g, j):
            return piece(self.src, self.dst, self.off + (NG + g) * self.seg, self.seg, self.pk[1], j, HI + g)

    class First(Stream):
        def lo(self, g, j):
            return piece(self.src, self.dst, g * 2 * self.seg, 2 * self.seg, self.pk, j, g * NP + j)

    def kv_piece(src, dst, h, b, pk, j, s):
        return piece(src.at[b, h, pl.ds(SK - WIN, WIN), :], dst.at[h % NSLOT, b], 0, WIN, pk, j, s)

    def v_lo(h, b, j):
        return kv_piece(v_hbm, v_v, h, b, PKV[0], j, ((h % 2) * NB + b) * NP + j)

    def k_hi(h, b, j):
        return kv_piece(k_hbm, k_v, h, b, PKV[1], j, HI + (h % 2) * NB + b)

    class KV01:
        lo = staticmethod(lambda g, j: v_lo(g // NB, g % NB, j))
        hi = staticmethod(lambda g, j: k_hi(g // NB, g % NB, j))

    def block(cur, nxt, body, init, pair=False):
        first = isinstance(cur, First)

        def group(g, c):
            if first:
                work = [(_first_tick(cur.pk, 128 * (u + 1)), 4 * g + u) for u in range(4)]
            elif pair:
                work = [(0, 2 * NG + 2 * g), (NP - 1, 2 * g)]
            else:
                work = [(0, 2 * NG + 2 * g), (1, 2 * NG + 2 * g + 1), (_first_tick(cur.pk[0], 128), 2 * g),
                        (NP - 1, 2 * g + 1)]
            for j in range(NP):
                cur.lo(g, j).wait()
                if j == 0 and not first:
                    for jj in range(NP):
                        cur.hi(g, jj).wait()
                nxt.lo(g, j).start(priority=1)
                nxt.hi(g, j).start(priority=0)
                for jw, u in work:
                    if jw == j and body is not None:
                        c = body(u, c)
            return c
        return lax.fori_loop(0, NG, group, init)

    s_bwq = First(bwq_hbm, bwq_v, PK0)
    s_bwuk, s_bwuv = Stream(bwuk_hbm, bwuk_v, PKB), Stream(bwuv_hbm, bwuv_v, PKB)
    s_wq = Stream(wq_hbm, wq_v, PKA)
    s_wo, s_bwo = Stream(wo_hbm, wo_v, PK8), Stream(bwo_hbm, bwo_v, PK8)
    s_c = [Stream(c_hbm, c_v, PK8, NB, b) for b in range(NB)]
    xa_cp = pltpu.make_async_copy(xa_hbm, xa_v, sem.at[XS])
    xb_cp = pltpu.make_async_copy(xb_hbm, xb_v, sem.at[XS + 1])

    for g in range(NG):
        for j in range(NP):
            s_bwq.lo(g, j).start(priority=1)
    xa_cp.start()
    xb_cp.start()

    row8 = lax.broadcasted_iota(jnp.int32, (8, 1), 0)

    def pad8(x4):
        return jnp.concatenate([x4.astype(F32), jnp.zeros((4, x4.shape[1]), F32)], axis=0).astype(BF)

    def rows(u, n, k=1):
        return pl.ds(u * n if isinstance(u, int) else pl.multiple_of(u * n, n), n * k)

    def deinterleave(src_ref, dst_ref, u):
        dst_ref[:, rows(u, 16), :] = jnp.swapaxes(src_ref[rows(u, 16 * NH), :].reshape(16, NH, DH), 0, 1)

    def body(u, c):
        deinterleave(bwq_v, w1_s, u)
        return c
    block(s_bwq, s_bwuk, body, 0)

    xa_cp.wait()
    xb_cp.wait()
    xa = pad8(xa_v[...])
    xb = pad8(xb_v[...])

    def body(u, c):
        deinterleave(bwuk_v, w2_s, u)
        qb_s[u] = _dot(xb, w1_s[u])
        return c
    block(s_bwuk, s_wq, body, 0)

    def body(h, c):
        ql = _dot_nt(qb_s[h].astype(BF), w2_s[h]) * scale
        for cb in range(DM // 128):
            qlat_s[cb, rows(h, 8), :] = ql[:, cb * 128:(cb + 1) * 128]
        return c
    block(s_wq, s_c[0], body, 0)

    clat_s[...] = jnp.zeros(clat_s.shape, F32)
    m_prev = None
    nu = 2 if PAIR else 1
    for b in range(NB + 1):
        if b < NB:
            ql = jnp.concatenate([qlat_s[cb, pl.ds(b, NH, stride=8), :] for cb in range(DM // 128)],
                                 axis=1).astype(BF)

        def body(u, c, b=b, m_prev=m_prev, ql=ql):
            m_run, l_run, acc = c
            if b < NB:
                s = _dot_nt(ql, c_v[rows(b * 32 + u, 128, nu), :])
                for k in range(nu):
                    s_s[b % 2, u + k] = s[:, k * 128:(k + 1) * 128]
                    m_run = jnp.maximum(m_run, s[:, k * 128:(k + 1) * 128])
            if b == 0:
                for k in range(nu):
                    w = jnp.concatenate([wq_v[sl * NH + u + k] for sl in range(DM // 8)], axis=0)
                    qa_s[u + k] = _dot(xa, w) * scale
            else:
                ps = [jnp.exp(s_s[(b - 1) % 2, u + k] - m_prev) for k in range(nu)]
                for p in ps:
                    l_run = l_run + p
                p = jnp.concatenate(ps, axis=1).astype(BF)
                acc = acc + _dot(p, c_v[rows((b - 1) * 32 + u, 128, nu), :])
            return m_run, l_run, acc
        init = (jnp.full((NH, 128), -jnp.inf, F32), jnp.zeros((NH, 128), F32), jnp.zeros((NH, DM), F32))
        cur = s_c[b] if b < NB else s_wo
        nxt = s_c[b + 1] if b + 1 < NB else (s_wo if b + 1 == NB else s_bwuv)
        m_run, l_run, acc = block(cur, nxt, body, init, pair=bool(PAIR))
        if b > 0:
            cl = acc / jnp.sum(l_run, axis=1, keepdims=True)
            for cb in range(DM // 128):
                clat_s[cb, pl.ds(b - 1, NH, stride=8), :] = cl[:, cb * 128:(cb + 1) * 128]
        if b < NB:
            m_prev = jnp.broadcast_to(jnp.max(m_run, axis=1, keepdims=True), (NH, 128))

    def body(u, c):
        deinterleave(bwuv_v, w1_s, u)
        return c
    block(s_bwuv, s_bwo, body, 0)

    block(s_bwo, KV01, None, 0)

    def softmax(s):
        p = jnp.exp(s - jnp.max(s, axis=1, keepdims=True))
        return (p * (1.0 / jnp.sum(p, axis=1, keepdims=True))).astype(BF)

    def scores(h, b, s, part=0, nparts=1):
        n = WIN // nparts
        return jnp.where(row8 == b, _dot_nt(qa_s[h].astype(BF), k_v[h % NSLOT, b, pl.ds(part * n, n), :]), s)

    s = jnp.zeros((8, WIN), F32)
    for b in range(NB):
        for j in range(NP):
            k_hi(0, b, j).wait()
    for b in range(NB):
        s = scores(0, b, s)
    p0 = softmax(s)

    def misc(h, b, st):
        if b == 0:
            hp = max(h - 1, 0) if isinstance(h, int) else jnp.maximum(h - 1, 0)
            st["acc_a"] = st["acc_a"] + _dot(st["o_prev"], wo_v[rows(hp, DH), :])
        elif b == 1:
            cl = jnp.concatenate([clat_s[cb, rows(h, 8), :] for cb in range(DM // 128)],
                                 axis=1).astype(BF)
            st["ctx"] = _dot(cl, w1_s[h]).astype(BF)
        elif b == 2:
            st["acc_b"] = st["acc_b"] + _dot(st["ctx"], bwo_v[rows(h, DH), :])

    def a_body(h, carry):
        acc_a, acc_b, o_prev, p = carry
        st = dict(acc_a=acc_a, acc_b=acc_b, o_prev=o_prev)
        ss = [jnp.zeros((8, WIN // len(QKJ)), F32) for _ in QKJ]
        o = jnp.zeros((8, DH), F32)
        p_next = p
        for b in range(NB):
            for j in range(NP):
                v_lo(h, b, j).wait()
                if j == 0:
                    for jj in range(NP):
                        k_hi(h + 1, b, jj).wait()
                v_lo(h + 2, b, j).start(priority=1)
                k_hi(h + 2, b, j).start(priority=0)
                if NOCOMP & 1:
                    continue
                if j in QKJ:
                    ss[QKJ.index(j)] = scores(h + 1, b, ss[QKJ.index(j)], QKJ.index(j), len(QKJ))
                if j == MJ:
                    misc(h, b, st)
                    if b == NB - 1:
                        p_next = softmax(jnp.concatenate(ss, axis=1))
                if j == NP - 1:
                    o = jnp.where(row8 == b, _dot(p, v_v[h % NSLOT, b]), o)
        return st["acc_a"], st["acc_b"], o.astype(BF), p_next

    zero = jnp.zeros((8, DM), F32)
    acc_a, acc_b, o_prev, p = lax.fori_loop(0, NH - 2, a_body, (zero, zero, jnp.zeros((8, DH), BF), p0))

    st = dict(acc_a=acc_a, acc_b=acc_b, o_prev=o_prev)
    for h in (NH - 2, NH - 1):
        s = jnp.zeros((8, WIN), F32)
        o = jnp.zeros((8, DH), F32)
        for b in range(NB):
            if h + 1 < NH:
                for j in range(NP):
                    k_hi(h + 1, b, j).wait()
                s = scores(h + 1, b, s)
            misc(h, b, st)
            for j in range(NP):
                v_lo(h, b, j).wait()
            o = jnp.where(row8 == b, _dot(p, v_v[h % NSLOT, b]), o)
        st["o_prev"] = o.astype(BF)
        if h + 1 < NH:
            p = softmax(s)
    acc_a = st["acc_a"] + _dot(st["o_prev"], wo_v[pl.ds((NH - 1) * DH, DH), :])
    acc_b = st["acc_b"]
    out_ref[:, :DM] = acc_a[:NB].astype(BF)
    out_ref[:, DM:] = acc_b[:NB].astype(BF)


@jax.jit
def pallas_concat_heads__sliding_block_cached__compressed_kv_cla__decode_kernel(
    A_x: jax.Array,
    A_k_cache: jax.Array,
    A_v_cache: jax.Array,
    A_wq: jax.Array,
    A_wo: jax.Array,
    B_x: jax.Array,
    B_c_kv: jax.Array,
    B_w_q: jax.Array,
    B_w_uk: jax.Array,
    B_w_uv: jax.Array,
    B_w_o: jax.Array,
):
    wq_tiles = A_wq.reshape(DM // 8, 8, NH, DH).transpose(0, 2, 1, 3).reshape(DM // 8 * NH, 8, DH)
    out = pl.pallas_call(
        _kernel,
        out_shape=jax.ShapeDtypeStruct((NB, 2 * DM), BF),
        in_specs=[pl.BlockSpec(memory_space=pl.ANY)] * 11,
        out_specs=pl.BlockSpec(memory_space=pltpu.VMEM),
        scratch_shapes=[
            pltpu.VMEM((NB, DM), BF), pltpu.VMEM((NB, DM), BF),
            pltpu.VMEM((DM // 8 * NH, 8, DH), BF), pltpu.VMEM((NH * DH, DM), BF),
            pltpu.VMEM((DM * NH, DH), BF), pltpu.VMEM((DM * NH, DH), BF), pltpu.VMEM((DM * NH, DH), BF),
            pltpu.VMEM((NH * DH, DM), BF),
            pltpu.VMEM((NB * SK, DM), BF),
            pltpu.VMEM((NSLOT, NB, WIN, DH), BF), pltpu.VMEM((NSLOT, NB, WIN, DH), BF),
            pltpu.VMEM((NH, 8, DH), F32), pltpu.VMEM((NH, 8, DH), F32),
            pltpu.VMEM((DM // 128, NH * 8, 128), F32),
            pltpu.VMEM((DM // 128, NH * 8, 128), F32),
            pltpu.VMEM((2, SK // 128, NH, 128), F32),
            pltpu.VMEM((NH, DM, DH), BF), pltpu.VMEM((NH, DM, DH), BF),
            pltpu.SemaphoreType.DMA((NG * NP + NG + 2,)),
        ],
        compiler_params=pltpu.CompilerParams(vmem_limit_bytes=100 * 1024 * 1024,
                                             disable_bounds_checks=True,
                                             disable_semaphore_checks=True),
    )(
        A_x.reshape(NB, DM), A_k_cache, A_v_cache, wq_tiles, A_wo,
        B_x.reshape(NB, DM), B_c_kv.reshape(NB * SK, DM),
        B_w_q.reshape(DM * NH, DH), B_w_uk.reshape(DM * NH, DH), B_w_uv.reshape(DM * NH, DH),
        B_w_o.reshape(NH * DH, DM),
    )
    return out.reshape(NB, 1, 2 * DM)
```

```python
import jax
import jax.numpy as jnp
from jax import lax
import jax.experimental.pallas as pl
import jax.experimental.pallas.tpu as pltpu

BF = jnp.bfloat16
F32 = jnp.float32
NT = (((1,), (1,)), ((), ()))

NB = 4
NH = 32
DH = 128
DM = 512
SK = 4096
WIN = 1024
NSLOT = 4
NG = 8
PKV = ([22, 64, 64, 64, 42], [30, 64, 64, 62, 36])
PKA = ([22, 64, 64, 64, 42], [28, 66, 62, 66, 34])
PKB = ([26, 64, 64, 64, 38], [32, 66, 62, 66, 30])
PK0 = [96, 128, 64, 128, 96]
MERGE = 0
HJ = 1
WJ = (0, 1, 2)
LASTWO = 1
NP = 5
assert all(sum(p) == 256 and len(p) == NP for pp in (PKV, PKA, PKB) for p in pp) and sum(PK0) == 512
NOCOMP = 0
PAIR = 1
QKJ = [0]
MJ = 2


def _dot(a, b):
    return jnp.dot(a, b, preferred_element_type=F32)


def _dot_nt(a, b):
    return lax.dot_general(a, b, NT, preferred_element_type=F32)


def _first_tick(pk, kib):
    return next(j for j in range(len(pk)) if sum(pk[:j + 1]) >= kib)


def _kernel(xa_hbm, k_hbm, v_hbm, wq_hbm, wo_hbm, xb_hbm, c_hbm, bwq_hbm, bwuk_hbm, bwuv_hbm, bwo_hbm,
            out_ref,
            xa_v, xb_v, wq_v, wo_v, bwq_v, bwuk_v, bwuv_v, bwo_v, c_v, k_v, v_v,
            qa_s, qb_s, qlat_s, clat_s, s_s, w1_s, w2_s,
            sem):
    scale = DH ** -0.5
    HI, XS = NG * NP, NG * NP + NG

    def piece(src, dst, base, seg, pk, j, s):
        a, n = sum(pk[:j]) * seg // sum(pk), pk[j] * seg // sum(pk)
        al = 8 if len(src.shape) == 2 else 1
        sl = pl.ds(base + a if isinstance(base, int) else pl.multiple_of(base + a, al), n)
        return pltpu.make_async_copy(src.at[sl], dst.at[sl], sem.at[s])

    class Stream:
        merge = bool(MERGE)

        def __init__(self, src, dst, pk, nblk=1, blk=0):
            self.src, self.dst, self.pk = src, dst, pk
            self.seg = src.shape[0] // (nblk * 2 * NG)
            self.off = blk * 2 * NG * self.seg

        def lo(self, g, j):
            return piece(self.src, self.dst, self.off + g * self.seg, self.seg, self.pk[0], j, g * NP + j)

        def hi(self, g, j):
            return piece(self.src, self.dst, self.off + (NG + g) * self.seg, self.seg, self.pk[1], j, HI + g)

    class First(Stream):
        merge = False

        def lo(self, g, j):
            return piece(self.src, self.dst, g * 2 * self.seg, 2 * self.seg, self.pk, j, g * NP + j)

    def kv_piece(src, dst, h, b, pk, j, s):
        return piece(src.at[b, h, pl.ds(SK - WIN, WIN), :], dst.at[h % NSLOT, b], 0, WIN, pk, j, s)

    def v_lo(h, b, j):
        return kv_piece(v_hbm, v_v, h, b, PKV[0], j, ((h % 2) * NB + b) * NP + j)

    def k_hi(h, b, j):
        return kv_piece(k_hbm, k_v, h, b, PKV[1], j, HI + (h % 2) * NB + b)

    class KV01:
        merge = False
        lo = staticmethod(lambda g, j: v_lo(g // NB, g % NB, j))
        hi = staticmethod(lambda g, j: k_hi(g // NB, g % NB, j))

    def block(cur, nxt, body, init, pair=False):
        first = isinstance(cur, First)

        def group(g, c):
            if first:
                work = [(_first_tick(cur.pk, 128 * (u + 1)), 4 * g + u) for u in range(4)]
            elif pair:
                work = [(HJ, 2 * NG + 2 * g), (NP - 1, 2 * g)]
            else:
                assert WJ[2] >= _first_tick(cur.pk[0], 128)
                work = [(WJ[0], 2 * NG + 2 * g), (WJ[1], 2 * NG + 2 * g + 1), (WJ[2], 2 * g), (NP - 1, 2 * g + 1)]
            for j in range(NP):
                cur.lo(g, j).wait()
                if j == 0 and not first:
                    for jj in range(NP):
                        cur.hi(g, jj).wait()
                nxt.lo(g, j).start(priority=1)
                if j == 0 and cur.merge:
                    @pl.when(g == 0)
                    def _():
                        cur.hi(NG - 1, NP - 1).start(priority=0)
                if j == 0 and nxt.merge:
                    @pl.when(g > 0)
                    def _():
                        nxt.hi(jnp.maximum(g - 1, 0), NP - 1).start(priority=0)
                if j < NP - 1 or not nxt.merge:
                    nxt.hi(g, j).start(priority=0)
                for jw, u in work:
                    if jw == j and body is not None:
                        c = body(u, c)
            return c
        return lax.fori_loop(0, NG, group, init)

    s_bwq = First(bwq_hbm, bwq_v, PK0)
    s_bwuk, s_bwuv = Stream(bwuk_hbm, bwuk_v, PKB), Stream(bwuv_hbm, bwuv_v, PKB)
    s_wq = Stream(wq_hbm, wq_v, PKA)
    s_wo, s_bwo = Stream(wo_hbm, wo_v, PKA), Stream(bwo_hbm, bwo_v, PKB)
    s_c = [Stream(c_hbm, c_v, PKB, NB, b) for b in range(NB)]
    xa_cp = pltpu.make_async_copy(xa_hbm, xa_v, sem.at[XS])
    xb_cp = pltpu.make_async_copy(xb_hbm, xb_v, sem.at[XS + 1])

    for g in range(NG):
        for j in range(NP):
            s_bwq.lo(g, j).start(priority=1)
    xa_cp.start()
    xb_cp.start()

    row8 = lax.broadcasted_iota(jnp.int32, (8, 1), 0)

    def pad8(x4):
        return jnp.concatenate([x4.astype(F32), jnp.zeros((4, x4.shape[1]), F32)], axis=0).astype(BF)

    def rows(u, n, k=1):
        return pl.ds(u * n if isinstance(u, int) else pl.multiple_of(u * n, n), n * k)

    def wide(ref, u, k=1):
        t = ref[rows(u, 64, k)].reshape(16 * k, DM // 128, 8, 128)
        return jnp.concatenate([t[:, j].reshape(128 * k, 128) for j in range(DM // 128)], axis=1)

    def deinterleave(src_ref, dst_ref, u):
        dst_ref[:, rows(u, 16), :] = jnp.swapaxes(src_ref[rows(u, 16 * NH), :].reshape(16, NH, DH), 0, 1)

    def body(u, c):
        deinterleave(bwq_v, w1_s, u)
        return c
    block(s_bwq, s_bwuk, body, 0)

    xa_cp.wait()
    xb_cp.wait()
    xa = pad8(xa_v[...])
    xb = pad8(xb_v[...])

    def body(u, c):
        deinterleave(bwuk_v, w2_s, u)
        qb_s[u] = _dot(xb, w1_s[u])
        return c
    block(s_bwuk, s_wq, body, 0)

    def body(h, c):
        ql = _dot_nt(qb_s[h].astype(BF), w2_s[h]) * scale
        for cb in range(DM // 128):
            qlat_s[cb, rows(h, 8), :] = ql[:, cb * 128:(cb + 1) * 128]
        return c
    block(s_wq, s_c[0], body, 0)

    clat_s[...] = jnp.zeros(clat_s.shape, F32)
    m_prev = None
    nu = 2 if PAIR else 1
    for b in range(NB + 1):
        if b < NB:
            ql = jnp.concatenate([qlat_s[cb, pl.ds(b, NH, stride=8), :] for cb in range(DM // 128)],
                                 axis=1).astype(BF)

        def body(u, c, b=b, m_prev=m_prev, ql=ql):
            m_run, l_run, acc = c
            if b < NB:
                s = _dot_nt(ql, wide(c_v, b * 32 + u, nu))
                for k in range(nu):
                    s_s[b % 2, u + k] = s[:, k * 128:(k + 1) * 128]
                    m_run = jnp.maximum(m_run, s[:, k * 128:(k + 1) * 128])
            if b == 0:
                for k in range(nu):
                    w = jnp.concatenate([wq_v[sl * NH + u + k] for sl in range(DM // 8)], axis=0)
                    qa_s[u + k] = _dot(xa, w) * scale
            else:
                ps = [jnp.exp(s_s[(b - 1) % 2, u + k] - m_prev) for k in range(nu)]
                for p in ps:
                    l_run = l_run + p
                p = jnp.concatenate(ps, axis=1).astype(BF)
                acc = acc + _dot(p, wide(c_v, (b - 1) * 32 + u, nu))
            return m_run, l_run, acc
        init = (jnp.full((NH, 128), -jnp.inf, F32), jnp.zeros((NH, 128), F32), jnp.zeros((NH, DM), F32))
        cur = s_c[b] if b < NB else s_wo
        nxt = s_c[b + 1] if b + 1 < NB else (s_wo if b + 1 == NB else s_bwuv)
        m_run, l_run, acc = block(cur, nxt, body, init, pair=bool(PAIR))
        if b > 0:
            cl = acc / jnp.sum(l_run, axis=1, keepdims=True)
            for cb in range(DM // 128):
                clat_s[cb, pl.ds(b - 1, NH, stride=8), :] = cl[:, cb * 128:(cb + 1) * 128]
        if b < NB:
            m_prev = jnp.broadcast_to(jnp.max(m_run, axis=1, keepdims=True), (NH, 128))

    def body(u, c):
        deinterleave(bwuv_v, w1_s, u)
        return c
    block(s_bwuv, s_bwo, body, 0)

    block(s_bwo, KV01, None, 0)

    def softmax(s):
        p = jnp.exp(s - jnp.max(s, axis=1, keepdims=True))
        return (p * (1.0 / jnp.sum(p, axis=1, keepdims=True))).astype(BF)

    def scores(h, b, s, part=0, nparts=1):
        n = WIN // nparts
        return jnp.where(row8 == b, _dot_nt(qa_s[h].astype(BF), k_v[h % NSLOT, b, pl.ds(part * n, n), :]), s)

    s = jnp.zeros((8, WIN), F32)
    for b in range(NB):
        for j in range(NP):
            k_hi(0, b, j).wait()
    for b in range(NB):
        s = scores(0, b, s)
    p0 = softmax(s)

    def misc(h, b, st):
        if b == 0:
            hp = max(h - 1, 0) if isinstance(h, int) else jnp.maximum(h - 1, 0)
            st["acc_a"] = st["acc_a"] + _dot(st["o_prev"], wide(wo_v, hp))
        elif b == 1:
            cl = jnp.concatenate([clat_s[cb, rows(h, 8), :] for cb in range(DM // 128)],
                                 axis=1).astype(BF)
            st["ctx"] = _dot(cl, w1_s[h]).astype(BF)
        elif b == 2:
            st["acc_b"] = st["acc_b"] + _dot(st["ctx"], wide(bwo_v, h))

    def a_body(h, carry):
        acc_a, acc_b, o_prev, p = carry
        st = dict(acc_a=acc_a, acc_b=acc_b, o_prev=o_prev)
        ss = [jnp.zeros((8, WIN // len(QKJ)), F32) for _ in QKJ]
        o = jnp.zeros((8, DH), F32)
        p_next = p
        for b in range(NB):
            for j in range(NP):
                v_lo(h, b, j).wait()
                if j == 0:
                    for jj in range(NP):
                        k_hi(h + 1, b, jj).wait()
                v_lo(h + 2, b, j).start(priority=1)
                k_hi(h + 2, b, j).start(priority=0)
                if NOCOMP & 1:
                    continue
                if j in QKJ:
                    ss[QKJ.index(j)] = scores(h + 1, b, ss[QKJ.index(j)], QKJ.index(j), len(QKJ))
                if j == MJ:
                    misc(h, b, st)
                    if b == NB - 1:
                        p_next = softmax(jnp.concatenate(ss, axis=1))
                if j == NP - 1:
                    o = jnp.where(row8 == b, _dot(p, v_v[h % NSLOT, b]), o)
        return st["acc_a"], st["acc_b"], o.astype(BF), p_next

    zero = jnp.zeros((8, DM), F32)
    acc_a, acc_b, o_prev, p = lax.fori_loop(0, NH - 2, a_body, (zero, zero, jnp.zeros((8, DH), BF), p0))

    st = dict(acc_a=acc_a, acc_b=acc_b, o_prev=o_prev)
    for h in (NH - 2, NH - 1):
        s = jnp.zeros((8, WIN), F32)
        o = jnp.zeros((8, DH), F32)
        for b in range(NB):
            if h + 1 < NH:
                for j in range(NP):
                    k_hi(h + 1, b, j).wait()
                s = scores(h + 1, b, s)
            misc(h, b, st)
            for j in range(NP):
                v_lo(h, b, j).wait()
            o = jnp.where(row8 == b, _dot(p, v_v[h % NSLOT, b]), o)
        st["o_prev"] = o.astype(BF)
        if h + 1 < NH:
            p = softmax(s)
    acc_a = st["acc_a"] + _dot(st["o_prev"], wide(wo_v, NH - 1))
    acc_b = st["acc_b"]
    out_ref[:, :DM] = acc_a[:NB].astype(BF)
    out_ref[:, DM:] = acc_b[:NB].astype(BF)


@jax.jit
def pallas_concat_heads__sliding_block_cached__compressed_kv_cla__decode_kernel(
    A_x: jax.Array,
    A_k_cache: jax.Array,
    A_v_cache: jax.Array,
    A_wq: jax.Array,
    A_wo: jax.Array,
    B_x: jax.Array,
    B_c_kv: jax.Array,
    B_w_q: jax.Array,
    B_w_uk: jax.Array,
    B_w_uv: jax.Array,
    B_w_o: jax.Array,
):
    def tiles(w):
        r, c = w.shape
        return w.reshape(r // 8, 8, c // 128, 128).transpose(0, 2, 1, 3).reshape(r * c // 1024, 8, 128)

    out = pl.pallas_call(
        _kernel,
        out_shape=jax.ShapeDtypeStruct((NB, 2 * DM), BF),
        in_specs=[pl.BlockSpec(memory_space=pl.ANY)] * 11,
        out_specs=pl.BlockSpec(memory_space=pltpu.VMEM),
        scratch_shapes=[
            pltpu.VMEM((NB, DM), BF), pltpu.VMEM((NB, DM), BF),
            pltpu.VMEM((2048, 8, 128), BF), pltpu.VMEM((2048, 8, 128), BF),
            pltpu.VMEM((DM * NH, DH), BF), pltpu.VMEM((DM * NH, DH), BF), pltpu.VMEM((DM * NH, DH), BF),
            pltpu.VMEM((2048, 8, 128), BF),
            pltpu.VMEM((NB * 2048, 8, 128), BF),
            pltpu.VMEM((NSLOT, NB, WIN, DH), BF), pltpu.VMEM((NSLOT, NB, WIN, DH), BF),
            pltpu.VMEM((NH, 8, DH), F32), pltpu.VMEM((NH, 8, DH), F32),
            pltpu.VMEM((DM // 128, NH * 8, 128), F32),
            pltpu.VMEM((DM // 128, NH * 8, 128), F32),
            pltpu.VMEM((2, SK // 128, NH, 128), F32),
            pltpu.VMEM((NH, DM, DH), BF), pltpu.VMEM((NH, DM, DH), BF),
            pltpu.SemaphoreType.DMA((NG * NP + NG + 2,)),
        ],
        compiler_params=pltpu.CompilerParams(vmem_limit_bytes=100 * 1024 * 1024,
                                             disable_bounds_checks=True,
                                             disable_semaphore_checks=True),
    )(
        A_x.reshape(NB, DM), A_k_cache, A_v_cache, tiles(A_wq), tiles(A_wo),
        B_x.reshape(NB, DM), tiles(B_c_kv.reshape(NB * SK, DM)),
        B_w_q.reshape(DM * NH, DH), B_w_uk.reshape(DM * NH, DH), B_w_uv.reshape(DM * NH, DH),
        tiles(B_w_o.reshape(NH * DH, DM)),
    )
    return out.reshape(NB, 1, 2 * DM)
```

```python
import jax
import jax.numpy as jnp
from jax import lax
import jax.experimental.pallas as pl
import jax.experimental.pallas.tpu as pltpu

BF = jnp.bfloat16
F32 = jnp.float32
NT = (((1,), (1,)), ((), ()))

NB = 4
NH = 32
DH = 128
DM = 512
SK = 4096
WIN = 1024
NSLOT = 4
NG = 8
CV = [26, 90, 154, 218]
CK = [30, 92, 158, 220]
QKJ = (1, 4)
MJ = (3, 6)
NQ = 8
PKA = ([22, 64, 64, 64, 42], [28, 66, 62, 66, 34])
PKB = ([26, 64, 64, 64, 38], [32, 66, 62, 66, 30])
PK0 = [96, 128, 64, 128, 96]
MERGE = 0
HJ = 1
WJ = (0, 1, 2)
LASTWO = 1
NP = 5
assert all(sum(p) == 256 and len(p) == NP for pp in (PKA, PKB) for p in pp) and sum(PK0) == 512
NOCOMP = 0
PAIR = 1


def _dot(a, b):
    return jnp.dot(a, b, preferred_element_type=F32)


def _dot_nt(a, b):
    return lax.dot_general(a, b, NT, preferred_element_type=F32)


def _first_tick(pk, kib):
    return next(j for j in range(len(pk)) if sum(pk[:j + 1]) >= kib)


def _kernel(xa_hbm, k_hbm, v_hbm, wq_hbm, wo_hbm, xb_hbm, c_hbm, bwq_hbm, bwuk_hbm, bwuv_hbm, bwo_hbm,
            out_ref,
            xa_v, xb_v, wq_v, wo_v, bwq_v, bwuk_v, bwuv_v, bwo_v, c_v, k_v, v_v,
            qa_s, qb_s, qlat_s, clat_s, s_s, w1_s, w2_s,
            sem):
    scale = DH ** -0.5
    HI, XS, VS, KS = NG * NP, NG * NP + NG, NG * NP + NG + 2, NG * NP + NG + 2 + 4 * NQ

    def piece(src, dst, base, seg, pk, j, s):
        a, n = sum(pk[:j]) * seg // sum(pk), pk[j] * seg // sum(pk)
        al = 8 if len(src.shape) == 2 else 1
        sl = pl.ds(base + a if isinstance(base, int) else pl.multiple_of(base + a, al), n)
        return pltpu.make_async_copy(src.at[sl], dst.at[sl], sem.at[s])

    class Stream:
        merge = bool(MERGE)

        def __init__(self, src, dst, pk, nblk=1, blk=0):
            self.src, self.dst, self.pk = src, dst, pk
            self.seg = src.shape[0] // (nblk * 2 * NG)
            self.off = blk * 2 * NG * self.seg

        def lo(self, g, j):
            return piece(self.src, self.dst, self.off + g * self.seg, self.seg, self.pk[0], j, g * NP + j)

        def hi(self, g, j):
            return piece(self.src, self.dst, self.off + (NG + g) * self.seg, self.seg, self.pk[1], j, HI + g)

    class First(Stream):
        merge = False

        def lo(self, g, j):
            return piece(self.src, self.dst, g * 2 * self.seg, 2 * self.seg, self.pk, j, g * NP + j)

    def kv_piece(src, dst, h, g, cuts, j, s):
        if j == 0:
            b0, nb, a, e = 0, 2, 0, cuts[0]
        elif j == NQ - 1:
            b0, nb, a, e = 0, 2, cuts[3], 256
        else:
            b0, nb, a, e = (j - 1) // 3, 1, cuts[(j - 1) % 3], cuts[(j - 1) % 3 + 1]
        bs, n = pl.ds(2 * g + b0, nb), (e - a) * 4
        return pltpu.make_async_copy(src.at[bs, h, pl.ds(SK - WIN + a * 4, n), :],
                                     dst.at[h % NSLOT, bs, pl.ds(a * 4, n), :], sem.at[s])

    def v_lo(h, g, j):
        return kv_piece(v_hbm, v_v, h, g, CV, j, VS + ((h % 2) * 2 + g) * NQ + j)

    def k_hi(h, g, j):
        return kv_piece(k_hbm, k_v, h, g, CK, j, KS + (h % 2) * 2 + g)

    def block(cur, nxt, body, init, pair=False):
        first = isinstance(cur, First)

        def group(g, c):
            if first:
                work = [(_first_tick(cur.pk, 128 * (u + 1)), 4 * g + u) for u in range(4)]
            elif pair:
                work = [(HJ, 2 * NG + 2 * g), (NP - 1, 2 * g)]
            else:
                assert WJ[2] >= _first_tick(cur.pk[0], 128)
                work = [(WJ[0], 2 * NG + 2 * g), (WJ[1], 2 * NG + 2 * g + 1), (WJ[2], 2 * g), (NP - 1, 2 * g + 1)]
            for j in range(NP):
                cur.lo(g, j).wait()
                if j == 0 and not first:
                    for jj in range(NP):
                        cur.hi(g, jj).wait()
                nxt.lo(g, j).start(priority=1)
                if j == 0 and cur.merge:
                    @pl.when(g == 0)
                    def _():
                        cur.hi(NG - 1, NP - 1).start(priority=0)
                if j == 0 and nxt.merge:
                    @pl.when(g > 0)
                    def _():
                        nxt.hi(jnp.maximum(g - 1, 0), NP - 1).start(priority=0)
                if j < NP - 1 or not nxt.merge:
                    nxt.hi(g, j).start(priority=0)
                for jw, u in work:
                    if jw == j and body is not None:
                        c = body(u, c)
            return c
        return lax.fori_loop(0, NG, group, init)

    s_bwq = First(bwq_hbm, bwq_v, PK0)
    s_bwuk, s_bwuv = Stream(bwuk_hbm, bwuk_v, PKB), Stream(bwuv_hbm, bwuv_v, PKB)
    s_wq = Stream(wq_hbm, wq_v, PKA)
    s_wo, s_bwo = Stream(wo_hbm, wo_v, PKA), Stream(bwo_hbm, bwo_v, PKB)
    s_c = [Stream(c_hbm, c_v, PKB, NB, b) for b in range(NB)]
    xa_cp = pltpu.make_async_copy(xa_hbm, xa_v, sem.at[XS])
    xb_cp = pltpu.make_async_copy(xb_hbm, xb_v, sem.at[XS + 1])

    for g in range(NG):
        for j in range(NP):
            s_bwq.lo(g, j).start(priority=1)
    xa_cp.start()
    xb_cp.start()

    row8 = lax.broadcasted_iota(jnp.int32, (8, 1), 0)

    def pad8(x4):
        return jnp.concatenate([x4.astype(F32), jnp.zeros((4, x4.shape[1]), F32)], axis=0).astype(BF)

    def rows(u, n, k=1):
        return pl.ds(u * n if isinstance(u, int) else pl.multiple_of(u * n, n), n * k)

    def wide(ref, u, k=1):
        t = ref[rows(u, 64, k)].reshape(16 * k, DM // 128, 8, 128)
        return jnp.concatenate([t[:, j].reshape(128 * k, 128) for j in range(DM // 128)], axis=1)

    def deinterleave(src_ref, dst_ref, u):
        dst_ref[:, rows(u, 16), :] = jnp.swapaxes(src_ref[rows(u, 16 * NH), :].reshape(16, NH, DH), 0, 1)

    def body(u, c):
        deinterleave(bwq_v, w1_s, u)
        return c
    block(s_bwq, s_bwuk, body, 0)

    xa_cp.wait()
    xb_cp.wait()
    xa = pad8(xa_v[...])
    xb = pad8(xb_v[...])

    def body(u, c):
        deinterleave(bwuk_v, w2_s, u)
        qb_s[u] = _dot(xb, w1_s[u])
        return c
    block(s_bwuk, s_wq, body, 0)

    def body(h, c):
        ql = _dot_nt(qb_s[h].astype(BF), w2_s[h]) * scale
        for cb in range(DM // 128):
            qlat_s[cb, rows(h, 8), :] = ql[:, cb * 128:(cb + 1) * 128]
        return c
    block(s_wq, s_c[0], body, 0)

    clat_s[...] = jnp.zeros(clat_s.shape, F32)
    m_prev = None
    nu = 2 if PAIR else 1
    for b in range(NB + 1):
        if b < NB:
            ql = jnp.concatenate([qlat_s[cb, pl.ds(b, NH, stride=8), :] for cb in range(DM // 128)],
                                 axis=1).astype(BF)

        def body(u, c, b=b, m_prev=m_prev, ql=ql):
            m_run, l_run, acc = c
            if b < NB:
                s = _dot_nt(ql, wide(c_v, b * 32 + u, nu))
                for k in range(nu):
                    s_s[b % 2, u + k] = s[:, k * 128:(k + 1) * 128]
                    m_run = jnp.maximum(m_run, s[:, k * 128:(k + 1) * 128])
            if b == 0:
                for k in range(nu):
                    w = jnp.concatenate([wq_v[sl * NH + u + k] for sl in range(DM // 8)], axis=0)
                    qa_s[u + k] = _dot(xa, w) * scale
            else:
                ps = [jnp.exp(s_s[(b - 1) % 2, u + k] - m_prev) for k in range(nu)]
                for p in ps:
                    l_run = l_run + p
                p = jnp.concatenate(ps, axis=1).astype(BF)
                acc = acc + _dot(p, wide(c_v, (b - 1) * 32 + u, nu))
            return m_run, l_run, acc
        init = (jnp.full((NH, 128), -jnp.inf, F32), jnp.zeros((NH, 128), F32), jnp.zeros((NH, DM), F32))
        cur = s_c[b] if b < NB else s_wo
        nxt = s_c[b + 1] if b + 1 < NB else (s_wo if b + 1 == NB else s_bwuv)
        m_run, l_run, acc = block(cur, nxt, body, init, pair=bool(PAIR))
        if b > 0:
            cl = acc / jnp.sum(l_run, axis=1, keepdims=True)
            for cb in range(DM // 128):
                clat_s[cb, pl.ds(b - 1, NH, stride=8), :] = cl[:, cb * 128:(cb + 1) * 128]
        if b < NB:
            m_prev = jnp.broadcast_to(jnp.max(m_run, axis=1, keepdims=True), (NH, 128))

    def body(u, c):
        deinterleave(bwuv_v, w1_s, u)
        return c
    block(s_bwuv, s_bwo, body, 0)

    kv0 = [(h, g, j) for h in range(2) for g in range(2) for j in range(NQ)]
    for g in range(NG):
        for j in range(NP):
            s_bwo.lo(g, j).wait()
            if j == 0:
                for jj in range(NP):
                    s_bwo.hi(g, jj).wait()
            if j < NP - 1:
                u = kv0.pop(0)
                v_lo(*u).start(priority=1)
                k_hi(*u).start(priority=0)

    def softmax(s):
        p = jnp.exp(s - jnp.max(s, axis=1, keepdims=True))
        return (p * (1.0 / jnp.sum(p, axis=1, keepdims=True))).astype(BF)

    def scores(h, b, s):
        return jnp.where(row8 == b, _dot_nt(qa_s[h].astype(BF), k_v[h % NSLOT, b]), s)

    s = jnp.zeros((8, WIN), F32)
    for g in range(2):
        for j in range(NQ):
            k_hi(0, g, j).wait()
    for b in range(NB):
        s = scores(0, b, s)
    p0 = softmax(s)

    def misc(h, b, st):
        if b == 0:
            hp = max(h - 1, 0) if isinstance(h, int) else jnp.maximum(h - 1, 0)
            st["acc_a"] = st["acc_a"] + _dot(st["o_prev"], wide(wo_v, hp))
        elif b == 1:
            cl = jnp.concatenate([clat_s[cb, rows(h, 8), :] for cb in range(DM // 128)],
                                 axis=1).astype(BF)
            st["ctx"] = _dot(cl, w1_s[h]).astype(BF)
        elif b == 2:
            st["acc_b"] = st["acc_b"] + _dot(st["ctx"], wide(bwo_v, h))

    def a_body(h, carry):
        acc_a, acc_b, o_prev, p = carry
        st = dict(acc_a=acc_a, acc_b=acc_b, o_prev=o_prev)
        s = jnp.zeros((8, WIN), F32)
        o = jnp.zeros((8, DH), F32)
        p_next = p
        for g in range(2):
            for j in range(NQ):
                v_lo(h, g, j).wait()
                if j == 0:
                    for jj in range(NQ):
                        k_hi(h + 1, g, jj).wait()
                v_lo(h + 2, g, j).start(priority=1)
                k_hi(h + 2, g, j).start(priority=0)
                if NOCOMP & 1:
                    continue
                if j in QKJ:
                    s = scores(h + 1, 2 * g + QKJ.index(j), s)
                if j in MJ:
                    b = 2 * g + MJ.index(j)
                    misc(h, b, st)
                    if b == NB - 1:
                        p_next = softmax(s)
                if j == NQ - 1:
                    for b in (2 * g, 2 * g + 1):
                        o = jnp.where(row8 == b, _dot(p, v_v[h % NSLOT, b]), o)
        return st["acc_a"], st["acc_b"], o.astype(BF), p_next

    zero = jnp.zeros((8, DM), F32)
    acc_a, acc_b, o_prev, p = lax.fori_loop(0, NH - 2, a_body, (zero, zero, jnp.zeros((8, DH), BF), p0))

    st = dict(acc_a=acc_a, acc_b=acc_b, o_prev=o_prev)
    cut = CV[3] * 4 // 128 * 128
    for h in (NH - 2, NH - 1):
        s = jnp.zeros((8, WIN), F32)
        o = jnp.zeros((8, DH), F32)
        for g in range(2):
            if h + 1 < NH:
                for j in range(NQ):
                    k_hi(h + 1, g, j).wait()
            for b in (2 * g, 2 * g + 1):
                if h + 1 < NH:
                    s = scores(h + 1, b, s)
                misc(h, b, st)
            if h + 1 < NH or g == 0:
                for j in range(NQ):
                    v_lo(h, g, j).wait()
                for b in (2 * g, 2 * g + 1):
                    o = jnp.where(row8 == b, _dot(p, v_v[h % NSLOT, b]), o)
            else:
                for j in range(NQ - 1):
                    v_lo(h, g, j).wait()
                part = [_dot(p[:, :cut], v_v[h % NSLOT, b, pl.ds(0, cut), :]) for b in (2, 3)]
                v_lo(h, g, NQ - 1).wait()
                for b in (2, 3):
                    o = jnp.where(row8 == b, part[b - 2] + _dot(p[:, cut:], v_v[h % NSLOT, b, pl.ds(cut, WIN - cut), :]), o)
        st["o_prev"] = o.astype(BF)
        if h + 1 < NH:
            p = softmax(s)
    acc_a = st["acc_a"] + _dot(st["o_prev"], wide(wo_v, NH - 1))
    acc_b = st["acc_b"]
    out_ref[:, :DM] = acc_a[:NB].astype(BF)
    out_ref[:, DM:] = acc_b[:NB].astype(BF)


@jax.jit
def pallas_concat_heads__sliding_block_cached__compressed_kv_cla__decode_kernel(
    A_x: jax.Array,
    A_k_cache: jax.Array,
    A_v_cache: jax.Array,
    A_wq: jax.Array,
    A_wo: jax.Array,
    B_x: jax.Array,
    B_c_kv: jax.Array,
    B_w_q: jax.Array,
    B_w_uk: jax.Array,
    B_w_uv: jax.Array,
    B_w_o: jax.Array,
):
    def tiles(w):
        r, c = w.shape
        return w.reshape(r // 8, 8, c // 128, 128).transpose(0, 2, 1, 3).reshape(r * c // 1024, 8, 128)

    out = pl.pallas_call(
        _kernel,
        out_shape=jax.ShapeDtypeStruct((NB, 2 * DM), BF),
        in_specs=[pl.BlockSpec(memory_space=pl.ANY)] * 11,
        out_specs=pl.BlockSpec(memory_space=pltpu.VMEM),
        scratch_shapes=[
            pltpu.VMEM((NB, DM), BF), pltpu.VMEM((NB, DM), BF),
            pltpu.VMEM((2048, 8, 128), BF), pltpu.VMEM((2048, 8, 128), BF),
            pltpu.VMEM((DM * NH, DH), BF), pltpu.VMEM((DM * NH, DH), BF), pltpu.VMEM((DM * NH, DH), BF),
            pltpu.VMEM((2048, 8, 128), BF),
            pltpu.VMEM((NB * 2048, 8, 128), BF),
            pltpu.VMEM((NSLOT, NB, WIN, DH), BF), pltpu.VMEM((NSLOT, NB, WIN, DH), BF),
            pltpu.VMEM((NH, 8, DH), F32), pltpu.VMEM((NH, 8, DH), F32),
            pltpu.VMEM((DM // 128, NH * 8, 128), F32),
            pltpu.VMEM((DM // 128, NH * 8, 128), F32),
            pltpu.VMEM((2, SK // 128, NH, 128), F32),
            pltpu.VMEM((NH, DM, DH), BF), pltpu.VMEM((NH, DM, DH), BF),
            pltpu.SemaphoreType.DMA((NG * NP + NG + 2 + 4 * NQ + 4,)),
        ],
        compiler_params=pltpu.CompilerParams(vmem_limit_bytes=100 * 1024 * 1024,
                                             disable_bounds_checks=True,
                                             disable_semaphore_checks=True),
    )(
        A_x.reshape(NB, DM), A_k_cache, A_v_cache, tiles(A_wq), tiles(A_wo),
        B_x.reshape(NB, DM), tiles(B_c_kv.reshape(NB * SK, DM)),
        B_w_q.reshape(DM * NH, DH), B_w_uk.reshape(DM * NH, DH), B_w_uv.reshape(DM * NH, DH),
        tiles(B_w_o.reshape(NH * DH, DM)),
    )
    return out.reshape(NB, 1, 2 * DM)
```

```python
import jax
import jax.numpy as jnp
from jax import lax
import jax.experimental.pallas as pl
import jax.experimental.pallas.tpu as pltpu

BF = jnp.bfloat16
F32 = jnp.float32
NT = (((1,), (1,)), ((), ()))

NB = 4
NH = 32
DH = 128
DM = 512
SK = 4096
WIN = 1024
NSLOT = 8
NG = 8
NQ = 8
DA = (26, 30)
DB = (30, 34)
HP = (0, -2, 0, -2)
CL = [26, 90, 154, 218]
CH = [30, 92, 158, 220]
SKEW = 0
SPLIT = 0
PVF = 0
SKB = 0
assert SKB <= 4
KSL = {0: 'qk0', 2: 'qk1', 4: 'qk2', 6: 'qk3'}
VSL = {0: 'sm', 1: 'ctx', 2: 'pv0', 3: 'outb', 4: 'pv1', 6: 'wo'}


def _dot(a, b):
    return jnp.dot(a, b, preferred_element_type=F32)


def _dot_nt(a, b):
    return lax.dot_general(a, b, NT, preferred_element_type=F32)


def _kernel(xa_hbm, k_hbm, v_hbm, wq_hbm, wo_hbm, xb_hbm, c_hbm, bwq_hbm, bwuk_hbm, bwuv_hbm, bwo_hbm,
            out_ref,
            xa_v, xb_v, wq_v, wo_v, bwq_v, bwuk_v, bwuv_v, bwo_v, c_v, k_v, v_v,
            qa_s, qb_s, qlat_s, clat_s, s0_s, s1_s, w1_s, w2_s,
            sem):
    scale = DH ** -0.5
    HIS, XS, LS, HS, ES = 64, 66, 68, 68 + 8 * NQ, 68 + 8 * NQ + 8

    def cp(src, dst, t0, nt, s):
        sl = pl.ds(t0, nt)
        return pltpu.make_async_copy(src.at[sl], dst.at[sl], sem.at[s])

    class Block:
        def __init__(self, src, dst, d, par, off=0):
            self.src, self.dst, self.par, self.off = src, dst, par, off
            self.dl, self.dh = d[0] // 2, d[1] // 2

        def lo(self, g, j):
            return cp(self.src, self.dst, self.off + self.dl + j * 32 + g * 128, 32, self.par * 32 + j + g * 4)

        def hi_start(self, g, j):
            s = HIS + self.par
            cut = lambda i: 1024 + self.dh + i * 32 + HP[i % 4] // 2

            def regular():
                cp(self.src, self.dst, self.off + cut(j - 1) + g * 128, cut(j) - cut(j - 1), s).start(priority=0)

            def edge():
                if j == 0:
                    cp(self.src, self.dst, self.off, self.dl, s).start(priority=0)
                    cp(self.src, self.dst, self.off + cut(31), 2048 - cut(31), s).start(priority=0)
                else:
                    cp(self.src, self.dst, self.off + 1024 + self.dl, cut(1) - 1024 - self.dl, s).start(priority=0)
            if j > 1:
                regular()
            elif isinstance(g, int):
                edge() if g == 0 else regular()
            else:
                pl.when(g == 0)(edge)
                pl.when(g > 0)(regular)

        def hi_wait(self):
            cp(self.src, self.dst, self.off, self.dl, HIS + self.par).wait()
            cp(self.src, self.dst, self.off + 1024 + self.dl, 1024 - self.dl, HIS + self.par).wait()

    def kv_piece(kv, h, pair, cuts, j, s):
        src, dst = ((k_hbm, k_v), (v_hbm, v_v))[kv]
        if j == 0:
            b0, nb, a, e = 0, 2, 0, cuts[0]
        elif j == NQ - 1:
            b0, nb, a, e = 0, 2, cuts[3], 256
        else:
            b0, nb, a, e = (j - 1) // 3, 1, cuts[(j - 1) % 3], cuts[(j - 1) % 3 + 1]
        bs, n = pl.ds(2 * pair + b0, nb), (e - a) * 4
        return pltpu.make_async_copy(src.at[bs, h, pl.ds(SK - WIN + a * 4, n), :],
                                     dst.at[h & (NSLOT - 1), bs, pl.ds(a * 4, n), :], sem.at[s])

    def kv_lo(h, kv, j):
        return kv_piece(kv, h, 0, CL, j, LS + ((h & 3) * 2 + kv) * NQ + j)

    def kv_hi(h, kv, j):
        return kv_piece(kv, h, 1, CH, j, HS + (h & 3) * 2 + kv)

    def kv_hi_wait(h, kv):
        for j in range(NQ):
            kv_hi(h, kv, j).wait()

    def kv_last(j):
        return kv_piece(1, NH - 1, 1, CL, j, ES + j)

    arrs = [(bwq_hbm, bwq_v, DB, 0), (bwuk_hbm, bwuk_v, DB, 0), (wq_hbm, wq_v, DA, 0)] + \
           [(c_hbm, c_v, DB, b * 2048) for b in range(NB)] + \
           [(bwuv_hbm, bwuv_v, DB, 0), (bwo_hbm, bwo_v, DB, 0), (wo_hbm, wo_v, DA, 0)]
    blocks = [Block(s, d, dd, i % 2, off) for i, (s, d, dd, off) in enumerate(arrs)]

    def run_block(k, jobs, init):
        def group(g, c):
            for j in range(4):
                blocks[k].lo(g, j).wait()
                if j == 0 and k > 0:
                    pl.when(g == 3)(blocks[k - 1].hi_wait)
                if j + SKB < 4:
                    blocks[k + 1].lo(g, j + SKB).start(priority=1)
                else:
                    pl.when(g < NG - 1)(lambda: blocks[k + 1].lo(jnp.minimum(g + 1, NG - 1), j + SKB - 4).start(priority=1))
                    pl.when(g == NG - 1)(lambda: (blocks[k + 2].lo(0, j + SKB - 4) if k + 2 < len(blocks)
                                                  else kv_lo(0, 0, j + SKB - 4)).start(priority=1))
                blocks[k].hi_start(g, j)
                for job in jobs.get(j, ()):
                    c = job(g, c)
            return c
        return lax.fori_loop(0, NG, group, init)

    def unit(g, j):
        return (4 * g + j + 2) & 31

    xa_cp = pltpu.make_async_copy(xa_hbm, xa_v, sem.at[XS])
    xb_cp = pltpu.make_async_copy(xb_hbm, xb_v, sem.at[XS + 1])

    for g in range(NG):
        for j in range(4):
            blocks[0].lo(g, j).start(priority=1)
    for j in range(SKB):
        blocks[1].lo(0, j).start(priority=1)
    xa_cp.start()
    xb_cp.start()

    row8 = lax.broadcasted_iota(jnp.int32, (8, 1), 0)

    def pad8(x4):
        return jnp.concatenate([x4.astype(F32), jnp.zeros((4, x4.shape[1]), F32)], axis=0).astype(BF)

    def rows(u, n, k=1):
        return pl.ds(u * n if isinstance(u, int) else pl.multiple_of(u * n, n), n * k)

    def wide(ref, u, k=1):
        t = ref[rows(u, 64, k)].reshape(16 * k, DM // 128, 8, 128)
        return jnp.concatenate([t[:, j].reshape(128 * k, 128) for j in range(DM // 128)], axis=1)

    def deinterleave(src_ref, dst_ref, j):
        def job(g, c):
            u = unit(g, j)
            dst_ref[:, rows(u, 16), :] = jnp.swapaxes(src_ref[rows(u, 64)].reshape(16, NH, DH), 0, 1)
            return c
        return job

    clat_s[...] = jnp.zeros(clat_s.shape, F32)
    run_block(0, {}, 0)
    xa_cp.wait()
    xb_cp.wait()
    xa = pad8(xa_v[...])
    xb = pad8(xb_v[...])

    run_block(1, {j: [deinterleave(bwq_v, w1_s, j)] for j in range(4)}, 0)

    run_block(2, {j: [deinterleave(bwuk_v, w2_s, j)] for j in range(4)}, 0)

    def qb_job(g, c):
        for h in range(4):
            qb_s[h] = _dot(xb, w1_s[4 * g + h])
        return c

    def ql_job(j):
        def job(g, c):
            h = 4 * g + j
            ql = _dot_nt(qb_s[j].astype(BF), w2_s[h]) * scale
            for cb in range(DM // 128):
                qlat_s[cb, rows(h, 8), :] = ql[:, cb * 128:(cb + 1) * 128]
            return c
        return job
    run_block(3, {0: [qb_job], 1: [ql_job(0), ql_job(1)], 2: [ql_job(2), ql_job(3)]}, 0)

    m_prev = None
    for b in range(NB + 1):
        if b < NB:
            ql = jnp.concatenate([qlat_s[cb, pl.ds(b, NH, stride=8), :] for cb in range(DM // 128)],
                                 axis=1).astype(BF)

        def qk_job(j, b=b, ql=ql):
            def job(g, c):
                m_run, l_run, acc = c
                u = unit(g, j)
                s = _dot_nt(ql, wide(c_v, b * 32 + u, 2))
                for k in range(2):
                    (s0_s, s1_s)[b % 2][u + k] = s[:, k * 128:(k + 1) * 128]
                    m_run = jnp.maximum(m_run, s[:, k * 128:(k + 1) * 128])
                return m_run, l_run, acc
            return job

        def pv_job(j, b=b, m_prev=m_prev):
            def job(g, c):
                m_run, l_run, acc = c
                u = 4 * g + j
                ps = [jnp.exp((s0_s, s1_s)[(b - 1) % 2][u + k] - m_prev) for k in range(2)]
                p = jnp.concatenate(ps, axis=1).astype(BF)
                return m_run, l_run + ps[0] + ps[1], acc + _dot(p, wide(c_v, (b - 1) * 32 + u, 2))
            return job

        def qa_job(j):
            def job(g, c):
                for h in (4 * g + j, 4 * g + j + 1):
                    w = jnp.concatenate([wq_v[sl * NH + h] for sl in range(DM // 8)], axis=0)
                    qa_s[h] = _dot(xa, w) * scale
                return c
            return job

        jobs = {j: [] for j in range(4)}
        for j in (0, 2):
            if b < NB and not PVF:
                jobs[j].append(qk_job(j))
            jobs[j + SPLIT].append(qa_job(j) if b == 0 else pv_job(j))
            if b < NB and PVF:
                jobs[j].append(qk_job(j))
        init = (jnp.full((NH, 128), -jnp.inf, F32), jnp.zeros((NH, 128), F32), jnp.zeros((NH, DM), F32))
        m_run, l_run, acc = run_block(4 + b, jobs, init)
        if b > 0:
            cl = acc / jnp.sum(l_run, axis=1, keepdims=True)
            for cb in range(DM // 128):
                clat_s[cb, pl.ds(b - 1, NH, stride=8), :] = cl[:, cb * 128:(cb + 1) * 128]
        if b < NB:
            m_prev = jnp.broadcast_to(jnp.max(m_run, axis=1, keepdims=True), (NH, 128))

    first = [(h, kv, j) for h in range(3) for kv in range(2) for j in range(NQ)][SKB:4 * NQ + SKEW]
    n_first = len(first)
    for t in range(32):
        blocks[9].lo(t // 4, t % 4).wait()
        if t == 12:
            blocks[8].hi_wait()
        while n_first - len(first) < -(-(t + 1) * n_first // 32):
            kv_lo(*first.pop(0)).start(priority=1)
        blocks[9].hi_start(t // 4, t % 4)
        deinterleave(bwuv_v, w1_s, t % 4)(t // 4, 0)

    def softmax(s):
        p = jnp.exp(s - jnp.max(s, axis=1, keepdims=True))
        return (p * (1.0 / jnp.sum(p, axis=1, keepdims=True))).astype(BF)

    def qk(h, b, s):
        return jnp.where(row8 == b, _dot_nt(qa_s[h].astype(BF), k_v[h & (NSLOT - 1), b]), s)

    def pv(h, pair, p, o):
        for b in (2 * pair, 2 * pair + 1):
            o = jnp.where(row8 == b, _dot(p, v_v[h & (NSLOT - 1), b]), o)
        return o

    def ctx_of(h):
        cl = jnp.concatenate([clat_s[cb, rows(h, 8), :] for cb in range(DM // 128)], axis=1).astype(BF)
        return _dot(cl, w1_s[h]).astype(BF)

    def lo_start(h, i):
        hh, kv, j = h + 2 + i // (2 * NQ), (i // NQ) % 2, i % NQ
        if isinstance(h, int):
            return kv_lo(hh, kv, j).start(priority=1)
        odd = (NH - 2) if kv == 1 else (NH - 1)
        pl.when(jnp.logical_and(hh != odd, hh < NH))(
            lambda: kv_lo(jnp.minimum(hh, NH - 1), kv, j).start(priority=1))
        pl.when(hh == odd)(lambda: kv_lo(2 * NH - 3 - odd, 1 - kv, j).start(priority=1))
        if i >= 2 * NQ:
            pl.when(hh == NH)(lambda: kv_last(j).start(priority=1))

    zero = jnp.zeros((8, DM), F32)
    acc_b = zero
    for kv in range(2):
        for j in range(NQ):
            kv_lo(0, kv, j).wait()
            lo_start(0, kv * NQ + j + SKEW)
            kv_hi(0, kv, j).start(priority=0)
            t = kv * NQ + j
            if t in (0, 4, 8):
                ctx = ctx_of(t // 4)
            elif t in (2, 6, 10):
                acc_b = acc_b + _dot(ctx, wide(bwo_v, t // 4))
    blocks[9].hi_wait()

    def job(name, h, st):
        if name.startswith("qk"):
            st["s"] = qk(h, int(name[2]), st["s"])
        elif name == "sm":
            st["p"] = softmax(st["s"])
        elif name.startswith("pv"):
            st["o"] = pv(h, int(name[2]), st["p"], st["o"])
        elif name == "wo":
            st["acc_a"] = st["acc_a"] + _dot(st["o"].astype(BF), wide(wo_v, h))
        elif name == "ctx":
            st["ctx"] = ctx_of(h + 3)
        elif name == "outb":
            st["acc_b"] = st["acc_b"] + _dot(st["ctx"], wide(bwo_v, h + 3))

    def fresh(**kw):
        return dict(s=jnp.zeros((8, WIN), F32), o=jnp.zeros((8, DH), F32), **kw)

    def a_body(h, carry):
        st = fresh(acc_a=carry[0], acc_b=carry[1])
        for kv, slots in enumerate((KSL, VSL)):
            for j in range(NQ):
                kv_lo(h, kv, j).wait()
                if slots.get(j) in ("qk2", "pv1"):
                    kv_hi_wait(h - 1, kv)
                lo_start(h, kv * NQ + j + SKEW)
                kv_hi(h, kv, j).start(priority=0)
                if j in slots:
                    job(slots[j], h - 1, st)
        return st["acc_a"], st["acc_b"]

    acc_a, acc_b = lax.fori_loop(1, NH - 2, a_body, (zero, acc_b))
    out_ref[:, DM:] = acc_b[:NB].astype(BF)

    X, Y, Z = NH - 3, NH - 2, NH - 1
    sx, sy, sz = fresh(acc_a=acc_a), fresh(), fresh()
    plan = [((Y, 0), {0: (sx, X, "qk0"), 2: (sx, X, "qk1"), 4: (sx, X, "qk2"), 6: (sx, X, "qk3")}),
            ((Z, 0), {0: (sx, X, "sm"), 1: (sx, X, "pv0"), 2: (sx, X, "pv1"), 3: (sx, X, "wo"),
                      4: (sy, Y, "qk0"), 6: (sy, Y, "qk1")}),
            ((Y, 1), {0: (sy, Y, "qk2"), 2: (sy, Y, "qk3"), 3: (sy, Y, "sm"), 4: (sz, Z, "qk0"), 6: (sz, Z, "qk1")})]
    for n, ((h, kv), slots) in enumerate(plan):
        for j in range(NQ):
            kv_lo(h, kv, j).wait()
            if j in slots and slots[j][2] in ("qk2", "pv1"):
                kv_hi_wait(slots[j][1], int(slots[j][2] == "pv1"))
            if n == 0 and j + SKEW < NQ:
                kv_last(j + SKEW).start(priority=1)
            kv_hi(h, kv, j).start(priority=0)
            if j in slots:
                job(slots[j][2], slots[j][1], slots[j][0])
    job("pv0", Y, sy)
    kv_hi_wait(Z, 0)
    job("qk2", Z, sz)
    job("qk3", Z, sz)
    job("sm", Z, sz)
    kv_hi_wait(Y, 1)
    job("pv1", Y, sy)
    sy["acc_a"] = sx["acc_a"]
    job("wo", Y, sy)
    for j in range(NQ):
        kv_lo(Z, 1, j).wait()
    job("pv0", Z, sz)
    for j in range(NQ - 1):
        kv_last(j).wait()
    cut, p, o = CL[3] * 4 // 128 * 128, sz["p"], sz["o"]
    for b in (2, 3):
        o = jnp.where(row8 == b, _dot(p[:, :cut], v_v[Z & (NSLOT - 1), b, pl.ds(0, cut), :]), o)
    kv_last(NQ - 1).wait()
    o2 = jnp.zeros((8, DH), F32)
    for b in (2, 3):
        o2 = jnp.where(row8 == b, _dot(p[:, cut:], v_v[Z & (NSLOT - 1), b, pl.ds(cut, WIN - cut), :]), o2)
    o = o + o2
    acc_a = sy["acc_a"] + _dot(o.astype(BF), wide(wo_v, Z))
    out_ref[:, :DM] = acc_a[:NB].astype(BF)


@jax.jit
def pallas_concat_heads__sliding_block_cached__compressed_kv_cla__decode_kernel(
    A_x: jax.Array,
    A_k_cache: jax.Array,
    A_v_cache: jax.Array,
    A_wq: jax.Array,
    A_wo: jax.Array,
    B_x: jax.Array,
    B_c_kv: jax.Array,
    B_w_q: jax.Array,
    B_w_uk: jax.Array,
    B_w_uv: jax.Array,
    B_w_o: jax.Array,
):
    def tiles(w):
        c = w.shape[-1]
        r = w.size // c
        return w.reshape(r // 8, 8, c // 128, 128).transpose(0, 2, 1, 3).reshape(r * c // 1024, 8, 128)

    out = pl.pallas_call(
        _kernel,
        out_shape=jax.ShapeDtypeStruct((NB, 2 * DM), BF),
        in_specs=[pl.BlockSpec(memory_space=pl.ANY)] * 11,
        out_specs=pl.BlockSpec(memory_space=pltpu.VMEM),
        scratch_shapes=[
            pltpu.VMEM((NB, DM), BF), pltpu.VMEM((NB, DM), BF),
        ] + [pltpu.VMEM((2048, 8, 128), BF)] * 6 + [
            pltpu.VMEM((NB * 2048, 8, 128), BF),
            pltpu.VMEM((NSLOT, NB, WIN, DH), BF), pltpu.VMEM((NSLOT, NB, WIN, DH), BF),
            pltpu.VMEM((NH, 8, DH), F32), pltpu.VMEM((4, 8, DH), F32),
            pltpu.VMEM((DM // 128, NH * 8, 128), F32),
            pltpu.VMEM((DM // 128, NH * 8, 128), F32),
            pltpu.VMEM((SK // 128, NH, 128), F32), pltpu.VMEM((SK // 128, NH, 128), F32),
            pltpu.VMEM((NH, DM, DH), BF), pltpu.VMEM((NH, DM, DH), BF),
            pltpu.SemaphoreType.DMA((68 + 8 * NQ + 8 + NQ,)),
        ],
        compiler_params=pltpu.CompilerParams(vmem_limit_bytes=100 * 1024 * 1024,
                                             disable_bounds_checks=True,
                                             disable_semaphore_checks=True),
    )(
        A_x.reshape(NB, DM), A_k_cache, A_v_cache, tiles(A_wq), tiles(A_wo),
        B_x.reshape(NB, DM), tiles(B_c_kv), tiles(B_w_q), tiles(B_w_uk), tiles(B_w_uv), tiles(B_w_o),
    )
    return out.reshape(NB, 1, 2 * DM)
```

```python
import jax
import jax.numpy as jnp
from jax import lax
import jax.experimental.pallas as pl
import jax.experimental.pallas.tpu as pltpu

BF = jnp.bfloat16
F32 = jnp.float32
NT = (((1,), (1,)), ((), ()))

NB = 4
NH = 32
DH = 128
DM = 512
SK = 4096
WIN = 1024
NSLOT = 8
NG = 8
NQ = 8
DA = (26, 30)
DB = (30, 34)
HP = (0, -2, 0, -2)
CL = [26, 90, 154, 218]
CH = [30, 92, 158, 220]
SKEW = 0
SPLIT = 0
PVF = 0
LATE = [1984, 2048]
SKB = 0
assert SKB <= 4
KSL = {0: 'qk0', 2: 'qk1', 4: 'qk2', 6: 'qk3'}
VSL = {0: 'sm', 1: 'ctx', 2: 'pv0', 3: 'outb', 4: 'pv1', 6: 'wo'}


def _dot(a, b):
    return jnp.dot(a, b, preferred_element_type=F32)


def _dot_nt(a, b):
    return lax.dot_general(a, b, NT, preferred_element_type=F32)


def _kernel(xa_hbm, k_hbm, v_hbm, wq_hbm, wo_hbm, xb_hbm, c_hbm, bwq_hbm, bwuk_hbm, bwuv_hbm, bwo_hbm,
            out_ref,
            xa_v, xb_v, wq_v, wo_v, bwq_v, bwuk_v, bwuv_v, bwo_v, c_v, k_v, v_v,
            qa_s, qb_s, qlat_s, clat_s, s0_s, s1_s, w1_s, w2_s, ob_s,
            sem):
    scale = DH ** -0.5
    HIS, XS, LS, HS, ES = 64, 66, 68, 68 + 8 * NQ, 68 + 8 * NQ + 8

    def cp(src, dst, t0, nt, s):
        sl = pl.ds(t0, nt)
        return pltpu.make_async_copy(src.at[sl], dst.at[sl], sem.at[s])

    class Block:
        def __init__(self, src, dst, d, par, off=0):
            self.src, self.dst, self.par, self.off = src, dst, par, off
            self.dl, self.dh = d[0] // 2, d[1] // 2
            self.end = 2048

        def lo(self, g, j):
            return cp(self.src, self.dst, self.off + self.dl + j * 32 + g * 128, 32, self.par * 32 + j + g * 4)

        def hi(self, g, j, edge):
            cut = lambda i: 1024 + self.dh + i * 32 + HP[i % 4] // 2
            if not edge:
                spans = [(cut(j - 1), cut(j), g * 128)]
            elif j == 0:
                spans = [(0, self.dl, 0), (cut(31), 2048, 0)]
            else:
                spans = [(1024 + self.dl, cut(1), 0)]
            if self.end < 2048:
                spans = [(a, min(e, self.end - o), o) for a, e, o in spans if a + o < self.end]
            return [cp(self.src, self.dst, self.off + a + o, e - a, HIS + self.par) for a, e, o in spans]

        def hi_start(self, g, j):
            def go(edge):
                def f():
                    for c in self.hi(g, j, edge):
                        c.start(priority=0)
                return f
            if j > 1 or isinstance(g, int):
                go(j <= 1 and g == 0)()
            else:
                pl.when(g == 0)(go(True))
                pl.when(g > 0)(go(False))

        def hi_wait(self):
            for g in range(NG):
                for j in range(4):
                    for c in self.hi(g, j, j <= 1 and g == 0):
                        c.wait()

    def kv_piece(kv, h, pair, cuts, j, s):
        src, dst = ((k_hbm, k_v), (v_hbm, v_v))[kv]
        if j == 0:
            b0, nb, a, e = 0, 2, 0, cuts[0]
        elif j == NQ - 1:
            b0, nb, a, e = 0, 2, cuts[3], 256
        else:
            b0, nb, a, e = (j - 1) // 3, 1, cuts[(j - 1) % 3], cuts[(j - 1) % 3 + 1]
        bs, n = pl.ds(2 * pair + b0, nb), (e - a) * 4
        return pltpu.make_async_copy(src.at[bs, h, pl.ds(SK - WIN + a * 4, n), :],
                                     dst.at[h & (NSLOT - 1), bs, pl.ds(a * 4, n), :], sem.at[s])

    def kv_lo(h, kv, j):
        return kv_piece(kv, h, 0, CL, j, LS + ((h & 3) * 2 + kv) * NQ + j)

    def kv_hi(h, kv, j):
        return kv_piece(kv, h, 1, CH, j, HS + (h & 3) * 2 + kv)

    def kv_hi_wait(h, kv):
        for j in range(NQ):
            kv_hi(h, kv, j).wait()

    def kv_last(j):
        return kv_piece(1, NH - 1, 1, CL, j, ES + j)

    arrs = [(bwq_hbm, bwq_v, DB, 0), (bwuk_hbm, bwuk_v, DB, 0), (wq_hbm, wq_v, DA, 0)] + \
           [(c_hbm, c_v, DB, b * 2048) for b in range(NB)] + \
           [(bwuv_hbm, bwuv_v, DB, 0), (bwo_hbm, bwo_v, DB, 0), (wo_hbm, wo_v, DA, 0)]
    blocks = [Block(s, d, dd, i % 2, off) for i, (s, d, dd, off) in enumerate(arrs)]

    blocks[9].end = LATE[0]

    def wo_late(j):
        return cp(wo_hbm, wo_v, LATE[j], LATE[j + 1] - LATE[j], ES + NQ + j)

    def run_block(k, jobs, init):
        def group(g, c):
            for j in range(4):
                blocks[k].lo(g, j).wait()
                if j == 0 and k > 0:
                    pl.when(g == 3)(blocks[k - 1].hi_wait)
                if j + SKB < 4:
                    blocks[k + 1].lo(g, j + SKB).start(priority=1)
                else:
                    pl.when(g < NG - 1)(lambda: blocks[k + 1].lo(jnp.minimum(g + 1, NG - 1), j + SKB - 4).start(priority=1))
                    pl.when(g == NG - 1)(lambda: (blocks[k + 2].lo(0, j + SKB - 4) if k + 2 < len(blocks)
                                                  else kv_lo(0, 0, j + SKB - 4)).start(priority=1))
                blocks[k].hi_start(g, j)
                for job in jobs.get(j, ()):
                    c = job(g, c)
            return c
        return lax.fori_loop(0, NG, group, init)

    def unit(g, j):
        return (4 * g + j + 2) & 31

    xa_cp = pltpu.make_async_copy(xa_hbm, xa_v, sem.at[XS])
    xb_cp = pltpu.make_async_copy(xb_hbm, xb_v, sem.at[XS + 1])

    for g in range(NG):
        for j in range(4):
            blocks[0].lo(g, j).start(priority=1)
    for j in range(SKB):
        blocks[1].lo(0, j).start(priority=1)
    xa_cp.start()
    xb_cp.start()

    row8 = lax.broadcasted_iota(jnp.int32, (8, 1), 0)

    def pad8(x4):
        return jnp.concatenate([x4.astype(F32), jnp.zeros((4, x4.shape[1]), F32)], axis=0).astype(BF)

    def rows(u, n, k=1):
        return pl.ds(u * n if isinstance(u, int) else pl.multiple_of(u * n, n), n * k)

    def wide(ref, u, k=1):
        t = ref[rows(u, 64, k)].reshape(16 * k, DM // 128, 8, 128)
        return jnp.concatenate([t[:, j].reshape(128 * k, 128) for j in range(DM // 128)], axis=1)

    def deinterleave(src_ref, dst_ref, j):
        def job(g, c):
            u = unit(g, j)
            dst_ref[:, rows(u, 16), :] = jnp.swapaxes(src_ref[rows(u, 64)].reshape(16, NH, DH), 0, 1)
            return c
        return job

    clat_s[...] = jnp.zeros(clat_s.shape, F32)
    run_block(0, {}, 0)
    xa_cp.wait()
    xb_cp.wait()
    xa = pad8(xa_v[...])
    xb = pad8(xb_v[...])

    run_block(1, {j: [deinterleave(bwq_v, w1_s, j)] for j in range(4)}, 0)

    run_block(2, {j: [deinterleave(bwuk_v, w2_s, j)] for j in range(4)}, 0)

    def qb_job(g, c):
        for h in range(4):
            qb_s[h] = _dot(xb, w1_s[4 * g + h])
        return c

    def ql_job(j):
        def job(g, c):
            h = 4 * g + j
            ql = _dot_nt(qb_s[j].astype(BF), w2_s[h]) * scale
            for cb in range(DM // 128):
                qlat_s[cb, rows(h, 8), :] = ql[:, cb * 128:(cb + 1) * 128]
            return c
        return job
    run_block(3, {0: [qb_job], 1: [ql_job(0), ql_job(1)], 2: [ql_job(2), ql_job(3)]}, 0)

    m_prev = None
    for b in range(NB + 1):
        if b < NB:
            ql = jnp.concatenate([qlat_s[cb, pl.ds(b, NH, stride=8), :] for cb in range(DM // 128)],
                                 axis=1).astype(BF)

        def qk_job(j, b=b, ql=ql):
            def job(g, c):
                m_run, l_run, acc = c
                u = unit(g, j)
                s = _dot_nt(ql, wide(c_v, b * 32 + u, 2))
                for k in range(2):
                    (s0_s, s1_s)[b % 2][u + k] = s[:, k * 128:(k + 1) * 128]
                    m_run = jnp.maximum(m_run, s[:, k * 128:(k + 1) * 128])
                return m_run, l_run, acc
            return job

        def pv_job(j, b=b, m_prev=m_prev):
            def job(g, c):
                m_run, l_run, acc = c
                u = 4 * g + j
                ps = [jnp.exp((s0_s, s1_s)[(b - 1) % 2][u + k] - m_prev) for k in range(2)]
                p = jnp.concatenate(ps, axis=1).astype(BF)
                return m_run, l_run + ps[0] + ps[1], acc + _dot(p, wide(c_v, (b - 1) * 32 + u, 2))
            return job

        def qa_job(j):
            def job(g, c):
                for h in (4 * g + j, 4 * g + j + 1):
                    w = jnp.concatenate([wq_v[sl * NH + h] for sl in range(DM // 8)], axis=0)
                    qa_s[h] = _dot(xa, w) * scale
                return c
            return job

        jobs = {j: [] for j in range(4)}
        for j in (0, 2):
            if b < NB and not PVF:
                jobs[j].append(qk_job(j))
            jobs[j + SPLIT].append(qa_job(j) if b == 0 else pv_job(j))
            if b < NB and PVF:
                jobs[j].append(qk_job(j))
        init = (jnp.full((NH, 128), -jnp.inf, F32), jnp.zeros((NH, 128), F32), jnp.zeros((NH, DM), F32))
        m_run, l_run, acc = run_block(4 + b, jobs, init)
        if b > 0:
            cl = acc / jnp.sum(l_run, axis=1, keepdims=True)
            for cb in range(DM // 128):
                clat_s[cb, pl.ds(b - 1, NH, stride=8), :] = cl[:, cb * 128:(cb + 1) * 128]
        if b < NB:
            m_prev = jnp.broadcast_to(jnp.max(m_run, axis=1, keepdims=True), (NH, 128))

    first = [(h, kv, j) for h in range(3) for kv in range(2) for j in range(NQ)][SKB:4 * NQ + SKEW]
    n_first = len(first)
    for t in range(32):
        blocks[9].lo(t // 4, t % 4).wait()
        if t == 12:
            blocks[8].hi_wait()
        while n_first - len(first) < -(-(t + 1) * n_first // 32):
            kv_lo(*first.pop(0)).start(priority=1)
        blocks[9].hi_start(t // 4, t % 4)
        deinterleave(bwuv_v, w1_s, t % 4)(t // 4, 0)

    def softmax(s):
        p = jnp.exp(s - jnp.max(s, axis=1, keepdims=True))
        return (p * (1.0 / jnp.sum(p, axis=1, keepdims=True))).astype(BF)

    def qk(h, b, s):
        return jnp.where(row8 == b, _dot_nt(qa_s[h].astype(BF), k_v[h & (NSLOT - 1), b]), s)

    def pv(h, pair, p, o):
        for b in (2 * pair, 2 * pair + 1):
            o = jnp.where(row8 == b, _dot(p, v_v[h & (NSLOT - 1), b]), o)
        return o

    def ctx_of(h):
        cl = jnp.concatenate([clat_s[cb, rows(h, 8), :] for cb in range(DM // 128)], axis=1).astype(BF)
        return _dot(cl, w1_s[h]).astype(BF)

    def lo_start(h, i):
        hh, kv, j = h + 2 + i // (2 * NQ), (i // NQ) % 2, i % NQ
        if isinstance(h, int):
            return kv_lo(hh, kv, j).start(priority=1)
        odd = (NH - 2) if kv == 1 else (NH - 1)
        pl.when(jnp.logical_and(hh != odd, hh < NH))(
            lambda: kv_lo(jnp.minimum(hh, NH - 1), kv, j).start(priority=1))
        pl.when(hh == odd)(lambda: kv_lo(2 * NH - 3 - odd, 1 - kv, j).start(priority=1))
        if i >= 2 * NQ:
            pl.when(hh == NH)(lambda: kv_last(j).start(priority=1))

    zero = jnp.zeros((8, DM), F32)
    acc_b = zero
    for kv in range(2):
        for j in range(NQ):
            kv_lo(0, kv, j).wait()
            lo_start(0, kv * NQ + j + SKEW)
            kv_hi(0, kv, j).start(priority=0)
            t = kv * NQ + j
            if t in (0, 4, 8):
                ctx = ctx_of(t // 4)
            elif t in (2, 6, 10):
                acc_b = acc_b + _dot(ctx, wide(bwo_v, t // 4))
    blocks[9].hi_wait()

    def job(name, h, st):
        if name.startswith("qk"):
            st["s"] = qk(h, int(name[2]), st["s"])
        elif name == "sm":
            st["p"] = softmax(st["s"])
        elif name.startswith("pv"):
            st["o"] = pv(h, int(name[2]), st["p"], st["o"])
        elif name == "wo":
            st["acc_a"] = st["acc_a"] + _dot(st["o"].astype(BF), wide(wo_v, h))
        elif name == "ctx":
            st["ctx"] = ctx_of(h + 3)
        elif name == "outb":
            st["acc_b"] = st["acc_b"] + _dot(st["ctx"], wide(bwo_v, h + 3))

    def fresh(**kw):
        return dict(s=jnp.zeros((8, WIN), F32), o=jnp.zeros((8, DH), F32), **kw)

    def a_body(h, carry):
        st = fresh(acc_a=carry[0], acc_b=carry[1])
        for kv, slots in enumerate((KSL, VSL)):
            for j in range(NQ):
                kv_lo(h, kv, j).wait()
                if slots.get(j) in ("qk2", "pv1"):
                    kv_hi_wait(h - 1, kv)
                lo_start(h, kv * NQ + j + SKEW)
                kv_hi(h, kv, j).start(priority=0)
                if j in slots:
                    job(slots[j], h - 1, st)
        return st["acc_a"], st["acc_b"]

    acc_a, acc_b = lax.fori_loop(1, NH - 2, a_body, (zero, acc_b))
    out_ref[:, DM:] = acc_b[:NB].astype(BF)

    X, Y, Z = NH - 3, NH - 2, NH - 1
    sx, sy, sz = fresh(acc_a=acc_a), fresh(), fresh()
    plan = [((Y, 0), {0: (sx, X, "qk0"), 2: (sx, X, "qk1"), 4: (sx, X, "qk2"), 6: (sx, X, "qk3")}),
            ((Z, 0), {0: (sx, X, "sm"), 1: (sx, X, "pv0"), 2: (sx, X, "pv1"), 3: (sx, X, "wo"),
                      4: (sy, Y, "qk0"), 6: (sy, Y, "qk1")}),
            ((Y, 1), {0: (sy, Y, "qk2"), 2: (sy, Y, "qk3"), 3: (sy, Y, "sm"), 4: (sz, Z, "qk0"), 6: (sz, Z, "qk1")})]
    for n, ((h, kv), slots) in enumerate(plan):
        for j in range(NQ):
            kv_lo(h, kv, j).wait()
            if j in slots and slots[j][2] in ("qk2", "pv1"):
                kv_hi_wait(slots[j][1], int(slots[j][2] == "pv1"))
            if n == 0 and j + SKEW < NQ:
                kv_last(j + SKEW).start(priority=1)
            if n == 1 and j < len(LATE) - 1:
                wo_late(j).start(priority=1)
            kv_hi(h, kv, j).start(priority=0)
            if j in slots:
                job(slots[j][2], slots[j][1], slots[j][0])
    job("pv0", Y, sy)
    kv_hi_wait(Z, 0)
    job("qk2", Z, sz)
    job("qk3", Z, sz)
    job("sm", Z, sz)
    kv_hi_wait(Y, 1)
    job("pv1", Y, sy)
    sy["acc_a"] = sx["acc_a"]
    job("wo", Y, sy)
    for j in range(NQ):
        kv_lo(Z, 1, j).wait()
    job("pv0", Z, sz)
    for j in range(NQ - 1):
        kv_last(j).wait()
    cut, p, o = CL[3] * 4 // 128 * 128, sz["p"], sz["o"]
    for b in (2, 3):
        o = jnp.where(row8 == b, _dot(p[:, :cut], v_v[Z & (NSLOT - 1), b, pl.ds(0, cut), :]), o)
    kv_last(NQ - 1).wait()
    o2 = jnp.zeros((8, DH), F32)
    for b in (2, 3):
        o2 = jnp.where(row8 == b, _dot(p[:, cut:], v_v[Z & (NSLOT - 1), b, pl.ds(cut, WIN - cut), :]), o2)
    o = (o + o2).astype(BF)
    if len(LATE) > 1:
        ob_s[...] = o
        for j in range(len(LATE) - 1):
            wo_late(j).wait()
        o = ob_s[...]
    acc_a = sy["acc_a"] + _dot(o, wide(wo_v, Z))
    out_ref[:, :DM] = acc_a[:NB].astype(BF)


@jax.jit
def pallas_concat_heads__sliding_block_cached__compressed_kv_cla__decode_kernel(
    A_x: jax.Array,
    A_k_cache: jax.Array,
    A_v_cache: jax.Array,
    A_wq: jax.Array,
    A_wo: jax.Array,
    B_x: jax.Array,
    B_c_kv: jax.Array,
    B_w_q: jax.Array,
    B_w_uk: jax.Array,
    B_w_uv: jax.Array,
    B_w_o: jax.Array,
):
    def tiles(w):
        c = w.shape[-1]
        r = w.size // c
        return w.reshape(r // 8, 8, c // 128, 128).transpose(0, 2, 1, 3).reshape(r * c // 1024, 8, 128)

    out = pl.pallas_call(
        _kernel,
        out_shape=jax.ShapeDtypeStruct((NB, 2 * DM), BF),
        in_specs=[pl.BlockSpec(memory_space=pl.ANY)] * 11,
        out_specs=pl.BlockSpec(memory_space=pltpu.VMEM),
        scratch_shapes=[
            pltpu.VMEM((NB, DM), BF), pltpu.VMEM((NB, DM), BF),
        ] + [pltpu.VMEM((2048, 8, 128), BF)] * 6 + [
            pltpu.VMEM((NB * 2048, 8, 128), BF),
            pltpu.VMEM((NSLOT, NB, WIN, DH), BF), pltpu.VMEM((NSLOT, NB, WIN, DH), BF),
            pltpu.VMEM((NH, 8, DH), F32), pltpu.VMEM((4, 8, DH), F32),
            pltpu.VMEM((DM // 128, NH * 8, 128), F32),
            pltpu.VMEM((DM // 128, NH * 8, 128), F32),
            pltpu.VMEM((SK // 128, NH, 128), F32), pltpu.VMEM((SK // 128, NH, 128), F32),
            pltpu.VMEM((NH, DM, DH), BF), pltpu.VMEM((NH, DM, DH), BF),
            pltpu.VMEM((8, DH), BF),
            pltpu.SemaphoreType.DMA((68 + 8 * NQ + 8 + NQ + 4,)),
        ],
        compiler_params=pltpu.CompilerParams(vmem_limit_bytes=100 * 1024 * 1024,
                                             disable_bounds_checks=True,
                                             disable_semaphore_checks=True),
    )(
        A_x.reshape(NB, DM), A_k_cache, A_v_cache, tiles(A_wq), tiles(A_wo),
        B_x.reshape(NB, DM), tiles(B_c_kv), tiles(B_w_q), tiles(B_w_uk), tiles(B_w_uv), tiles(B_w_o),
    )
    return out.reshape(NB, 1, 2 * DM)
```

```python
import jax
import jax.numpy as jnp
from jax import lax
import jax.experimental.pallas as pl
import jax.experimental.pallas.tpu as pltpu

BF = jnp.bfloat16
F32 = jnp.float32
NT = (((1,), (1,)), ((), ()))

NB = 4
NH = 32
DH = 128
DM = 512
SK = 4096
WIN = 1024
NSLOT = 8
NG = 8
NQ = 8
NC = DM // 128
DA = (26, 30)
DB = (30, 34)
HP = (0, -2, 0, -2)
CL = (26, 90, 154, 218)
CH = (30, 92, 158, 220)
HIS, XS, LS, HS, ES, NSEM = 32, 34, 36, 36 + 4 * NQ, 40 + 4 * NQ, 41 + 5 * NQ
K_JOBS = {0: "qk0", 2: "qk1", 4: "qk2", 6: "qk3"}
V_JOBS = {0: "sm", 1: "ctx", 2: "pv0", 3: "outb", 4: "pv1", 6: "wo"}


def _dot(a, b):
    return jnp.dot(a, b, preferred_element_type=F32)


def _dot_nt(a, b):
    return lax.dot_general(a, b, NT, preferred_element_type=F32)


def _kernel(xa_hbm, k_hbm, v_hbm, wq_hbm, wo_hbm, xb_hbm, c_hbm, bwq_hbm, bwuk_hbm, bwuv_hbm, bwo_hbm,
            out_ref,
            xa_v, xb_v, wq_v, wo_v, bwq_v, bwuk_v, bwuv_v, bwo_v, c_v, k_v, v_v,
            qa_s, qb_s, qlat_s, clat_s, s0_s, s1_s, w1_s, w2_s, o_s,
            sem):
    scale = DH ** -0.5

    def cp(src, dst, t0, nt, s):
        sl = pl.ds(t0, nt)
        return pltpu.make_async_copy(src.at[sl], dst.at[sl], sem.at[s])

    class Block:
        def __init__(self, src, dst, d, par, off, end=2048):
            self.src, self.dst, self.par, self.off, self.end = src, dst, par, off, end
            self.dl, self.dh = d[0] // 2, d[1] // 2

        def lo(self, g, j):
            return cp(self.src, self.dst, self.off + self.dl + j * 32 + g * 128, 32, j + g * 4)

        def hi(self, g, j, edge):
            cut = lambda i: 1024 + self.dh + i * 32 + HP[i % 4] // 2
            if not edge:
                spans = [(cut(j - 1), cut(j), g * 128)]
            elif j == 0:
                spans = [(0, self.dl, 0), (cut(31), 2048, 0)]
            else:
                spans = [(1024 + self.dl, cut(1), 0)]
            if self.end < 2048:
                spans = [(a, min(e, self.end - o), o) for a, e, o in spans if a + o < self.end]
            return [cp(self.src, self.dst, self.off + a + o, e - a, HIS + self.par) for a, e, o in spans]

        def hi_start(self, g, j):
            def go(edge):
                def start():
                    for c in self.hi(g, j, edge):
                        c.start(priority=0)
                return start
            if j > 1 or isinstance(g, int):
                go(j <= 1 and g == 0)()
            else:
                pl.when(g == 0)(go(True))
                pl.when(g > 0)(go(False))

        def hi_wait(self):
            for g in range(NG):
                for j in range(4):
                    for c in self.hi(g, j, j <= 1 and g == 0):
                        c.wait()

    late = 2048 - 64
    arrs = [(bwq_hbm, bwq_v, DB, 0), (bwuk_hbm, bwuk_v, DB, 0), (wq_hbm, wq_v, DA, 0)] + \
           [(c_hbm, c_v, DB, b * 2048) for b in range(NB)] + \
           [(bwuv_hbm, bwuv_v, DB, 0), (bwo_hbm, bwo_v, DB, 0), (wo_hbm, wo_v, DA, 0, late)]
    blocks = [Block(a[0], a[1], a[2], i % 2, *a[3:]) for i, a in enumerate(arrs)]

    def kv_piece(kv, h, pair, cuts, j, s):
        src, dst = ((k_hbm, k_v), (v_hbm, v_v))[kv]
        if j == 0:
            b0, nb, a, e = 0, 2, 0, cuts[0]
        elif j == NQ - 1:
            b0, nb, a, e = 0, 2, cuts[3], 256
        else:
            b0, nb, a, e = (j - 1) // 3, 1, cuts[(j - 1) % 3], cuts[(j - 1) % 3 + 1]
        bs, n = pl.ds(2 * pair + b0, nb), (e - a) * 4
        return pltpu.make_async_copy(src.at[bs, h, pl.ds(SK - WIN + a * 4, n), :],
                                     dst.at[h & (NSLOT - 1), bs, pl.ds(a * 4, n), :], sem.at[s])

    def kv_lo(h, kv, j, pos=None):
        par, grp = (h & 1, kv) if pos is None else pos
        return kv_piece(kv, h, 0, CL, j, LS + (par * 2 + grp) * NQ + j)

    def kv_hi(h, kv, j):
        return kv_piece(kv, h, 1, CH, j, HS + (h & 1) * 2 + kv)

    def kv_hi_wait(h, kv):
        for j in range(NQ):
            kv_hi(h, kv, j).wait()

    def v_last(j):
        return kv_piece(1, NH - 1, 1, CL, j, ES + j)

    def wo_last():
        return cp(wo_hbm, wo_v, late, 2048 - late, ES + NQ)

    def run_block(k, jobs, init):
        def group(g, c):
            for j in range(4):
                blocks[k].lo(g, j).wait()
                if j == 0 and k > 0:
                    pl.when(g == 3)(blocks[k - 1].hi_wait)
                blocks[k + 1].lo(g, j).start(priority=1)
                blocks[k].hi_start(g, j)
                for job in jobs.get(j, ()):
                    c = job(g, c)
            return c
        return lax.fori_loop(0, NG, group, init)

    def unit(g, j):
        return (4 * g + j + 2) & 31

    xa_cp = pltpu.make_async_copy(xa_hbm, xa_v, sem.at[XS])
    xb_cp = pltpu.make_async_copy(xb_hbm, xb_v, sem.at[XS + 1])

    for g in range(NG):
        for j in range(4):
            blocks[0].lo(g, j).start(priority=1)
    xa_cp.start()
    xb_cp.start()

    row8 = lax.broadcasted_iota(jnp.int32, (8, 1), 0)

    def pad8(x4):
        return jnp.concatenate([x4.astype(F32), jnp.zeros((4, x4.shape[1]), F32)], axis=0).astype(BF)

    def rows(u, n, k=1):
        return pl.ds(u * n if isinstance(u, int) else pl.multiple_of(u * n, n), n * k)

    def wide(ref, u, k=1):
        t = ref[rows(u, 64, k)].reshape(16 * k, NC, 8, 128)
        return jnp.concatenate([t[:, j].reshape(128 * k, 128) for j in range(NC)], axis=1)

    def deinterleave(src_ref, dst_ref, j):
        def job(g, c):
            u = unit(g, j)
            dst_ref[:, rows(u, 16), :] = jnp.swapaxes(src_ref[rows(u, 64)].reshape(16, NH, DH), 0, 1)
            return c
        return job

    clat_s[...] = jnp.zeros(clat_s.shape, F32)
    run_block(0, {}, 0)
    xa_cp.wait()
    xb_cp.wait()
    xa = pad8(xa_v[...])
    xb = pad8(xb_v[...])
    run_block(1, {j: [deinterleave(bwq_v, w1_s, j)] for j in range(4)}, 0)
    run_block(2, {j: [deinterleave(bwuk_v, w2_s, j)] for j in range(4)}, 0)

    def qb_job(g, c):
        for j in range(4):
            qb_s[j] = _dot(xb, w1_s[4 * g + j])
        return c

    def ql_job(j):
        def job(g, c):
            h = 4 * g + j
            ql = _dot_nt(qb_s[j].astype(BF), w2_s[h]) * scale
            for cb in range(NC):
                qlat_s[cb, rows(h, 8), :] = ql[:, cb * 128:(cb + 1) * 128]
            return c
        return job
    run_block(3, {0: [qb_job], 1: [ql_job(0), ql_job(1)], 2: [ql_job(2), ql_job(3)]}, 0)

    m_prev = None
    for b in range(NB + 1):
        if b < NB:
            ql = jnp.concatenate([qlat_s[cb, pl.ds(b, NH, stride=8), :] for cb in range(NC)],
                                 axis=1).astype(BF)

        def qk_job(j, b=b, ql=ql):
            def job(g, c):
                m_run, l_run, acc = c
                u = unit(g, j)
                s = _dot_nt(ql, wide(c_v, b * 32 + u, 2))
                for k in range(2):
                    (s0_s, s1_s)[b % 2][u + k] = s[:, k * 128:(k + 1) * 128]
                    m_run = jnp.maximum(m_run, s[:, k * 128:(k + 1) * 128])
                return m_run, l_run, acc
            return job

        def pv_job(j, b=b, m_prev=m_prev):
            def job(g, c):
                m_run, l_run, acc = c
                u = 4 * g + j
                ps = [jnp.exp((s0_s, s1_s)[(b - 1) % 2][u + k] - m_prev) for k in range(2)]
                p = jnp.concatenate(ps, axis=1).astype(BF)
                return m_run, l_run + ps[0] + ps[1], acc + _dot(p, wide(c_v, (b - 1) * 32 + u, 2))
            return job

        def qa_job(j):
            def job(g, c):
                for h in (4 * g + j, 4 * g + j + 1):
                    w = jnp.concatenate([wq_v[sl * NH + h] for sl in range(DM // 8)], axis=0)
                    qa_s[h] = _dot(xa, w) * scale
                return c
            return job

        jobs = {j: ([qk_job(j)] if b < NB else []) + [qa_job(j) if b == 0 else pv_job(j)] for j in (0, 2)}
        init = (jnp.full((NH, 128), -jnp.inf, F32), jnp.zeros((NH, 128), F32), jnp.zeros((NH, DM), F32))
        m_run, l_run, acc = run_block(4 + b, jobs, init)
        if b > 0:
            cl = acc / jnp.sum(l_run, axis=1, keepdims=True)
            for cb in range(NC):
                clat_s[cb, pl.ds(b - 1, NH, stride=8), :] = cl[:, cb * 128:(cb + 1) * 128]
        if b < NB:
            m_prev = jnp.broadcast_to(jnp.max(m_run, axis=1, keepdims=True), (NH, 128))

    for t in range(32):
        blocks[9].lo(t // 4, t % 4).wait()
        if t == 12:
            blocks[8].hi_wait()
        kv_lo(t // (2 * NQ), (t // NQ) % 2, t % NQ).start(priority=1)
        blocks[9].hi_start(t // 4, t % 4)
        deinterleave(bwuv_v, w1_s, t % 4)(t // 4, 0)

    X, Y, Z = NH - 3, NH - 2, NH - 1

    def ctx_of(h):
        cl = jnp.concatenate([clat_s[cb, rows(h, 8), :] for cb in range(NC)], axis=1).astype(BF)
        return _dot(cl, w1_s[h]).astype(BF)

    def job(name, h, st):
        slot = h & (NSLOT - 1)
        if name.startswith("qk"):
            b = int(name[2])
            st["s"] = jnp.where(row8 == b, _dot_nt(qa_s[h].astype(BF), k_v[slot, b]), st["s"])
        elif name == "sm":
            p = jnp.exp(st["s"] - jnp.max(st["s"], axis=1, keepdims=True))
            st["p"] = (p * (1.0 / jnp.sum(p, axis=1, keepdims=True))).astype(BF)
        elif name.startswith("pv"):
            for b in (2 * int(name[2]), 2 * int(name[2]) + 1):
                st["o"] = jnp.where(row8 == b, _dot(st["p"], v_v[slot, b]), st["o"])
        elif name == "wo":
            st["acc_a"] = st["acc_a"] + _dot(st["o"].astype(BF), wide(wo_v, h))
        elif name == "ctx":
            st["ctx"] = ctx_of(h + 3)
        elif name == "outb":
            st["acc_b"] = st["acc_b"] + _dot(st["ctx"], wide(bwo_v, h + 3))

    def fresh(**kw):
        return dict(s=jnp.zeros((8, WIN), F32), o=jnp.zeros((8, DH), F32), **kw)

    zero = jnp.zeros((8, DM), F32)
    acc_b = zero
    for t in range(2 * NQ):
        kv_lo(0, t // NQ, t % NQ).wait()
        kv_lo(2, t // NQ, t % NQ).start(priority=1)
        kv_hi(0, t // NQ, t % NQ).start(priority=0)
        if t in (0, 4, 8):
            ctx = ctx_of(t // 4)
        elif t in (2, 6, 10):
            acc_b = acc_b + _dot(ctx, wide(bwo_v, t // 4))
    blocks[9].hi_wait()

    def a_body(h, carry):
        st = fresh(acc_a=carry[0], acc_b=carry[1])
        for kv, jobs in enumerate((K_JOBS, V_JOBS)):
            swap, other = (Z, Y) if kv == 0 else (Y, Z)
            for j in range(NQ):
                kv_lo(h, kv, j).wait()
                if jobs.get(j) in ("qk2", "pv1"):
                    kv_hi_wait(h - 1, kv)
                pl.when(h + 2 != swap)(lambda: kv_lo(h + 2, kv, j).start(priority=1))
                pl.when(h + 2 == swap)(lambda: kv_lo(other, 1 - kv, j, (swap & 1, kv)).start(priority=1))
                kv_hi(h, kv, j).start(priority=0)
                if j in jobs:
                    job(jobs[j], h - 1, st)
        return st["acc_a"], st["acc_b"]

    acc_a, acc_b = lax.fori_loop(1, Y, a_body, (zero, acc_b))
    out_ref[:, DM:] = acc_b[:NB].astype(BF)

    sx, sy, sz = fresh(acc_a=acc_a), fresh(), fresh()
    plan = [((Y, 0, None), {0: (sx, X, "qk0"), 2: (sx, X, "qk1"), 4: (sx, X, "qk2"), 6: (sx, X, "qk3")}),
            ((Z, 0, (Y & 1, 1)), {0: (sx, X, "sm"), 1: (sx, X, "pv0"), 2: (sx, X, "pv1"), 3: (sx, X, "wo"),
                                  4: (sy, Y, "qk0"), 6: (sy, Y, "qk1")}),
            ((Y, 1, (Z & 1, 0)), {0: (sy, Y, "qk2"), 2: (sy, Y, "qk3"), 3: (sy, Y, "sm"),
                                  4: (sz, Z, "qk0"), 6: (sz, Z, "qk1")})]
    for n, ((h, kv, pos), jobs) in enumerate(plan):
        for j in range(NQ):
            kv_lo(h, kv, j, pos).wait()
            if j in jobs and jobs[j][2] in ("qk2", "pv1"):
                kv_hi_wait(jobs[j][1], int(jobs[j][2] == "pv1"))
            if n == 0:
                v_last(j).start(priority=1)
            elif n == 1 and j == 0:
                wo_last().start(priority=1)
            kv_hi(h, kv, j).start(priority=0)
            if j in jobs:
                job(jobs[j][2], jobs[j][1], jobs[j][0])
    job("pv0", Y, sy)
    kv_hi_wait(Z, 0)
    job("qk2", Z, sz)
    job("qk3", Z, sz)
    job("sm", Z, sz)
    kv_hi_wait(Y, 1)
    job("pv1", Y, sy)
    sy["acc_a"] = sx["acc_a"]
    job("wo", Y, sy)
    for j in range(NQ):
        kv_lo(Z, 1, j).wait()
    job("pv0", Z, sz)
    for j in range(NQ):
        v_last(j).wait()
    job("pv1", Z, sz)
    o_s[...] = sz["o"].astype(BF)
    wo_last().wait()
    acc_a = sy["acc_a"] + _dot(o_s[...], wide(wo_v, Z))
    out_ref[:, :DM] = acc_a[:NB].astype(BF)


@jax.jit
def pallas_concat_heads__sliding_block_cached__compressed_kv_cla__decode_kernel(
    A_x: jax.Array,
    A_k_cache: jax.Array,
    A_v_cache: jax.Array,
    A_wq: jax.Array,
    A_wo: jax.Array,
    B_x: jax.Array,
    B_c_kv: jax.Array,
    B_w_q: jax.Array,
    B_w_uk: jax.Array,
    B_w_uv: jax.Array,
    B_w_o: jax.Array,
):
    def tiles(w):
        c = w.shape[-1]
        r = w.size // c
        return w.reshape(r // 8, 8, c // 128, 128).transpose(0, 2, 1, 3).reshape(r * c // 1024, 8, 128)

    out = pl.pallas_call(
        _kernel,
        out_shape=jax.ShapeDtypeStruct((NB, 2 * DM), BF),
        in_specs=[pl.BlockSpec(memory_space=pl.ANY)] * 11,
        out_specs=pl.BlockSpec(memory_space=pltpu.VMEM),
        scratch_shapes=[
            pltpu.VMEM((NB, DM), BF), pltpu.VMEM((NB, DM), BF),
        ] + [pltpu.VMEM((2048, 8, 128), BF)] * 6 + [
            pltpu.VMEM((NB * 2048, 8, 128), BF),
            pltpu.VMEM((NSLOT, NB, WIN, DH), BF), pltpu.VMEM((NSLOT, NB, WIN, DH), BF),
            pltpu.VMEM((NH, 8, DH), F32), pltpu.VMEM((4, 8, DH), F32),
            pltpu.VMEM((NC, NH * 8 + 8, 128), F32),
            pltpu.VMEM((NC, NH * 8 + 8, 128), F32),
            pltpu.VMEM((SK // 128, NH, 128), F32), pltpu.VMEM((SK // 128, NH, 128), F32),
            pltpu.VMEM((NH, DM, DH), BF), pltpu.VMEM((NH, DM, DH), BF),
            pltpu.VMEM((8, DH), BF),
            pltpu.SemaphoreType.DMA((NSEM,)),
        ],
        compiler_params=pltpu.CompilerParams(vmem_limit_bytes=100 * 1024 * 1024,
                                             disable_bounds_checks=True,
                                             disable_semaphore_checks=True),
    )(
        A_x.reshape(NB, DM), A_k_cache, A_v_cache, tiles(A_wq), tiles(A_wo),
        B_x.reshape(NB, DM), tiles(B_c_kv), tiles(B_w_q), tiles(B_w_uk), tiles(B_w_uv), tiles(B_w_o),
    )
    return out.reshape(NB, 1, 2 * DM)
```

```python
import jax
import jax.numpy as jnp
from jax import lax
import jax.experimental.pallas as pl
import jax.experimental.pallas.tpu as pltpu

BF = jnp.bfloat16
F32 = jnp.float32
NT = (((1,), (1,)), ((), ()))

NB = 4
NH = 32
DH = 128
DM = 512
SK = 4096
WIN = 1024
NSLOT = 8
NG = 8
NQ = 8
NC = DM // 128
LT = 64
DA = (26, 30)
DB = (30, 34)
HP = (0, -2, 0, -2)
CL = (26, 90, 154, 218)
CH = (30, 92, 158, 220)
HIS, XS, LS, HS, ES, NSEM = 32, 34, 36, 36 + 4 * NQ, 40 + 4 * NQ, 41 + 5 * NQ
K_JOBS = {0: "qk0", 2: "qk1", 4: "qk2", 6: "qk3"}
V_JOBS = {0: "sm", 1: "ctx", 2: "pv0", 3: "outb", 4: "pv1", 6: "wo"}


def _dot(a, b):
    return jnp.dot(a, b, preferred_element_type=F32)


def _dot_nt(a, b):
    return lax.dot_general(a, b, NT, preferred_element_type=F32)


def _kernel(xa_hbm, k_hbm, v_hbm, wq_hbm, wo_hbm, xb_hbm, c_hbm, bwq_hbm, bwuk_hbm, bwuv_hbm, bwo_hbm,
            out_ref,
            xa_v, xb_v, wq_v, wo_v, bwq_v, bwuk_v, bwuv_v, bwo_v, c_v, k_v, v_v,
            qa_s, qb_s, qlat_s, clat_s, s0_s, s1_s, w1_s, w2_s, o_s,
            sem):
    scale = DH ** -0.5

    def cp(src, dst, t0, nt, s):
        sl = pl.ds(t0, nt)
        return pltpu.make_async_copy(src.at[sl], dst.at[sl], sem.at[s])

    class Block:
        def __init__(self, src, dst, d, par, off, end=2048):
            self.src, self.dst, self.par, self.off, self.end = src, dst, par, off, end
            self.dl, self.dh = d[0] // 2, d[1] // 2

        def lo(self, g, j):
            return cp(self.src, self.dst, self.off + self.dl + j * 32 + g * 128, 32, j + g * 4)

        def hi(self, g, j, edge):
            cut = lambda i: 1024 + self.dh + i * 32 + HP[i % 4] // 2
            if not edge:
                spans = [(cut(j - 1), cut(j), g * 128)]
            elif j == 0:
                spans = [(0, self.dl, 0), (cut(31), 2048, 0)]
            else:
                spans = [(1024 + self.dl, cut(1), 0)]
            if self.end < 2048:
                spans = [(a, min(e, self.end - o), o) for a, e, o in spans if a + o < self.end]
            return [cp(self.src, self.dst, self.off + a + o, e - a, HIS + self.par) for a, e, o in spans]

        def hi_start(self, g, j):
            def go(edge):
                def start():
                    for c in self.hi(g, j, edge):
                        c.start(priority=0)
                return start
            if j > 1 or isinstance(g, int):
                go(j <= 1 and g == 0)()
            else:
                pl.when(g == 0)(go(True))
                pl.when(g > 0)(go(False))

        def hi_wait(self):
            for g in range(NG):
                for j in range(4):
                    for c in self.hi(g, j, j <= 1 and g == 0):
                        c.wait()

    late = 2048 - LT
    arrs = [(bwq_hbm, bwq_v, DB, 0), (bwuk_hbm, bwuk_v, DB, 0), (wq_hbm, wq_v, DA, 0)] + \
           [(c_hbm, c_v, DB, b * 2048) for b in range(NB)] + \
           [(bwuv_hbm, bwuv_v, DB, 0), (bwo_hbm, bwo_v, DB, 0), (wo_hbm, wo_v, DA, 0, late)]
    blocks = [Block(a[0], a[1], a[2], i % 2, *a[3:]) for i, a in enumerate(arrs)]

    def kv_piece(kv, h, pair, cuts, j, s):
        src, dst = ((k_hbm, k_v), (v_hbm, v_v))[kv]
        if j == 0:
            b0, nb, a, e = 0, 2, 0, cuts[0]
        elif j == NQ - 1:
            b0, nb, a, e = 0, 2, cuts[3], 256
        else:
            b0, nb, a, e = (j - 1) // 3, 1, cuts[(j - 1) % 3], cuts[(j - 1) % 3 + 1]
        bs, n = pl.ds(2 * pair + b0, nb), (e - a) * 4
        return pltpu.make_async_copy(src.at[bs, h, pl.ds(SK - WIN + a * 4, n), :],
                                     dst.at[h & (NSLOT - 1), bs, pl.ds(a * 4, n), :], sem.at[s])

    def kv_lo(h, kv, j, pos=None):
        par, grp = (h & 1, kv) if pos is None else pos
        return kv_piece(kv, h, 0, CL, j, LS + (par * 2 + grp) * NQ + j)

    def kv_hi(h, kv, j):
        return kv_piece(kv, h, 1, CH, j, HS + (h & 1) * 2 + kv)

    def kv_hi_wait(h, kv):
        for j in range(NQ):
            kv_hi(h, kv, j).wait()

    def v_last(j):
        return kv_piece(1, NH - 1, 1, CL, j, ES + j)

    def wo_last():
        return cp(wo_hbm, wo_v, late, 2048 - late, ES + NQ)

    def run_block(k, jobs, init):
        def group(g, c):
            for j in range(4):
                blocks[k].lo(g, j).wait()
                if j == 0 and k > 0:
                    pl.when(g == 3)(blocks[k - 1].hi_wait)
                blocks[k + 1].lo(g, j).start(priority=1)
                blocks[k].hi_start(g, j)
                for job in jobs.get(j, ()):
                    c = job(g, c)
            return c
        return lax.fori_loop(0, NG, group, init)

    def unit(g, j):
        return (4 * g + j + 2) & 31

    xa_cp = pltpu.make_async_copy(xa_hbm, xa_v, sem.at[XS])
    xb_cp = pltpu.make_async_copy(xb_hbm, xb_v, sem.at[XS + 1])

    for g in range(NG):
        for j in range(4):
            blocks[0].lo(g, j).start(priority=1)
    xa_cp.start()
    xb_cp.start()

    row8 = lax.broadcasted_iota(jnp.int32, (8, 1), 0)

    def pad8(x4):
        return jnp.concatenate([x4.astype(F32), jnp.zeros((4, x4.shape[1]), F32)], axis=0).astype(BF)

    def rows(u, n, k=1):
        return pl.ds(u * n if isinstance(u, int) else pl.multiple_of(u * n, n), n * k)

    def wide(ref, u, k=1):
        t = ref[rows(u, 64, k)].reshape(16 * k, NC, 8, 128)
        return jnp.concatenate([t[:, j].reshape(128 * k, 128) for j in range(NC)], axis=1)

    def deinterleave(src_ref, dst_ref, j):
        def job(g, c):
            u = unit(g, j)
            dst_ref[:, rows(u, 16), :] = jnp.swapaxes(src_ref[rows(u, 64)].reshape(16, NH, DH), 0, 1)
            return c
        return job

    clat_s[...] = jnp.zeros(clat_s.shape, F32)
    run_block(0, {}, 0)
    xa_cp.wait()
    xb_cp.wait()
    xa = pad8(xa_v[...])
    xb = pad8(xb_v[...])
    run_block(1, {j: [deinterleave(bwq_v, w1_s, j)] for j in range(4)}, 0)
    run_block(2, {j: [deinterleave(bwuk_v, w2_s, j)] for j in range(4)}, 0)

    def qb_job(g, c):
        for j in range(4):
            qb_s[j] = _dot(xb, w1_s[4 * g + j])
        return c

    def ql_job(j):
        def job(g, c):
            h = 4 * g + j
            ql = _dot_nt(qb_s[j].astype(BF), w2_s[h]) * scale
            for cb in range(NC):
                qlat_s[cb, rows(h, 8), :] = ql[:, cb * 128:(cb + 1) * 128]
            return c
        return job
    run_block(3, {0: [qb_job], 1: [ql_job(0), ql_job(1)], 2: [ql_job(2), ql_job(3)]}, 0)

    m_prev = None
    for b in range(NB + 1):
        if b < NB:
            ql = jnp.concatenate([qlat_s[cb, pl.ds(b, NH, stride=8), :] for cb in range(NC)],
                                 axis=1).astype(BF)

        def qk_job(j, b=b, ql=ql):
            def job(g, c):
                m_run, l_run, acc = c
                u = unit(g, j)
                s = _dot_nt(ql, wide(c_v, b * 32 + u, 2))
                for k in range(2):
                    (s0_s, s1_s)[b % 2][u + k] = s[:, k * 128:(k + 1) * 128]
                    m_run = jnp.maximum(m_run, s[:, k * 128:(k + 1) * 128])
                return m_run, l_run, acc
            return job

        def pv_job(j, b=b, m_prev=m_prev):
            def job(g, c):
                m_run, l_run, acc = c
                u = 4 * g + j
                ps = [jnp.exp((s0_s, s1_s)[(b - 1) % 2][u + k] - m_prev) for k in range(2)]
                p = jnp.concatenate(ps, axis=1).astype(BF)
                return m_run, l_run + ps[0] + ps[1], acc + _dot(p, wide(c_v, (b - 1) * 32 + u, 2))
            return job

        def qa_job(j):
            def job(g, c):
                for h in (4 * g + j, 4 * g + j + 1):
                    w = jnp.concatenate([wq_v[sl * NH + h] for sl in range(DM // 8)], axis=0)
                    qa_s[h] = _dot(xa, w) * scale
                return c
            return job

        jobs = {j: ([qk_job(j)] if b < NB else []) + [qa_job(j) if b == 0 else pv_job(j)] for j in (0, 2)}
        init = (jnp.full((NH, 128), -jnp.inf, F32), jnp.zeros((NH, 128), F32), jnp.zeros((NH, DM), F32))
        m_run, l_run, acc = run_block(4 + b, jobs, init)
        if b > 0:
            cl = acc / jnp.sum(l_run, axis=1, keepdims=True)
            for cb in range(NC):
                clat_s[cb, pl.ds(b - 1, NH, stride=8), :] = cl[:, cb * 128:(cb + 1) * 128]
        if b < NB:
            m_prev = jnp.broadcast_to(jnp.max(m_run, axis=1, keepdims=True), (NH, 128))

    for t in range(32):
        blocks[9].lo(t // 4, t % 4).wait()
        if t == 12:
            blocks[8].hi_wait()
        kv_lo(t // (2 * NQ), (t // NQ) % 2, t % NQ).start(priority=1)
        blocks[9].hi_start(t // 4, t % 4)
        deinterleave(bwuv_v, w1_s, t % 4)(t // 4, 0)

    X, Y, Z = NH - 3, NH - 2, NH - 1

    def ctx_of(h):
        cl = jnp.concatenate([clat_s[cb, rows(h, 8), :] for cb in range(NC)], axis=1).astype(BF)
        return _dot(cl, w1_s[h]).astype(BF)

    def job(name, h, st):
        slot = h & (NSLOT - 1)
        if name.startswith("qk"):
            b = int(name[2])
            st["s"] = jnp.where(row8 == b, _dot_nt(qa_s[h].astype(BF), k_v[slot, b]), st["s"])
        elif name == "sm":
            p = jnp.exp(st["s"] - jnp.max(st["s"], axis=1, keepdims=True))
            st["p"] = (p * (1.0 / jnp.sum(p, axis=1, keepdims=True))).astype(BF)
        elif name.startswith("pv"):
            for b in (2 * int(name[2]), 2 * int(name[2]) + 1):
                st["o"] = jnp.where(row8 == b, _dot(st["p"], v_v[slot, b]), st["o"])
        elif name == "wo":
            st["acc_a"] = st["acc_a"] + _dot(st["o"].astype(BF), wide(wo_v, h))
        elif name == "ctx":
            st["ctx"] = ctx_of(h + 3)
        elif name == "outb":
            st["acc_b"] = st["acc_b"] + _dot(st["ctx"], wide(bwo_v, h + 3))

    def fresh(**kw):
        return dict(s=jnp.zeros((8, WIN), F32), o=jnp.zeros((8, DH), F32), **kw)

    zero = jnp.zeros((8, DM), F32)
    acc_b = zero
    for t in range(2 * NQ):
        kv_lo(0, t // NQ, t % NQ).wait()
        kv_lo(2, t // NQ, t % NQ).start(priority=1)
        kv_hi(0, t // NQ, t % NQ).start(priority=0)
        if t in (0, 4, 8):
            ctx = ctx_of(t // 4)
        elif t in (2, 6, 10):
            acc_b = acc_b + _dot(ctx, wide(bwo_v, t // 4))
    blocks[9].hi_wait()

    def a_body(h, carry):
        st = fresh(acc_a=carry[0], acc_b=carry[1])
        for kv, jobs in enumerate((K_JOBS, V_JOBS)):
            swap, other = (Z, Y) if kv == 0 else (Y, Z)
            for j in range(NQ):
                kv_lo(h, kv, j).wait()
                if jobs.get(j) in ("qk2", "pv1"):
                    kv_hi_wait(h - 1, kv)
                pl.when(h + 2 != swap)(lambda: kv_lo(h + 2, kv, j).start(priority=1))
                pl.when(h + 2 == swap)(lambda: kv_lo(other, 1 - kv, j, (swap & 1, kv)).start(priority=1))
                kv_hi(h, kv, j).start(priority=0)
                if j in jobs:
                    job(jobs[j], h - 1, st)
        return st["acc_a"], st["acc_b"]

    acc_a, acc_b = lax.fori_loop(1, Y, a_body, (zero, acc_b))
    out_ref[:, DM:] = acc_b[:NB].astype(BF)

    sx, sy, sz = fresh(acc_a=acc_a), fresh(), fresh()
    v_order = [0, NQ - 1] + list(range(1, NQ - 1))
    plan = [((Y, 0, None), {0: (sx, X, "qk0"), 2: (sx, X, "qk1"), 4: (sx, X, "qk2"), 6: (sx, X, "qk3")}),
            ((Z, 0, (Y & 1, 1)), {0: (sx, X, "sm"), 1: (sx, X, "pv0"), 2: (sx, X, "pv1"), 3: (sx, X, "wo"),
                                  4: (sy, Y, "qk0"), 6: (sy, Y, "qk1")}),
            ((Y, 1, (Z & 1, 0)), {0: (sy, Y, "qk2"), 2: (sy, Y, "qk3"), 3: (sy, Y, "sm"),
                                  4: (sz, Z, "qk0"), 6: (sz, Z, "qk1")})]
    for n, ((h, kv, pos), jobs) in enumerate(plan):
        for j in range(NQ):
            kv_lo(h, kv, j, pos).wait()
            if j in jobs and jobs[j][2] in ("qk2", "pv1"):
                kv_hi_wait(jobs[j][1], int(jobs[j][2] == "pv1"))
            if n == 0:
                v_last(v_order[j]).start(priority=1)
            elif n == 1 and j == 0:
                wo_last().start(priority=1)
            kv_hi(h, kv, j).start(priority=0)
            if j in jobs:
                job(jobs[j][2], jobs[j][1], jobs[j][0])
    job("pv0", Y, sy)
    kv_hi_wait(Z, 0)
    job("qk2", Z, sz)
    job("qk3", Z, sz)
    job("sm", Z, sz)
    kv_hi_wait(Y, 1)
    job("pv1", Y, sy)
    sy["acc_a"] = sx["acc_a"]
    job("wo", Y, sy)
    for j in range(NQ):
        kv_lo(Z, 1, j).wait()
    job("pv0", Z, sz)
    o = sz["o"]
    for b, js in ((2, v_order[:5]), (3, v_order[5:])):
        for j in js:
            v_last(j).wait()
        o = jnp.where(row8 == b, _dot(sz["p"], v_v[Z & (NSLOT - 1), b]), o)
    o_s[...] = o.astype(BF)
    wo_last().wait()
    acc_a = sy["acc_a"] + _dot(o_s[...], wide(wo_v, Z))
    out_ref[:, :DM] = acc_a[:NB].astype(BF)


@jax.jit
def pallas_concat_heads__sliding_block_cached__compressed_kv_cla__decode_kernel(
    A_x: jax.Array,
    A_k_cache: jax.Array,
    A_v_cache: jax.Array,
    A_wq: jax.Array,
    A_wo: jax.Array,
    B_x: jax.Array,
    B_c_kv: jax.Array,
    B_w_q: jax.Array,
    B_w_uk: jax.Array,
    B_w_uv: jax.Array,
    B_w_o: jax.Array,
):
    def tiles(w):
        c = w.shape[-1]
        r = w.size // c
        return w.reshape(r // 8, 8, c // 128, 128).transpose(0, 2, 1, 3).reshape(r * c // 1024, 8, 128)

    out = pl.pallas_call(
        _kernel,
        out_shape=jax.ShapeDtypeStruct((NB, 2 * DM), BF),
        in_specs=[pl.BlockSpec(memory_space=pl.ANY)] * 11,
        out_specs=pl.BlockSpec(memory_space=pltpu.VMEM),
        scratch_shapes=[
            pltpu.VMEM((NB, DM), BF), pltpu.VMEM((NB, DM), BF),
        ] + [pltpu.VMEM((2048, 8, 128), BF)] * 6 + [
            pltpu.VMEM((NB * 2048, 8, 128), BF),
            pltpu.VMEM((NSLOT, NB, WIN, DH), BF), pltpu.VMEM((NSLOT, NB, WIN, DH), BF),
            pltpu.VMEM((NH, 8, DH), F32), pltpu.VMEM((4, 8, DH), F32),
            pltpu.VMEM((NC, NH * 8 + 8, 128), F32),
            pltpu.VMEM((NC, NH * 8 + 8, 128), F32),
            pltpu.VMEM((SK // 128, NH, 128), F32), pltpu.VMEM((SK // 128, NH, 128), F32),
            pltpu.VMEM((NH, DM, DH), BF), pltpu.VMEM((NH, DM, DH), BF),
            pltpu.VMEM((8, DH), BF),
            pltpu.SemaphoreType.DMA((NSEM,)),
        ],
        compiler_params=pltpu.CompilerParams(vmem_limit_bytes=100 * 1024 * 1024,
                                             disable_bounds_checks=True,
                                             disable_semaphore_checks=True),
    )(
        A_x.reshape(NB, DM), A_k_cache, A_v_cache, tiles(A_wq), tiles(A_wo),
        B_x.reshape(NB, DM), tiles(B_c_kv), tiles(B_w_q), tiles(B_w_uk), tiles(B_w_uv), tiles(B_w_o),
    )
    return out.reshape(NB, 1, 2 * DM)
```

```python
import jax
import jax.numpy as jnp
from jax import lax
import jax.experimental.pallas as pl
import jax.experimental.pallas.tpu as pltpu

BF = jnp.bfloat16
F32 = jnp.float32
NT = (((1,), (1,)), ((), ()))

NB = 4
NH = 32
DH = 128
DM = 512
SK = 4096
WIN = 1024
NSLOT = 8
NG = 8
NQ = 8
NC = DM // 128
HH = NH // 2
LT = 64
DA = (26, 30)
DB = (30, 34)
HP = (0, -2, 0, -2)
CL = (26, 90, 154, 218)
CH = (30, 92, 158, 220)
HIS, XS, LS, HS, ES, NSEM = 32, 34, 36, 36 + 4 * NQ, 40 + 4 * NQ, 41 + 5 * NQ
K_JOBS = {0: "qk0", 2: "qk1", 4: "qk2", 6: "qk3"}
V_JOBS = {0: "sm", 1: "ctx", 2: "pv0", 3: "outb", 4: "pv1", 6: "wo"}


def _dot(a, b):
    return jnp.dot(a, b, preferred_element_type=F32)


def _dot_nt(a, b):
    return lax.dot_general(a, b, NT, preferred_element_type=F32)


def _kernel(xa_hbm, k_hbm, v_hbm, wq_hbm, wo_hbm, xb_hbm, c_hbm, bwq_hbm, bwuk_hbm, bwuv_hbm, bwo_hbm,
            out_ref,
            xa_v, xb_v, wq_v, wo_v, bwq_v, bwuk_v, bwuv_v, bwo_v, c_v, k_v, v_v,
            qa_s, qb_s, qlat_s, clat_s, s0_s, s1_s, w1_s, w2_s, o_s, acc_s,
            sem):
    scale = DH ** -0.5

    def cp(src, dst, t0, nt, s):
        sl = pl.ds(t0, nt)
        return pltpu.make_async_copy(src.at[sl], dst.at[sl], sem.at[s])

    class Block:
        def __init__(self, src, dst, d, par, off, end=2048):
            self.src, self.dst, self.par, self.off, self.end = src, dst, par, off, end
            self.dl, self.dh = d[0] // 2, d[1] // 2

        def lo(self, g, j):
            return cp(self.src, self.dst, self.off + self.dl + j * 32 + g * 128, 32, j + g * 4)

        def hi(self, g, j, edge):
            cut = lambda i: 1024 + self.dh + i * 32 + HP[i % 4] // 2
            if not edge:
                spans = [(cut(j - 1), cut(j), g * 128)]
            elif j == 0:
                spans = [(0, self.dl, 0), (cut(31), 2048, 0)]
            else:
                spans = [(1024 + self.dl, cut(1), 0)]
            if self.end < 2048:
                spans = [(a, min(e, self.end - o), o) for a, e, o in spans if a + o < self.end]
            return [cp(self.src, self.dst, self.off + a + o, e - a, HIS + self.par) for a, e, o in spans]

        def hi_start(self, g, j):
            def go(edge):
                def start():
                    for c in self.hi(g, j, edge):
                        c.start(priority=0)
                return start
            if j > 1 or isinstance(g, int):
                go(j <= 1 and g == 0)()
            else:
                pl.when(g == 0)(go(True))
                pl.when(g > 0)(go(False))

        def hi_wait(self):
            for g in range(NG):
                for j in range(4):
                    for c in self.hi(g, j, j <= 1 and g == 0):
                        c.wait()

    late = 2048 - LT
    arrs = [(bwq_hbm, bwq_v, DB, 0), (bwuk_hbm, bwuk_v, DB, 0), (wq_hbm, wq_v, DA, 0)] + \
           [(c_hbm, c_v, DB, b * 2048) for b in range(NB)] + \
           [(bwuv_hbm, bwuv_v, DB, 0), (bwo_hbm, bwo_v, DB, 0), (wo_hbm, wo_v, DA, 0, late)]
    blocks = [Block(a[0], a[1], a[2], i % 2, *a[3:]) for i, a in enumerate(arrs)]

    def kv_piece(kv, i, role, cuts, j, s):
        src, dst = ((k_hbm, k_v), (v_hbm, v_v))[kv]
        if j == 0:
            t0, nt, a, e = 0, 2, 0, cuts[0]
        elif j == NQ - 1:
            t0, nt, a, e = 0, 2, cuts[3], 256
        else:
            t0, nt, a, e = (j - 1) % 2, 1, cuts[(j - 1) // 2], cuts[(j - 1) // 2 + 1]
        n = (e - a) * 4
        return pltpu.make_async_copy(
            src.at[2 * (i & 1) + role, pl.ds(t0, nt), i >> 1, pl.ds(SK - WIN + a * 4, n), :],
            dst.at[i & (NSLOT - 1), pl.ds(2 * role + t0, nt), pl.ds(a * 4, n), :], sem.at[s])

    def kv_lo(i, kv, j, pos=None):
        par, grp = (i & 1, kv) if pos is None else pos
        return kv_piece(kv, i, 0, CL, j, LS + (par * 2 + grp) * NQ + j)

    def kv_hi(i, kv, j):
        return kv_piece(kv, i, 1, CH, j, HS + (i & 1) * 2 + kv)

    def kv_hi_wait(i, kv):
        for j in range(NQ):
            kv_hi(i, kv, j).wait()

    def v_last(j):
        return kv_piece(1, NH - 1, 1, CL, j, ES + j)

    def wo_last():
        return cp(wo_hbm, wo_v, late, 2048 - late, ES + NQ)

    def run_block(k, jobs, init):
        def group(g, c):
            for j in range(4):
                blocks[k].lo(g, j).wait()
                if j == 0 and k > 0:
                    pl.when(g == 3)(blocks[k - 1].hi_wait)
                blocks[k + 1].lo(g, j).start(priority=1)
                blocks[k].hi_start(g, j)
                for job in jobs.get(j, ()):
                    c = job(g, c)
            return c
        return lax.fori_loop(0, NG, group, init)

    def unit(g, j):
        return (4 * g + j + 2) & 31

    xa_cp = pltpu.make_async_copy(xa_hbm, xa_v, sem.at[XS])
    xb_cp = pltpu.make_async_copy(xb_hbm, xb_v, sem.at[XS + 1])

    for g in range(NG):
        for j in range(4):
            blocks[0].lo(g, j).start(priority=1)
    xa_cp.start()
    xb_cp.start()

    row8 = lax.broadcasted_iota(jnp.int32, (8, 1), 0)

    def pad8(x4):
        return jnp.concatenate([x4.astype(F32), jnp.zeros((4, x4.shape[1]), F32)], axis=0).astype(BF)

    def rows(u, n, k=1):
        return pl.ds(u * n if isinstance(u, int) else pl.multiple_of(u * n, n), n * k)

    def wide(ref, u, k=1):
        t = ref[rows(u, 64, k)].reshape(16 * k, NC, 8, 128)
        return jnp.concatenate([t[:, j].reshape(128 * k, 128) for j in range(NC)], axis=1)

    def deinterleave(src_ref, dst_ref, j):
        def job(g, c):
            u = unit(g, j)
            dst_ref[:, rows(u, 16), :] = jnp.swapaxes(src_ref[rows(u, 64)].reshape(16, NH, DH), 0, 1)
            return c
        return job

    clat_s[...] = jnp.zeros(clat_s.shape, F32)
    run_block(0, {}, 0)
    xa_cp.wait()
    xb_cp.wait()
    xa = jnp.concatenate([xa_v[...].astype(F32)] * 2, axis=0).astype(BF)
    xb = pad8(xb_v[...])
    run_block(1, {j: [deinterleave(bwq_v, w1_s, j)] for j in range(4)}, 0)
    run_block(2, {j: [deinterleave(bwuk_v, w2_s, j)] for j in range(4)}, 0)

    def qb_job(g, c):
        for j in range(4):
            qb_s[j] = _dot(xb, w1_s[4 * g + j])
        return c

    def ql_job(j):
        def job(g, c):
            h = 4 * g + j
            ql = _dot_nt(qb_s[j].astype(BF), w2_s[h]) * scale
            for cb in range(NC):
                qlat_s[cb, rows(h, 8), :] = ql[:, cb * 128:(cb + 1) * 128]
            return c
        return job
    run_block(3, {0: [qb_job], 1: [ql_job(0), ql_job(1)], 2: [ql_job(2), ql_job(3)]}, 0)

    m_prev = None
    for b in range(NB + 1):
        if b < NB:
            ql = jnp.concatenate([qlat_s[cb, pl.ds(b, NH, stride=8), :] for cb in range(NC)],
                                 axis=1).astype(BF)

        def qk_job(j, b=b, ql=ql):
            def job(g, c):
                m_run, l_run, acc = c
                u = unit(g, j)
                s = _dot_nt(ql, wide(c_v, b * 32 + u, 2))
                for k in range(2):
                    (s0_s, s1_s)[b % 2][u + k] = s[:, k * 128:(k + 1) * 128]
                    m_run = jnp.maximum(m_run, s[:, k * 128:(k + 1) * 128])
                return m_run, l_run, acc
            return job

        def pv_job(j, b=b, m_prev=m_prev):
            def job(g, c):
                m_run, l_run, acc = c
                u = 4 * g + j
                ps = [jnp.exp((s0_s, s1_s)[(b - 1) % 2][u + k] - m_prev) for k in range(2)]
                p = jnp.concatenate(ps, axis=1).astype(BF)
                return m_run, l_run + ps[0] + ps[1], acc + _dot(p, wide(c_v, (b - 1) * 32 + u, 2))
            return job

        def qa_job(j):
            def job(g, c):
                h = 2 * g + j // 2
                q = [_dot(xa, jnp.concatenate([wq_v[sl * NH + hh] for sl in range(DM // 8)], axis=0))
                     for hh in (h, h + HH)]
                qa_s[h] = jnp.where(row8 < NB, q[1], q[0]) * scale
                return c
            return job

        jobs = {j: ([qk_job(j)] if b < NB else []) + [qa_job(j) if b == 0 else pv_job(j)] for j in (0, 2)}
        init = (jnp.full((NH, 128), -jnp.inf, F32), jnp.zeros((NH, 128), F32), jnp.zeros((NH, DM), F32))
        m_run, l_run, acc = run_block(4 + b, jobs, init)
        if b > 0:
            cl = acc / jnp.sum(l_run, axis=1, keepdims=True)
            for cb in range(NC):
                clat_s[cb, pl.ds(b - 1, NH, stride=8), :] = cl[:, cb * 128:(cb + 1) * 128]
        if b < NB:
            m_prev = jnp.broadcast_to(jnp.max(m_run, axis=1, keepdims=True), (NH, 128))

    for t in range(32):
        blocks[9].lo(t // 4, t % 4).wait()
        if t == 12:
            blocks[8].hi_wait()
        kv_lo(t // (2 * NQ), (t // NQ) % 2, t % NQ).start(priority=1)
        blocks[9].hi_start(t // 4, t % 4)
        deinterleave(bwuv_v, w1_s, t % 4)(t // 4, 0)

    X, Y, Z = NH - 3, NH - 2, NH - 1

    def ctx_of(h):
        cl = jnp.concatenate([clat_s[cb, rows(h, 8), :] for cb in range(NC)], axis=1).astype(BF)
        return _dot(cl, w1_s[h]).astype(BF)

    def row_of(i, t):
        return row8 == 2 * (i & 1) + t // 2 + NB * (1 - t % 2)

    def job(name, i, st):
        slot = i & (NSLOT - 1)
        if name.startswith("qk"):
            t = int(name[2])
            st["s"] = jnp.where(row_of(i, t), _dot_nt(qa_s[i >> 1].astype(BF), k_v[slot, t]), st["s"])
        elif name == "sm":
            p = jnp.exp(st["s"] - jnp.max(st["s"], axis=1, keepdims=True))
            st["p"] = (p * (1.0 / jnp.sum(p, axis=1, keepdims=True))).astype(BF)
        elif name.startswith("pv"):
            for t in (2 * int(name[2]), 2 * int(name[2]) + 1):
                st["o"] = jnp.where(row_of(i, t), _dot(st["p"], v_v[slot, t]), st["o"])
        elif name == "wo":
            o = st["o"].astype(BF)
            st["acc_a"] = st["acc_a"] + jnp.where(row8 < NB, _dot(o, wide(wo_v, (i >> 1) + HH)),
                                                  _dot(o, wide(wo_v, i >> 1)))
        elif name == "ctx":
            st["ctx"] = ctx_of(i + 3)
        elif name == "outb":
            st["acc_b"] = st["acc_b"] + _dot(st["ctx"], wide(bwo_v, i + 3))

    def fresh(**kw):
        return dict(s=jnp.zeros((8, WIN), F32), o=jnp.zeros((8, DH), F32), **kw)

    zero = jnp.zeros((8, DM), F32)
    acc_b = zero
    for t in range(2 * NQ):
        kv_lo(0, t // NQ, t % NQ).wait()
        kv_lo(2, t // NQ, t % NQ).start(priority=1)
        kv_hi(0, t // NQ, t % NQ).start(priority=0)
        if t in (0, 4, 8):
            ctx = ctx_of(t // 4)
        elif t in (2, 6, 10):
            acc_b = acc_b + _dot(ctx, wide(bwo_v, t // 4))
    blocks[9].hi_wait()

    def a_body(h, carry):
        st = fresh(acc_a=carry[0], acc_b=carry[1])
        for kv, jobs in enumerate((K_JOBS, V_JOBS)):
            swap, other = (Z, Y) if kv == 0 else (Y, Z)
            for j in range(NQ):
                kv_lo(h, kv, j).wait()
                if jobs.get(j) in ("qk2", "pv1"):
                    kv_hi_wait(h - 1, kv)
                pl.when(h + 2 != swap)(lambda: kv_lo(h + 2, kv, j).start(priority=1))
                pl.when(h + 2 == swap)(lambda: kv_lo(other, 1 - kv, j, (swap & 1, kv)).start(priority=1))
                kv_hi(h, kv, j).start(priority=0)
                if j in jobs:
                    job(jobs[j], h - 1, st)
        return st["acc_a"], st["acc_b"]

    acc_a, acc_b = lax.fori_loop(1, Y, a_body, (zero, acc_b))
    out_ref[:, DM:] = acc_b[:NB].astype(BF)

    sx, sy, sz = fresh(acc_a=acc_a), fresh(), fresh()
    v_order = [0, NQ - 1, 1, 3, 5, 2, 4, 6]
    plan = [((Y, 0, None), {0: (sx, X, "qk0"), 2: (sx, X, "qk1"), 4: (sx, X, "qk2"), 6: (sx, X, "qk3")}),
            ((Z, 0, (Y & 1, 1)), {0: (sx, X, "sm"), 1: (sx, X, "pv0"), 2: (sx, X, "pv1"), 3: (sx, X, "wo"),
                                  4: (sy, Y, "qk0"), 6: (sy, Y, "qk1")}),
            ((Y, 1, (Z & 1, 0)), {0: (sy, Y, "qk2"), 2: (sy, Y, "qk3"), 3: (sy, Y, "sm"),
                                  4: (sz, Z, "qk0"), 6: (sz, Z, "qk1")})]
    for n, ((h, kv, pos), jobs) in enumerate(plan):
        for j in range(NQ):
            kv_lo(h, kv, j, pos).wait()
            if j in jobs and jobs[j][2] in ("qk2", "pv1"):
                kv_hi_wait(jobs[j][1], int(jobs[j][2] == "pv1"))
            if n == 0:
                v_last(v_order[j]).start(priority=1)
            elif n == 1 and j == 0:
                wo_last().start(priority=1)
            kv_hi(h, kv, j).start(priority=0)
            if j in jobs:
                job(jobs[j][2], jobs[j][1], jobs[j][0])
    job("pv0", Y, sy)
    kv_hi_wait(Z, 0)
    job("qk2", Z, sz)
    job("qk3", Z, sz)
    job("sm", Z, sz)
    kv_hi_wait(Y, 1)
    job("pv1", Y, sy)
    sz["o"] = sy["o"]
    for j in range(NQ):
        kv_lo(Z, 1, j).wait()
    job("pv0", Z, sz)
    for j in v_order[:5]:
        v_last(j).wait()
    o = jnp.where(row_of(Z, 2), _dot(sz["p"], v_v[Z & (NSLOT - 1), 2]), sz["o"])
    for j in v_order[5:]:
        v_last(j).wait()
    acc_a = sx["acc_a"] + jnp.where(row8 < NB, 0.0, _dot(o.astype(BF), wide(wo_v, HH - 1)))
    acc_s[...] = acc_a + pltpu.roll(acc_a, NB, 0)
    o = jnp.where(row_of(Z, 3), _dot(sz["p"], v_v[Z & (NSLOT - 1), 3]), o)
    o_s[...] = o.astype(BF)
    wo_last().wait()
    out_ref[:, :DM] = (acc_s[...] + _dot(o_s[...], wide(wo_v, NH - 1)))[:NB].astype(BF)


@jax.jit
def pallas_concat_heads__sliding_block_cached__compressed_kv_cla__decode_kernel(
    A_x: jax.Array,
    A_k_cache: jax.Array,
    A_v_cache: jax.Array,
    A_wq: jax.Array,
    A_wo: jax.Array,
    B_x: jax.Array,
    B_c_kv: jax.Array,
    B_w_q: jax.Array,
    B_w_uk: jax.Array,
    B_w_uv: jax.Array,
    B_w_o: jax.Array,
):
    def tiles(w):
        c = w.shape[-1]
        r = w.size // c
        return w.reshape(r // 8, 8, c // 128, 128).transpose(0, 2, 1, 3).reshape(r * c // 1024, 8, 128)

    out = pl.pallas_call(
        _kernel,
        out_shape=jax.ShapeDtypeStruct((NB, 2 * DM), BF),
        in_specs=[pl.BlockSpec(memory_space=pl.ANY)] * 11,
        out_specs=pl.BlockSpec(memory_space=pltpu.VMEM),
        scratch_shapes=[
            pltpu.VMEM((NB, DM), BF), pltpu.VMEM((NB, DM), BF),
        ] + [pltpu.VMEM((2048, 8, 128), BF)] * 6 + [
            pltpu.VMEM((NB * 2048, 8, 128), BF),
            pltpu.VMEM((NSLOT, NB, WIN, DH), BF), pltpu.VMEM((NSLOT, NB, WIN, DH), BF),
            pltpu.VMEM((HH, 8, DH), F32), pltpu.VMEM((4, 8, DH), F32),
            pltpu.VMEM((NC, NH * 8 + 8, 128), F32),
            pltpu.VMEM((NC, NH * 8 + 8, 128), F32),
            pltpu.VMEM((SK // 128, NH, 128), F32), pltpu.VMEM((SK // 128, NH, 128), F32),
            pltpu.VMEM((NH, DM, DH), BF), pltpu.VMEM((NH, DM, DH), BF),
            pltpu.VMEM((8, DH), BF), pltpu.VMEM((8, DM), F32),
            pltpu.SemaphoreType.DMA((NSEM,)),
        ],
        compiler_params=pltpu.CompilerParams(vmem_limit_bytes=100 * 1024 * 1024,
                                             disable_bounds_checks=True,
                                             disable_semaphore_checks=True),
    )(
        A_x.reshape(NB, DM), A_k_cache.reshape(NB, 2, HH, SK, DH), A_v_cache.reshape(NB, 2, HH, SK, DH),
        tiles(A_wq), tiles(A_wo),
        B_x.reshape(NB, DM), tiles(B_c_kv), tiles(B_w_q), tiles(B_w_uk), tiles(B_w_uv), tiles(B_w_o),
    )
    return out.reshape(NB, 1, 2 * DM)
```

```python
import jax
import jax.numpy as jnp
from jax import lax
import jax.experimental.pallas as pl
import jax.experimental.pallas.tpu as pltpu

BF = jnp.bfloat16
F32 = jnp.float32
NT = (((1,), (1,)), ((), ()))

NB = 4
NH = 32
DH = 128
DM = 512
SK = 4096
WIN = 1024
NSLOT = 8
NG = 8
NQ = 8
NC = DM // 128
HH = NH // 2
LT = 64
DA = (26, 30)
DB = (30, 34)
HP = (0, -2, 0, -2)
CL = (28, 90, 154, 220)
CH = (30, 92, 158, 220)
CE = (26, 90, 154, 218)
HIS, XS, LS, HS, ES, NSEM = 32, 34, 36, 36 + 4 * NQ, 40 + 4 * NQ, 41 + 5 * NQ
K_JOBS = {0: "qk0", 2: "qk1", 4: "qk2", 6: "qk3"}
V_JOBS = {0: "sm", 1: "ctx", 2: "pv0", 3: "outb", 4: "pv1", 6: "wo"}


def _dot(a, b):
    return jnp.dot(a, b, preferred_element_type=F32)


def _dot_nt(a, b):
    return lax.dot_general(a, b, NT, preferred_element_type=F32)


def _kernel(xa_hbm, k_hbm, v_hbm, wq_hbm, wo_hbm, xb_hbm, c_hbm, bwq_hbm, bwuk_hbm, bwuv_hbm, bwo_hbm,
            out_ref,
            xa_v, xb_v, wq_v, wo_v, bwq_v, bwuk_v, bwuv_v, bwo_v, c_v, k_v, v_v,
            qa_s, qb_s, qlat_s, clat_s, s0_s, s1_s, w1_s, w2_s, o_s, acc_s,
            sem):
    scale = DH ** -0.5

    def cp(src, dst, t0, nt, s):
        sl = pl.ds(t0, nt)
        return pltpu.make_async_copy(src.at[sl], dst.at[sl], sem.at[s])

    class Block:
        def __init__(self, src, dst, d, par, off, end=2048):
            self.src, self.dst, self.par, self.off, self.end = src, dst, par, off, end
            self.dl, self.dh = d[0] // 2, d[1] // 2

        def lo(self, g, j):
            return cp(self.src, self.dst, self.off + self.dl + j * 32 + g * 128, 32, j + g * 4)

        def hi(self, g, j, edge):
            cut = lambda i: 1024 + self.dh + i * 32 + HP[i % 4] // 2
            if not edge:
                spans = [(cut(j - 1), cut(j), g * 128)]
            elif j == 0:
                spans = [(0, self.dl, 0), (cut(31), 2048, 0)]
            else:
                spans = [(1024 + self.dl, cut(1), 0)]
            if self.end < 2048:
                spans = [(a, min(e, self.end - o), o) for a, e, o in spans if a + o < self.end]
            return [cp(self.src, self.dst, self.off + a + o, e - a, HIS + self.par) for a, e, o in spans]

        def hi_start(self, g, j):
            def go(edge):
                def start():
                    for c in self.hi(g, j, edge):
                        c.start(priority=0)
                return start
            if j > 1 or isinstance(g, int):
                go(j <= 1 and g == 0)()
            else:
                pl.when(g == 0)(go(True))
                pl.when(g > 0)(go(False))

        def hi_wait(self):
            for g in range(NG):
                for j in range(4):
                    for c in self.hi(g, j, j <= 1 and g == 0):
                        c.wait()

    late = 2048 - LT
    arrs = [(bwq_hbm, bwq_v, DB, 0), (bwuk_hbm, bwuk_v, DB, 0), (wq_hbm, wq_v, DA, 0)] + \
           [(c_hbm, c_v, DB, b * 2048) for b in range(NB)] + \
           [(bwuv_hbm, bwuv_v, DB, 0), (bwo_hbm, bwo_v, DB, 0), (wo_hbm, wo_v, DA, 0, late)]
    blocks = [Block(a[0], a[1], a[2], i % 2, *a[3:]) for i, a in enumerate(arrs)]

    def kv_piece(kv, i, role, cuts, j, s):
        src, dst = ((k_hbm, k_v), (v_hbm, v_v))[kv]
        if j == 0:
            t0, nt, a, e = 0, 2, 0, cuts[0]
        elif j == NQ - 1:
            t0, nt, a, e = 0, 2, cuts[3], 256
        else:
            t0, nt, a, e = (j - 1) % 2, 1, cuts[(j - 1) // 2], cuts[(j - 1) // 2 + 1]
        n = (e - a) * 4
        return pltpu.make_async_copy(
            src.at[(i & 1) + 2 * role, pl.ds(t0, nt), i >> 1, pl.ds(SK - WIN + a * 4, n), :],
            dst.at[i & (NSLOT - 1), pl.ds(2 * role + t0, nt), pl.ds(a * 4, n), :], sem.at[s])

    def kv_lo(i, kv, j, pos=None):
        par, grp = (i & 1, kv) if pos is None else pos
        return kv_piece(kv, i, 0, CL, j, LS + (par * 2 + grp) * NQ + j)

    def kv_hi(i, kv, j):
        return kv_piece(kv, i, 1, CH, j, HS + (i & 1) * 2 + kv)

    def kv_hi_wait(i, kv):
        for j in range(NQ):
            kv_hi(i, kv, j).wait()

    def v_last(j):
        return kv_piece(1, NH - 1, 1, CE, j, ES + j)

    def wo_last():
        return cp(wo_hbm, wo_v, late, 2048 - late, ES + NQ)

    def run_block(k, jobs, init):
        def group(g, c):
            for j in range(4):
                blocks[k].lo(g, j).wait()
                if j == 0 and k > 0:
                    pl.when(g == 3)(blocks[k - 1].hi_wait)
                blocks[k + 1].lo(g, j).start(priority=1)
                blocks[k].hi_start(g, j)
                for job in jobs.get(j, ()):
                    c = job(g, c)
            return c
        return lax.fori_loop(0, NG, group, init)

    def unit(g, j):
        return (4 * g + j + 2) & 31

    xa_cp = pltpu.make_async_copy(xa_hbm, xa_v, sem.at[XS])
    xb_cp = pltpu.make_async_copy(xb_hbm, xb_v, sem.at[XS + 1])

    for g in range(NG):
        for j in range(4):
            blocks[0].lo(g, j).start(priority=1)
    xa_cp.start()
    xb_cp.start()

    row8 = lax.broadcasted_iota(jnp.int32, (8, 1), 0)

    def pad8(x4):
        return jnp.concatenate([x4.astype(F32), jnp.zeros((4, x4.shape[1]), F32)], axis=0).astype(BF)

    def rows(u, n, k=1):
        return pl.ds(u * n if isinstance(u, int) else pl.multiple_of(u * n, n), n * k)

    def wide(ref, u, k=1):
        t = ref[rows(u, 64, k)].reshape(16 * k, NC, 8, 128)
        return jnp.concatenate([t[:, j].reshape(128 * k, 128) for j in range(NC)], axis=1)

    def deinterleave(src_ref, dst_ref, j):
        def job(g, c):
            u = unit(g, j)
            dst_ref[:, rows(u, 16), :] = jnp.swapaxes(src_ref[rows(u, 64)].reshape(16, NH, DH), 0, 1)
            return c
        return job

    clat_s[...] = jnp.zeros(clat_s.shape, F32)
    run_block(0, {}, 0)
    xa_cp.wait()
    xb_cp.wait()
    xa = jnp.concatenate([xa_v[...].astype(F32)] * 2, axis=0).astype(BF)
    xb = pad8(xb_v[...])
    run_block(1, {j: [deinterleave(bwq_v, w1_s, j)] for j in range(4)}, 0)
    run_block(2, {j: [deinterleave(bwuk_v, w2_s, j)] for j in range(4)}, 0)

    def qb_job(g, c):
        for j in range(4):
            qb_s[j] = _dot(xb, w1_s[4 * g + j])
        return c

    def ql_job(j):
        def job(g, c):
            h = 4 * g + j
            ql = _dot_nt(qb_s[j].astype(BF), w2_s[h]) * scale
            for cb in range(NC):
                qlat_s[cb, rows(h, 8), :] = ql[:, cb * 128:(cb + 1) * 128]
            return c
        return job
    run_block(3, {0: [qb_job], 1: [ql_job(0), ql_job(1)], 2: [ql_job(2), ql_job(3)]}, 0)

    m_prev = None
    for b in range(NB + 1):
        if b < NB:
            ql = jnp.concatenate([qlat_s[cb, pl.ds(b, NH, stride=8), :] for cb in range(NC)],
                                 axis=1).astype(BF)

        def qk_job(j, b=b, ql=ql):
            def job(g, c):
                m_run, l_run, acc = c
                u = unit(g, j)
                s = _dot_nt(ql, wide(c_v, b * 32 + u, 2))
                for k in range(2):
                    (s0_s, s1_s)[b % 2][u + k] = s[:, k * 128:(k + 1) * 128]
                    m_run = jnp.maximum(m_run, s[:, k * 128:(k + 1) * 128])
                return m_run, l_run, acc
            return job

        def pv_job(j, b=b, m_prev=m_prev):
            def job(g, c):
                m_run, l_run, acc = c
                u = 4 * g + j
                ps = [jnp.exp((s0_s, s1_s)[(b - 1) % 2][u + k] - m_prev) for k in range(2)]
                p = jnp.concatenate(ps, axis=1).astype(BF)
                return m_run, l_run + ps[0] + ps[1], acc + _dot(p, wide(c_v, (b - 1) * 32 + u, 2))
            return job

        def qa_job(j):
            def job(g, c):
                h = 2 * g + j // 2
                q = [_dot(xa, jnp.concatenate([wq_v[sl * NH + hh] for sl in range(DM // 8)], axis=0))
                     for hh in (h, h + HH)]
                qa_s[h] = jnp.where(row8 < NB, q[1], q[0]) * scale
                return c
            return job

        jobs = {j: ([qk_job(j)] if b < NB else []) + [qa_job(j) if b == 0 else pv_job(j)] for j in (0, 2)}
        init = (jnp.full((NH, 128), -jnp.inf, F32), jnp.zeros((NH, 128), F32), jnp.zeros((NH, DM), F32))
        m_run, l_run, acc = run_block(4 + b, jobs, init)
        if b > 0:
            cl = acc / jnp.sum(l_run, axis=1, keepdims=True)
            for cb in range(NC):
                clat_s[cb, pl.ds(b - 1, NH, stride=8), :] = cl[:, cb * 128:(cb + 1) * 128]
        if b < NB:
            m_prev = jnp.broadcast_to(jnp.max(m_run, axis=1, keepdims=True), (NH, 128))

    for t in range(32):
        blocks[9].lo(t // 4, t % 4).wait()
        if t == 12:
            blocks[8].hi_wait()
        kv_lo(t // (2 * NQ), (t // NQ) % 2, t % NQ).start(priority=1)
        blocks[9].hi_start(t // 4, t % 4)
        deinterleave(bwuv_v, w1_s, t % 4)(t // 4, 0)

    X, Y, Z = NH - 3, NH - 2, NH - 1

    def ctx_of(h):
        cl = jnp.concatenate([clat_s[cb, rows(h, 8), :] for cb in range(NC)], axis=1).astype(BF)
        return _dot(cl, w1_s[h]).astype(BF)

    def row_of(i, t):
        return row8 == (i & 1) + 2 * (t // 2) + NB * (1 - t % 2)

    def job(name, i, st):
        slot = i & (NSLOT - 1)
        if name.startswith("qk"):
            t = int(name[2])
            st["s"] = jnp.where(row_of(i, t), _dot_nt(qa_s[i >> 1].astype(BF), k_v[slot, t]), st["s"])
        elif name == "sm":
            p = jnp.exp(st["s"] - jnp.max(st["s"], axis=1, keepdims=True))
            st["p"] = (p * (1.0 / jnp.sum(p, axis=1, keepdims=True))).astype(BF)
        elif name.startswith("pv"):
            for t in (2 * int(name[2]), 2 * int(name[2]) + 1):
                st["o"] = jnp.where(row_of(i, t), _dot(st["p"], v_v[slot, t]), st["o"])
        elif name == "wo":
            o = st["o"].astype(BF)
            st["acc_a"] = st["acc_a"] + jnp.where(row8 < NB, _dot(o, wide(wo_v, (i >> 1) + HH)),
                                                  _dot(o, wide(wo_v, i >> 1)))
        elif name == "ctx":
            st["ctx"] = ctx_of(i + 3)
        elif name == "outb":
            st["acc_b"] = st["acc_b"] + _dot(st["ctx"], wide(bwo_v, i + 3))

    def fresh(**kw):
        return dict(s=jnp.zeros((8, WIN), F32), o=jnp.zeros((8, DH), F32), **kw)

    zero = jnp.zeros((8, DM), F32)
    acc_b = zero
    for t in range(2 * NQ):
        kv_lo(0, t // NQ, t % NQ).wait()
        kv_lo(2, t // NQ, t % NQ).start(priority=1)
        kv_hi(0, t // NQ, t % NQ).start(priority=0)
        if t in (0, 4, 8):
            ctx = ctx_of(t // 4)
        elif t in (2, 6, 10):
            acc_b = acc_b + _dot(ctx, wide(bwo_v, t // 4))
    blocks[9].hi_wait()

    def a_body(i, carry):
        st = fresh(acc_a=carry[0], acc_b=carry[1])
        for kv, jobs in enumerate((K_JOBS, V_JOBS)):
            swap, other = (Z, Y) if kv == 0 else (Y, Z)
            for j in range(NQ):
                kv_lo(i, kv, j).wait()
                if jobs.get(j) in ("qk2", "pv1"):
                    kv_hi_wait(i - 1, kv)
                pl.when(i + 2 != swap)(lambda: kv_lo(i + 2, kv, j).start(priority=1))
                pl.when(i + 2 == swap)(lambda: kv_lo(other, 1 - kv, j, (swap & 1, kv)).start(priority=1))
                kv_hi(i, kv, j).start(priority=0)
                if j in jobs:
                    job(jobs[j], i - 1, st)
        return st["acc_a"], st["acc_b"]

    acc_a, acc_b = lax.fori_loop(1, Y, a_body, (zero, acc_b))
    out_ref[:, DM:] = acc_b[:NB].astype(BF)

    sx, sy, sz = fresh(acc_a=acc_a), fresh(), fresh()
    v_order = [0, NQ - 1, 1, 3, 5, 2, 4, 6]
    plan = [((Y, 0, None), {0: (sx, X, "qk0"), 2: (sx, X, "qk1"), 4: (sx, X, "qk2"), 6: (sx, X, "qk3")}),
            ((Z, 0, (Y & 1, 1)), {0: (sx, X, "sm"), 1: (sx, X, "pv0"), 2: (sx, X, "pv1"), 3: (sx, X, "wo"),
                                  4: (sy, Y, "qk0"), 6: (sy, Y, "qk1")}),
            ((Y, 1, (Z & 1, 0)), {0: (sy, Y, "qk2"), 2: (sy, Y, "qk3"), 3: (sy, Y, "sm"),
                                  4: (sz, Z, "qk0"), 6: (sz, Z, "qk1")})]
    for n, ((i, kv, pos), jobs) in enumerate(plan):
        for j in range(NQ):
            kv_lo(i, kv, j, pos).wait()
            if j in jobs and jobs[j][2] in ("qk2", "pv1"):
                kv_hi_wait(jobs[j][1], int(jobs[j][2] == "pv1"))
            if n == 0:
                v_last(v_order[j]).start(priority=1)
            elif n == 1 and j == 0:
                wo_last().start(priority=1)
            kv_hi(i, kv, j).start(priority=0)
            if j in jobs:
                job(jobs[j][2], jobs[j][1], jobs[j][0])
    job("pv0", Y, sy)
    kv_hi_wait(Z, 0)
    job("qk2", Z, sz)
    job("qk3", Z, sz)
    job("sm", Z, sz)
    kv_hi_wait(Y, 1)
    job("pv1", Y, sy)
    sz["o"] = sy["o"]
    for j in range(NQ):
        kv_lo(Z, 1, j).wait()
    job("pv0", Z, sz)
    for j in v_order[:5]:
        v_last(j).wait()
    o = jnp.where(row_of(Z, 2), _dot(sz["p"], v_v[Z & (NSLOT - 1), 2]), sz["o"])
    for j in v_order[5:]:
        v_last(j).wait()
    acc_a = sx["acc_a"] + jnp.where(row8 < NB, 0.0, _dot(o.astype(BF), wide(wo_v, HH - 1)))
    acc_s[...] = acc_a[:NB] + acc_a[NB:]
    o = jnp.where(row_of(Z, 3), _dot(sz["p"], v_v[Z & (NSLOT - 1), 3]), o)
    o_s[...] = o.astype(BF)
    wo_last().wait()
    out_ref[:, :DM] = (acc_s[...] + _dot(o_s[...], wide(wo_v, NH - 1))[:NB]).astype(BF)


@jax.jit
def pallas_concat_heads__sliding_block_cached__compressed_kv_cla__decode_kernel(
    A_x: jax.Array,
    A_k_cache: jax.Array,
    A_v_cache: jax.Array,
    A_wq: jax.Array,
    A_wo: jax.Array,
    B_x: jax.Array,
    B_c_kv: jax.Array,
    B_w_q: jax.Array,
    B_w_uk: jax.Array,
    B_w_uv: jax.Array,
    B_w_o: jax.Array,
):
    def tiles(w):
        c = w.shape[-1]
        r = w.size // c
        return w.reshape(r // 8, 8, c // 128, 128).transpose(0, 2, 1, 3).reshape(r * c // 1024, 8, 128)

    out = pl.pallas_call(
        _kernel,
        out_shape=jax.ShapeDtypeStruct((NB, 2 * DM), BF),
        in_specs=[pl.BlockSpec(memory_space=pl.ANY)] * 11,
        out_specs=pl.BlockSpec(memory_space=pltpu.VMEM),
        scratch_shapes=[
            pltpu.VMEM((NB, DM), BF), pltpu.VMEM((NB, DM), BF),
        ] + [pltpu.VMEM((2048, 8, 128), BF)] * 6 + [
            pltpu.VMEM((NB * 2048, 8, 128), BF),
            pltpu.VMEM((NSLOT, NB, WIN, DH), BF), pltpu.VMEM((NSLOT, NB, WIN, DH), BF),
            pltpu.VMEM((HH, 8, DH), F32), pltpu.VMEM((4, 8, DH), F32),
            pltpu.VMEM((NC, NH * 8 + 8, 128), F32),
            pltpu.VMEM((NC, NH * 8 + 8, 128), F32),
            pltpu.VMEM((SK // 128, NH, 128), F32), pltpu.VMEM((SK // 128, NH, 128), F32),
            pltpu.VMEM((NH, DM, DH), BF), pltpu.VMEM((NH, DM, DH), BF),
            pltpu.VMEM((8, DH), BF), pltpu.VMEM((NB, DM), F32),
            pltpu.SemaphoreType.DMA((NSEM,)),
        ],
        compiler_params=pltpu.CompilerParams(vmem_limit_bytes=100 * 1024 * 1024,
                                             disable_bounds_checks=True,
                                             disable_semaphore_checks=True),
    )(
        A_x.reshape(NB, DM), A_k_cache.reshape(NB, 2, HH, SK, DH), A_v_cache.reshape(NB, 2, HH, SK, DH),
        tiles(A_wq), tiles(A_wo),
        B_x.reshape(NB, DM), tiles(B_c_kv), tiles(B_w_q), tiles(B_w_uk), tiles(B_w_uv), tiles(B_w_o),
    )
    return out.reshape(NB, 1, 2 * DM)
```

```python
import jax
import jax.numpy as jnp
from jax import lax
import jax.experimental.pallas as pl
import jax.experimental.pallas.tpu as pltpu

BF = jnp.bfloat16
F32 = jnp.float32
NT = (((1,), (1,)), ((), ()))

NB = 4
NH = 32
DH = 128
DM = 512
SK = 4096
WIN = 1024
NSLOT = 8
NG = 8
NQ = 8
NC = DM // 128
HH = NH // 2
LT = 64
DA = (24, 28)
DB = (28, 32)
LP = (0, -2, 0, 2)
HP = (0, 2, 2, 0)
CL = ((28, 92, 154, 222), (28, 92, 154, 222))
CH = ((30, 96, 158, 222), (30, 92, 158, 222))
CE = ((26, 90, 154, 218), (26, 90, 154, 218))
HIS, XS, LS, HS, ES, NSEM = 32, 34, 36, 36 + 4 * NQ, 40 + 4 * NQ, 41 + 5 * NQ
K_JOBS = {0: "qk0", 2: "qk1", 4: "qk2", 6: "qk3"}
V_JOBS = {0: "sm", 1: "ctx", 2: "pv0", 3: "outb", 4: "pv1", 6: "wo"}


def _dot(a, b):
    return jnp.dot(a, b, preferred_element_type=F32)


def _dot_nt(a, b):
    return lax.dot_general(a, b, NT, preferred_element_type=F32)


def _kernel(xa_hbm, k_hbm, v_hbm, wq_hbm, wo_hbm, xb_hbm, c_hbm, bwq_hbm, bwuk_hbm, bwuv_hbm, bwo_hbm,
            out_ref,
            xa_v, xb_v, wq_v, wo_v, bwq_v, bwuk_v, bwuv_v, bwo_v, c_v, k_v, v_v,
            qa_s, qb_s, qlat_s, clat_s, s0_s, s1_s, w1_s, w2_s, o_s, acc_s,
            sem):
    scale = DH ** -0.5

    def cp(src, dst, t0, nt, s):
        sl = pl.ds(t0, nt)
        return pltpu.make_async_copy(src.at[sl], dst.at[sl], sem.at[s])

    class Block:
        def __init__(self, src, dst, d, par, off, end=2048):
            self.src, self.dst, self.par, self.off, self.end = src, dst, par, off, end
            self.dl, self.dh = d[0] // 2, d[1] // 2

        def lo(self, g, j):
            return cp(self.src, self.dst, self.off + self.dl + j * 32 + LP[j] // 2 + g * 128,
                      32 + LP[(j + 1) % 4] // 2 - LP[j] // 2, j + g * 4)

        def hi(self, g, j, edge):
            cut = lambda i: 1024 + self.dh + i * 32 + HP[i % 4] // 2
            if not edge:
                spans = [(cut(j - 1), cut(j), g * 128)]
            elif j == 0:
                spans = [(0, self.dl, 0), (cut(31), 2048, 0)]
            else:
                spans = [(1024 + self.dl, cut(1), 0)]
            if self.end < 2048:
                spans = [(a, min(e, self.end - o), o) for a, e, o in spans if a + o < self.end]
            return [cp(self.src, self.dst, self.off + a + o, e - a, HIS + self.par) for a, e, o in spans]

        def hi_start(self, g, j):
            def go(edge):
                def start():
                    for c in self.hi(g, j, edge):
                        c.start(priority=0)
                return start
            if j > 1 or isinstance(g, int):
                go(j <= 1 and g == 0)()
            else:
                pl.when(g == 0)(go(True))
                pl.when(g > 0)(go(False))

        def hi_wait(self):
            for g in range(NG):
                for j in range(4):
                    for c in self.hi(g, j, j <= 1 and g == 0):
                        c.wait()

    late = 2048 - LT
    arrs = [(bwq_hbm, bwq_v, DB, 0), (bwuk_hbm, bwuk_v, DB, 0), (wq_hbm, wq_v, DA, 0)] + \
           [(c_hbm, c_v, DB, b * 2048) for b in range(NB)] + \
           [(bwuv_hbm, bwuv_v, DB, 0), (bwo_hbm, bwo_v, DB, 0), (wo_hbm, wo_v, DA, 0, late)]
    blocks = [Block(a[0], a[1], a[2], i % 2, *a[3:]) for i, a in enumerate(arrs)]

    def kv_piece(kv, i, role, cuts, j, s):
        src, dst = ((k_hbm, k_v), (v_hbm, v_v))[kv]
        if j == 0:
            t0, nt, a, e = 0, 2, 0, cuts[0][0]
        elif j == NQ - 1:
            t0, nt, a, e = 0, 2, cuts[0][3], 256
        else:
            t0, nt = (j - 1) % 2, 1
            a, e = cuts[t0][(j - 1) // 2], cuts[t0][(j - 1) // 2 + 1]
        n = (e - a) * 4
        return pltpu.make_async_copy(
            src.at[(i & 1) + 2 * role, pl.ds(t0, nt), i >> 1, pl.ds(SK - WIN + a * 4, n), :],
            dst.at[i & (NSLOT - 1), pl.ds(2 * role + t0, nt), pl.ds(a * 4, n), :], sem.at[s])

    def kv_lo(i, kv, j, pos=None):
        par, grp = (i & 1, kv) if pos is None else pos
        return kv_piece(kv, i, 0, CL, j, LS + (par * 2 + grp) * NQ + j)

    def kv_hi(i, kv, j):
        return kv_piece(kv, i, 1, CH, j, HS + (i & 1) * 2 + kv)

    def kv_hi_wait(i, kv):
        for j in range(NQ):
            kv_hi(i, kv, j).wait()

    def v_last(j):
        return kv_piece(1, NH - 1, 1, CE, j, ES + j)

    def wo_last():
        return cp(wo_hbm, wo_v, late, 2048 - late, ES + NQ)

    def run_block(k, jobs, init):
        def group(g, c):
            for j in range(4):
                blocks[k].lo(g, j).wait()
                if j == 0 and k > 0:
                    pl.when(g == 3)(blocks[k - 1].hi_wait)
                blocks[k + 1].lo(g, j).start(priority=1)
                blocks[k].hi_start(g, j)
                for job in jobs.get(j, ()):
                    c = job(g, c)
            return c
        return lax.fori_loop(0, NG, group, init)

    def unit(g, j):
        return (4 * g + j + 2) & 31

    xa_cp = pltpu.make_async_copy(xa_hbm, xa_v, sem.at[XS])
    xb_cp = pltpu.make_async_copy(xb_hbm, xb_v, sem.at[XS + 1])

    for g in range(NG):
        for j in range(4):
            blocks[0].lo(g, j).start(priority=1)
    xa_cp.start()
    xb_cp.start()

    row8 = lax.broadcasted_iota(jnp.int32, (8, 1), 0)

    def pad8(x4):
        return jnp.concatenate([x4.astype(F32), jnp.zeros((4, x4.shape[1]), F32)], axis=0).astype(BF)

    def rows(u, n, k=1):
        return pl.ds(u * n if isinstance(u, int) else pl.multiple_of(u * n, n), n * k)

    def wide(ref, u, k=1):
        t = ref[rows(u, 64, k)].reshape(16 * k, NC, 8, 128)
        return jnp.concatenate([t[:, j].reshape(128 * k, 128) for j in range(NC)], axis=1)

    def deinterleave(src_ref, dst_ref, j):
        def job(g, c):
            u = unit(g, j)
            dst_ref[:, rows(u, 16), :] = jnp.swapaxes(src_ref[rows(u, 64)].reshape(16, NH, DH), 0, 1)
            return c
        return job

    clat_s[...] = jnp.zeros(clat_s.shape, F32)
    run_block(0, {}, 0)
    xa_cp.wait()
    xb_cp.wait()
    xa = jnp.concatenate([xa_v[...].astype(F32)] * 2, axis=0).astype(BF)
    xb = pad8(xb_v[...])
    run_block(1, {j: [deinterleave(bwq_v, w1_s, j)] for j in range(4)}, 0)
    run_block(2, {j: [deinterleave(bwuk_v, w2_s, j)] for j in range(4)}, 0)

    def qb_job(g, c):
        for j in range(4):
            qb_s[j] = _dot(xb, w1_s[4 * g + j])
        return c

    def ql_job(j):
        def job(g, c):
            h = 4 * g + j
            ql = _dot_nt(qb_s[j].astype(BF), w2_s[h]) * scale
            for cb in range(NC):
                qlat_s[cb, rows(h, 8), :] = ql[:, cb * 128:(cb + 1) * 128]
            return c
        return job
    run_block(3, {0: [qb_job], 1: [ql_job(0), ql_job(1)], 2: [ql_job(2), ql_job(3)]}, 0)

    m_prev = None
    for b in range(NB + 1):
        if b < NB:
            ql = jnp.concatenate([qlat_s[cb, pl.ds(b, NH, stride=8), :] for cb in range(NC)],
                                 axis=1).astype(BF)

        def qk_job(j, b=b, ql=ql):
            def job(g, c):
                m_run, l_run, acc = c
                u = unit(g, j)
                s = _dot_nt(ql, wide(c_v, b * 32 + u, 2))
                for k in range(2):
                    (s0_s, s1_s)[b % 2][u + k] = s[:, k * 128:(k + 1) * 128]
                    m_run = jnp.maximum(m_run, s[:, k * 128:(k + 1) * 128])
                return m_run, l_run, acc
            return job

        def pv_job(j, b=b, m_prev=m_prev):
            def job(g, c):
                m_run, l_run, acc = c
                u = 4 * g + j
                ps = [jnp.exp((s0_s, s1_s)[(b - 1) % 2][u + k] - m_prev) for k in range(2)]
                p = jnp.concatenate(ps, axis=1).astype(BF)
                return m_run, l_run + ps[0] + ps[1], acc + _dot(p, wide(c_v, (b - 1) * 32 + u, 2))
            return job

        def qa_job(j):
            def job(g, c):
                h = 2 * g + j // 2
                q = [_dot(xa, jnp.concatenate([wq_v[sl * NH + hh] for sl in range(DM // 8)], axis=0))
                     for hh in (h, h + HH)]
                qa_s[h] = jnp.where(row8 < NB, q[1], q[0]) * scale
                return c
            return job

        jobs = {j: ([qk_job(j)] if b < NB else []) + [qa_job(j) if b == 0 else pv_job(j)] for j in (0, 2)}
        init = (jnp.full((NH, 128), -jnp.inf, F32), jnp.zeros((NH, 128), F32), jnp.zeros((NH, DM), F32))
        m_run, l_run, acc = run_block(4 + b, jobs, init)
        if b > 0:
            cl = acc / jnp.sum(l_run, axis=1, keepdims=True)
            for cb in range(NC):
                clat_s[cb, pl.ds(b - 1, NH, stride=8), :] = cl[:, cb * 128:(cb + 1) * 128]
        if b < NB:
            m_prev = jnp.broadcast_to(jnp.max(m_run, axis=1, keepdims=True), (NH, 128))

    for t in range(32):
        blocks[9].lo(t // 4, t % 4).wait()
        if t == 12:
            blocks[8].hi_wait()
        kv_lo(t // (2 * NQ), (t // NQ) % 2, t % NQ).start(priority=1)
        blocks[9].hi_start(t // 4, t % 4)
        deinterleave(bwuv_v, w1_s, t % 4)(t // 4, 0)

    X, Y, Z = NH - 3, NH - 2, NH - 1

    def ctx_of(h):
        cl = jnp.concatenate([clat_s[cb, rows(h, 8), :] for cb in range(NC)], axis=1).astype(BF)
        return _dot(cl, w1_s[h]).astype(BF)

    def row_of(i, t):
        return row8 == (i & 1) + 2 * (t // 2) + NB * (1 - t % 2)

    def job(name, i, st):
        slot = i & (NSLOT - 1)
        if name.startswith("qk"):
            t = int(name[2])
            st["s"] = jnp.where(row_of(i, t), _dot_nt(qa_s[i >> 1].astype(BF), k_v[slot, t]), st["s"])
        elif name == "sm":
            p = jnp.exp(st["s"] - jnp.max(st["s"], axis=1, keepdims=True))
            st["p"] = (p * (1.0 / jnp.sum(p, axis=1, keepdims=True))).astype(BF)
        elif name.startswith("pv"):
            for t in (2 * int(name[2]), 2 * int(name[2]) + 1):
                st["o"] = jnp.where(row_of(i, t), _dot(st["p"], v_v[slot, t]), st["o"])
        elif name == "wo":
            o = st["o"].astype(BF)
            st["acc_a"] = st["acc_a"] + jnp.where(row8 < NB, _dot(o, wide(wo_v, (i >> 1) + HH)),
                                                  _dot(o, wide(wo_v, i >> 1)))
        elif name == "ctx":
            st["ctx"] = ctx_of(i + 3)
        elif name == "outb":
            st["acc_b"] = st["acc_b"] + _dot(st["ctx"], wide(bwo_v, i + 3))

    def fresh(**kw):
        return dict(s=jnp.zeros((8, WIN), F32), o=jnp.zeros((8, DH), F32), **kw)

    zero = jnp.zeros((8, DM), F32)
    acc_b = zero
    for t in range(2 * NQ):
        kv_lo(0, t // NQ, t % NQ).wait()
        kv_lo(2, t // NQ, t % NQ).start(priority=1)
        kv_hi(0, t // NQ, t % NQ).start(priority=0)
        if t in (0, 4, 8):
            ctx = ctx_of(t // 4)
        elif t in (2, 6, 10):
            acc_b = acc_b + _dot(ctx, wide(bwo_v, t // 4))
    blocks[9].hi_wait()

    def a_body(i, carry):
        st = fresh(acc_a=carry[0], acc_b=carry[1])
        for kv, jobs in enumerate((K_JOBS, V_JOBS)):
            swap, other = (Z, Y) if kv == 0 else (Y, Z)
            for j in range(NQ):
                kv_lo(i, kv, j).wait()
                if jobs.get(j) in ("qk2", "pv1"):
                    kv_hi_wait(i - 1, kv)
                pl.when(i + 2 != swap)(lambda: kv_lo(i + 2, kv, j).start(priority=1))
                pl.when(i + 2 == swap)(lambda: kv_lo(other, 1 - kv, j, (swap & 1, kv)).start(priority=1))
                kv_hi(i, kv, j).start(priority=0)
                if j in jobs:
                    job(jobs[j], i - 1, st)
        return st["acc_a"], st["acc_b"]

    acc_a, acc_b = lax.fori_loop(1, Y, a_body, (zero, acc_b))
    out_ref[:, DM:] = acc_b[:NB].astype(BF)

    sx, sy, sz = fresh(acc_a=acc_a), fresh(), fresh()
    v_order = [0, NQ - 1, 1, 3, 5, 2, 4, 6]
    plan = [((Y, 0, None), {0: (sx, X, "qk0"), 2: (sx, X, "qk1"), 4: (sx, X, "qk2"), 6: (sx, X, "qk3")}),
            ((Z, 0, (Y & 1, 1)), {0: (sx, X, "sm"), 1: (sx, X, "pv0"), 2: (sx, X, "pv1"), 3: (sx, X, "wo"),
                                  4: (sy, Y, "qk0"), 6: (sy, Y, "qk1")}),
            ((Y, 1, (Z & 1, 0)), {0: (sy, Y, "qk2"), 2: (sy, Y, "qk3"), 3: (sy, Y, "sm"),
                                  4: (sz, Z, "qk0"), 6: (sz, Z, "qk1")})]
    for n, ((i, kv, pos), jobs) in enumerate(plan):
        for j in range(NQ):
            kv_lo(i, kv, j, pos).wait()
            if j in jobs and jobs[j][2] in ("qk2", "pv1"):
                kv_hi_wait(jobs[j][1], int(jobs[j][2] == "pv1"))
            if n == 0:
                v_last(v_order[j]).start(priority=1)
            elif n == 1 and j == 0:
                wo_last().start(priority=1)
            kv_hi(i, kv, j).start(priority=0)
            if j in jobs:
                job(jobs[j][2], jobs[j][1], jobs[j][0])
    job("pv0", Y, sy)
    kv_hi_wait(Z, 0)
    job("qk2", Z, sz)
    job("qk3", Z, sz)
    job("sm", Z, sz)
    kv_hi_wait(Y, 1)
    job("pv1", Y, sy)
    sz["o"] = sy["o"]
    for j in range(NQ):
        kv_lo(Z, 1, j).wait()
    job("pv0", Z, sz)
    for j in v_order[:5]:
        v_last(j).wait()
    o = jnp.where(row_of(Z, 2), _dot(sz["p"], v_v[Z & (NSLOT - 1), 2]), sz["o"])
    for j in v_order[5:]:
        v_last(j).wait()
    acc_a = sx["acc_a"] + jnp.where(row8 < NB, 0.0, _dot(o.astype(BF), wide(wo_v, HH - 1)))
    acc_s[...] = acc_a[:NB] + acc_a[NB:]
    o = jnp.where(row_of(Z, 3), _dot(sz["p"], v_v[Z & (NSLOT - 1), 3]), o)
    o_s[...] = o.astype(BF)
    wo_last().wait()
    out_ref[:, :DM] = (acc_s[...] + _dot(o_s[...], wide(wo_v, NH - 1))[:NB]).astype(BF)


@jax.jit
def pallas_concat_heads__sliding_block_cached__compressed_kv_cla__decode_kernel(
    A_x: jax.Array,
    A_k_cache: jax.Array,
    A_v_cache: jax.Array,
    A_wq: jax.Array,
    A_wo: jax.Array,
    B_x: jax.Array,
    B_c_kv: jax.Array,
    B_w_q: jax.Array,
    B_w_uk: jax.Array,
    B_w_uv: jax.Array,
    B_w_o: jax.Array,
):
    def tiles(w):
        c = w.shape[-1]
        r = w.size // c
        return w.reshape(r // 8, 8, c // 128, 128).transpose(0, 2, 1, 3).reshape(r * c // 1024, 8, 128)

    out = pl.pallas_call(
        _kernel,
        out_shape=jax.ShapeDtypeStruct((NB, 2 * DM), BF),
        in_specs=[pl.BlockSpec(memory_space=pl.ANY)] * 11,
        out_specs=pl.BlockSpec(memory_space=pltpu.VMEM),
        scratch_shapes=[
            pltpu.VMEM((NB, DM), BF), pltpu.VMEM((NB, DM), BF),
        ] + [pltpu.VMEM((2048, 8, 128), BF)] * 6 + [
            pltpu.VMEM((NB * 2048, 8, 128), BF),
            pltpu.VMEM((NSLOT, NB, WIN, DH), BF), pltpu.VMEM((NSLOT, NB, WIN, DH), BF),
            pltpu.VMEM((HH, 8, DH), F32), pltpu.VMEM((4, 8, DH), F32),
            pltpu.VMEM((NC, NH * 8 + 8, 128), F32),
            pltpu.VMEM((NC, NH * 8 + 8, 128), F32),
            pltpu.VMEM((SK // 128, NH, 128), F32), pltpu.VMEM((SK // 128, NH, 128), F32),
            pltpu.VMEM((NH, DM, DH), BF), pltpu.VMEM((NH, DM, DH), BF),
            pltpu.VMEM((8, DH), BF), pltpu.VMEM((NB, DM), F32),
            pltpu.SemaphoreType.DMA((NSEM,)),
        ],
        compiler_params=pltpu.CompilerParams(vmem_limit_bytes=100 * 1024 * 1024,
                                             disable_bounds_checks=True,
                                             disable_semaphore_checks=True),
    )(
        A_x.reshape(NB, DM), A_k_cache.reshape(NB, 2, HH, SK, DH), A_v_cache.reshape(NB, 2, HH, SK, DH),
        tiles(A_wq), tiles(A_wo),
        B_x.reshape(NB, DM), tiles(B_c_kv), tiles(B_w_q), tiles(B_w_uk), tiles(B_w_uv), tiles(B_w_o),
    )
    return out.reshape(NB, 1, 2 * DM)
```
